```python
import os as _os
_os.environ.setdefault("JAX_PLATFORMS", "cpu")
import jax
import jax.numpy as jnp

def _softmax(x, axis=-1):
    return jax.nn.softmax(x, axis=axis)
def _gelu(x):
    return jax.nn.gelu(x, approximate=True)
def _silu(x):
    return jax.nn.silu(x)
def _sigmoid(x):
    return jax.nn.sigmoid(x)
def _layernorm(x, axis=-1, eps=1e-5):
    m = jnp.mean(x, axis=axis, keepdims=True)
    v = jnp.var(x, axis=axis, keepdims=True)
    return (x - m) / jnp.sqrt(v + eps)
def _scatter_add(tgt, idx, src, axis=0):
    return tgt.at[idx].add(src)
def _segment_sum(src, seg, n):
    return jax.ops.segment_sum(src, seg, n)
class _Rng:
    def __init__(self, key):
        self._k = key
    def _next(self):
        self._k, sub = jax.random.split(self._k)
        return sub
    def normal(self, shape):
        return jax.random.normal(self._next(), shape, dtype=jnp.bfloat16)
    def randint(self, lo, hi, shape):
        return jax.random.randint(self._next(), shape, lo, hi, dtype=jnp.int32)
    def uniform(self, shape, lo=0.0, hi=1.0):
        return jax.random.uniform(self._next(), shape, jnp.bfloat16, lo, hi)
    def permutation(self, n):
        return jax.random.permutation(self._next(), n)


kernel_name = 'gated_mix__mha_block__ssm_conv_h3__prompt'

def setup_inputs():
    _rng = _Rng(jax.random.key(int.from_bytes(__import__("os").urandom(4), "little")))
    _w = (lambda a: (lambda t: t.astype(jnp.bfloat16) if jnp.issubdtype(t.dtype, jnp.floating) else t)(jnp.asarray(a)))
    def _A_setup():
        B, S, D, H = 1, 2048, 640, 32
        return {
            "x": _w((lambda *s: _rng.normal(s) * 0.05)(B, S, D)),
            "wqkv": _w((lambda *s: _rng.normal(s) * 0.4)(D, 3 * D)),
            "wo": _w((lambda *s: _rng.normal(s) * 0.05)(D, D)),
        }
    _A_in = _A_setup()

    def _B_setup():
        B, S, D = 1, 2048, 640
        ks = 4
        return {
            "q": _w((lambda *s: _rng.normal(s) * 0.05)(B, S, D)),
            "k": _w((lambda *s: _rng.normal(s) * 0.4)(B, S, D)),
            "v": _w((lambda *s: _rng.normal(s) * 0.4)(B, S, D)),
            "shift_k": _w((lambda *s: _rng.normal(s) * 0.4)(D, ks) * 0.5),
            "ssm_k": _w((lambda *s: _rng.normal(s) * 0.4)(D, S) * (1.0 / S ** 0.5)),
            "ssm_D": _w((lambda *s: _rng.normal(s) * 0.4)(D)),
        }
    _B_in = _B_setup()

    return {
        "A_x": _A_in["x"],
        "A_wqkv": _A_in["wqkv"],
        "A_wo": _A_in["wo"],
        "B_q": _B_in["q"],
        "B_k": _B_in["k"],
        "B_v": _B_in["v"],
        "B_shift_k": _B_in["shift_k"],
        "B_ssm_k": _B_in["ssm_k"],
        "B_ssm_D": _B_in["ssm_D"],
        "gate_w": _w((lambda *s: _rng.normal(s) * 0.05)(640) * 16.0),
    }

def reference(A_x, A_wqkv, A_wo, B_q, B_k, B_v, B_shift_k, B_ssm_k, B_ssm_D, gate_w):
    def _A_ref(x, wqkv, wo):
        B, S, D = x.shape
        H = 32
        Dh = D // H
        qkv = (lambda x, *d: x.transpose(*d))((x @ wqkv).reshape(B, S, 3, H, Dh), 2, 0, 3, 1, 4)
        q, k, v = qkv[0], qkv[1], qkv[2]
        scores = jnp.einsum("bhqd,bhkd->bhqk", q, k) * (Dh ** -0.5)
        p = _softmax(scores, axis=-1)
        o = jnp.einsum("bhqk,bhkd->bhqd", p, v)
        return (lambda x, *d: x.transpose(*d))(o, 0, 2, 1, 3).reshape(B, S, D) @ wo

    def _B_ref(q, k, v, shift_k, ssm_k, ssm_D):
        B, S, D = q.shape
        ks = shift_k.shape[-1]
        k_pad = jnp.pad(k, ((0, 0), (ks - 1, 0), (0, 0)))
        k_shift = jnp.zeros_like(k)
        for t in range(ks):
            k_shift = k_shift + k_pad[:, t:t + S, :] * shift_k[:, ks - 1 - t][None, None, :]
        kv = k_shift * v
        L = 2 * S
        kv_pad = jnp.pad(kv, ((0, 0), (0, S), (0, 0)))
        kf_pad = jnp.pad(ssm_k, ((0, 0), (0, S)))
        kv_f = (lambda x, axes=(-2,-1): jnp.fft.rfft2(x.astype(jnp.float32), axes=axes))(kv_pad[:, None, :, :], axes=(1, 2))
        kf_f = (lambda x, axes=(-2,-1): jnp.fft.rfft2(x.astype(jnp.float32), axes=axes))(kf_pad[:, None, :], axes=(1, 2))
        kf_f = (lambda x, *d: x.transpose(*d))(kf_f, 1, 2, 0)
        y_f = kv_f * kf_f[None, :, :, :]
        y = (lambda x, s, axes=(-2,-1): jnp.fft.irfft2(x, s=s, axes=axes).astype(jnp.bfloat16))(y_f, (1, L), axes=(1, 2))[:, 0, :S, :]
        y = y + kv * ssm_D[None, None, :]
        return q * y

    x = A_x
    g = _sigmoid((x * gate_w).sum(-1, keepdims=True))
    a = _A_ref(x, A_wqkv, A_wo)
    b = _B_ref(x, B_k, B_v, B_shift_k, B_ssm_k, B_ssm_D)
    return g * a + (1 - g) * b
```

```python
import os
import numpy as np
import jax
import jax.numpy as jnp
from jax import lax
import jax.experimental.pallas as pl
import jax.experimental.pallas.tpu as pltpu

S, D, H, DH = 2048, 640, 32, 20
NP = H // 2
TB = 512
NB = S // TB
C = 128
NC = S // C
CB = TB // C
LT = D // 128
F32, BF16, I32, I8 = jnp.float32, jnp.bfloat16, jnp.int32, jnp.int8
NT = (((1,), (1,)), ((), ()))
NN = (((1,), (0,)), ((), ()))
TQ = 512
TK = 256
MB = 4
QMAX = 2038.0
MAGIC = 12582912.0
MAGIC_BITS = 0x4B400000
LOG2E = 1.4426950408889634
SCALE2 = (DH ** -0.5) * LOG2E
FORCE_SLOW = int(os.environ.get('FORCE_SLOW', '0'))
TOKR = int(os.environ.get('TOKR', '248'))


def _dft_tables():
    f = np.concatenate([np.arange(0, 128, 2), np.arange(1, 128, 2)]).astype(np.float64)
    n = np.arange(128, dtype=np.float64)
    ang = 2.0 * np.pi * (f[:, None] + 0.5) * n[None, :] / 256.0
    fwd = np.concatenate([np.cos(ang), -np.sin(ang)], axis=0)
    inv = np.concatenate([np.cos(ang).T, -np.sin(ang).T], axis=1) / 128.0
    return fwd.astype(np.float32), inv.astype(np.float32)


def _limbs(r, inv):
    t = lax.bitcast_convert_type(r * inv + MAGIC, I32) - (MAGIC_BITS - 8)
    hi = t >> 4
    lo = (t & 15) - 8
    top = (t + 120) >> 8
    return hi, lo, top


def _kernel(x_hbm, wqkv_hbm, wo_hbm, k_hbm, v_hbm, ssm_hbm, shift_ref, dvec_ref, gw_ref,
            fwd_ref, inv_ref, out_hbm,
            x_v, wqkv_v, wo_v, k_v, v_v, ssm_v, out_v,
            wt, q8, k8t, k8, vt, sq, sk, kn2, vmx, ot, kf, kvb, us, hs, hprev, ys, qkt, kn, sems):
    def cp_w(i):
        return pltpu.make_async_copy(wqkv_hbm.at[:, i * D:(i + 1) * D], wqkv_v.at[:, i * D:(i + 1) * D], sems.at[i])

    def cp_x(i):
        return pltpu.make_async_copy(x_hbm.at[0, pl.ds(i * TB, TB), :], x_v.at[pl.ds(i * TB, TB), :], sems.at[3 + i])

    cp_k = pltpu.make_async_copy(k_hbm.at[0], k_v, sems.at[7])
    cp_v = pltpu.make_async_copy(v_hbm.at[0], v_v, sems.at[8])
    cp_s = pltpu.make_async_copy(ssm_hbm, ssm_v, sems.at[9])
    cp_o = pltpu.make_async_copy(wo_hbm, wo_v, sems.at[10])

    def cp_out(i):
        return pltpu.make_async_copy(out_v.at[pl.ds(i * TB, TB), :], out_hbm.at[0, pl.ds(i * TB, TB), :],
                                     sems.at[11 + i])

    for i in range(3):
        cp_w(i).start()
    for i in range(NB):
        cp_x(i).start()
    cp_s.start()
    cp_k.start()
    cp_v.start()
    cp_o.start()

    ri = lax.broadcasted_iota(I32, (128, 128), 0)
    ci = lax.broadcasted_iota(I32, (128, 128), 1)
    eye_bf = jnp.where(ri == ci, 1.0, 0.0).astype(BF16)
    perm_i8 = jnp.where((112 - (ri & 112)) + (ri & 15) == ci, 1, 0).astype(I8)

    for i in range(3):
        cp_w(i).wait()
        blk = jnp.concatenate([wqkv_v[:, (i * LT + cb) * 128:(i * LT + cb + 1) * 128] for cb in range(LT)], axis=0)
        t = lax.dot_general(eye_bf, blk, NT, preferred_element_type=F32).astype(BF16)
        for cb in range(LT):
            wt[(i * LT + cb) * 128:(i * LT + cb + 1) * 128, :] = t[:, cb * D:(cb + 1) * D]

    low4 = lax.broadcasted_iota(I32, (8, TB), 0) < 4
    zero8 = jnp.zeros((8, TB), I32)

    def headred(a, op, red):
        mid = a[16:24]
        ma = op(op(a[0:8], a[8:16]), jnp.where(low4, mid, 0.0))
        mb = op(op(a[24:32], a[32:40]), jnp.where(low4, 0.0, mid))
        return red(ma, axis=0, keepdims=True), red(mb, axis=0, keepdims=True)

    def pairscale(ia, ib):
        a8 = jnp.broadcast_to(ia, (8, TB))
        b8 = jnp.broadcast_to(ib, (8, TB))
        return jnp.concatenate([a8, a8, jnp.where(low4, a8, b8), b8, b8], axis=0)

    def p1(tb, carry):
        t0 = pl.multiple_of(tb * TB, TB)
        cp_x(tb).wait()
        xb = x_v[pl.ds(t0, TB), :]
        for g in range(4):
            rk = lax.dot_general(wt[D + 160 * g:D + 160 * (g + 1), :], xb, NT, preferred_element_type=F32)
            for j in range(4):
                p = 4 * g + j
                r = rk[40 * j:40 * (j + 1)]
                ma, mb = headred(jnp.abs(r), jnp.maximum, jnp.max)
                na, nb = headred(r * r, jnp.add, jnp.sum)
                kn2[2 * p:2 * p + 1, pl.ds(t0, TB)] = na
                kn2[2 * p + 1:2 * p + 2, pl.ds(t0, TB)] = nb
                ma = jnp.maximum(jnp.max(ma, axis=1, keepdims=True), 1e-30)
                mb = jnp.maximum(jnp.max(mb, axis=1, keepdims=True), 1e-30)
                hi, lo, top = _limbs(r, pairscale(QMAX / ma, QMAX / mb))
                sk[tb, 2 * p:2 * p + 1, :] = jnp.broadcast_to(ma, (1, 128))
                sk[tb, 2 * p + 1:2 * p + 2, :] = jnp.broadcast_to(mb, (1, 128))
                k8t[128 * p:128 * (p + 1), :] = jnp.concatenate([hi, lo, top, zero8], axis=0).astype(I8)
        cst = 256.0 / (QMAX * QMAX) * SCALE2
        for g in range(4):
            rq = lax.dot_general(wt[160 * g:160 * (g + 1), :], xb, NT, preferred_element_type=F32)
            for j in range(4):
                p = 4 * g + j
                r = rq[40 * j:40 * (j + 1)]
                ma, mb = headred(jnp.abs(r), jnp.maximum, jnp.max)
                ma = jnp.maximum(ma, 1e-30)
                mb = jnp.maximum(mb, 1e-30)
                hi, lo, top = _limbs(r, pairscale(QMAX / ma, QMAX / mb))
                sq[2 * p:2 * p + 1, pl.ds(t0, TB)] = ma * cst
                sq[2 * p + 1:2 * p + 2, pl.ds(t0, TB)] = mb * cst
                pa, pb = [], []
                for l in (hi, top, lo):
                    pa += [l[0:16], jnp.where(low4, l[16:24], 0), zero8, zero8]
                    pb += [zero8, zero8, jnp.where(low4, 0, l[16:24]), l[24:40]]
                pa.append(zero8)
                pb.append(zero8)
                q8[2 * p, :, pl.ds(t0, TB)] = jnp.concatenate(pa, axis=0).astype(I8)
                q8[2 * p + 1, :, pl.ds(t0, TB)] = jnp.concatenate(pb, axis=0).astype(I8)
        for kt in range(TB // 128):
            kk = lax.dot_general(perm_i8, k8t[:, kt * 128:(kt + 1) * 128], NT, preferred_element_type=I32)
            kk = kk.astype(I8)
            for p in range(NP):
                k8[p, pl.ds(pl.multiple_of(t0 + kt * 128, 128), 128), :] = kk[:, 128 * p:128 * (p + 1)]
        vm = jnp.zeros((8, TB), F32)
        for g in range(4):
            rv = lax.dot_general(wt[2 * D + 160 * g:2 * D + 160 * (g + 1), :], xb, NT, preferred_element_type=F32)
            vm = jnp.maximum(vm, jnp.max(jnp.abs(rv).reshape(20, 8, TB), axis=0))
            for j in range(4):
                p = 4 * g + j
                r = rv[40 * j:40 * (j + 1)]
                mid = r[16:24]
                vt[2 * p, :, pl.ds(t0, TB)] = jnp.concatenate([r[0:16], jnp.where(low4, mid, 1.0)], axis=0)
                vt[2 * p + 1, :, pl.ds(t0, TB)] = jnp.concatenate([jnp.where(low4, 1.0, mid), r[24:40]], axis=0)
        vmx[:, pl.ds(t0, TB)] = vm
        return carry

    lax.fori_loop(0, NB, p1, 0)

    cst = 256.0 / (QMAX * QMAX) * SCALE2
    qinf = jnp.max(sq[...], axis=1, keepdims=True) * (SCALE2 / cst)
    kl2 = jnp.max(kn2[...], axis=1, keepdims=True)
    bad = jnp.where(qinf * qinf * kl2 * DH <= 60.0 * 60.0, 0.0, 1.0)
    for tb in range(NB):
        ksum = jnp.sum(kn2[:, tb * TB:(tb + 1) * TB], axis=1, keepdims=True)
        kinf = sk[tb][:, 0:1]
        bad = bad + jnp.where(kinf * kinf * (DH * TB) <= 64.0 * ksum, 0.0, 1.0)
    nbad = jnp.sum(bad) + jnp.sum(jnp.where(vmx[...] <= 2.0 ** 50, 0.0, 1.0))
    fast = nbad == (0.0 if not FORCE_SLOW else -1.0)

    cp_s.wait()
    cp_k.wait()
    cp_v.wait()
    kf[0:8, :] = jnp.zeros((8, D), F32)
    hprev[...] = jnp.zeros((256, D), F32)
    sh = shift_ref[...].astype(F32)

    def put(ref, m, c, val):
        for ft in range(16):
            for lt in range(LT):
                ref[ft, (lt * 3 + m) * NC + c] = val[8 * ft:8 * (ft + 1), 128 * lt:128 * (lt + 1)]

    def p3(tb, carry):
        t0 = pl.multiple_of(tb * TB, TB)
        hb = jnp.concatenate([ssm_v[:, pl.ds(pl.multiple_of(t0 + i * C, C), C)] for i in range(CB)], axis=0)
        hh = lax.dot_general(fwd_ref[...], hb, NT, preferred_element_type=F32)
        prev = hprev[...]
        for i in range(CB):
            cur = hh[:, i * D:(i + 1) * D]
            cr = jnp.concatenate([cur[0:64] - prev[128:192], cur[64:128] + prev[192:256]], axis=0)
            cim = jnp.concatenate([cur[128:192] + prev[0:64], cur[192:256] - prev[64:128]], axis=0)
            put(hs, 0, tb * CB + i, cr)
            put(hs, 1, tb * CB + i, cim - cr)
            put(hs, 2, tb * CB + i, cim + cr)
            prev = cur
        hprev[...] = prev
        kf[pl.ds(t0 + 8, TB), :] = k_v[pl.ds(t0, TB), :].astype(F32)
        kvs = []
        for i in range(CB):
            r0 = pl.multiple_of(t0 + i * C, C)
            win = kf[pl.ds(r0, C + 8), :]
            ks = win[8:] * sh[0:1] + win[7:C + 7] * sh[1:2] + win[6:C + 6] * sh[2:3] + win[5:C + 5] * sh[3:4]
            kv = (ks * v_v[pl.ds(r0, C), :].astype(F32)).astype(BF16)
            kvb[pl.ds(r0, C), :] = kv
            kvs.append(kv)
        u = jnp.dot(fwd_ref[...], jnp.concatenate(kvs, axis=1), preferred_element_type=F32)
        for i in range(CB):
            a, b = u[:128, i * D:(i + 1) * D], u[128:, i * D:(i + 1) * D]
            put(us, 0, tb * CB + i, a + b)
            put(us, 1, tb * CB + i, a)
            put(us, 2, tb * CB + i, b)
        return carry

    lax.fori_loop(0, NB, p3, 0)

    def mac_units(ft):
        f0 = pl.multiple_of(ft * 8, 8)
        f1 = pl.multiple_of(128 + ft * 8, 8)
        units = []
        for lt in range(LT):
            ls = slice(lt * 128, (lt + 1) * 128)
            for ab in range(NC // MB):
                st = {}
                for m in range(3):
                    for cb in range(ab + 1):
                        def unit(z=None, ls=ls, lt=lt, ab=ab, m=m, cb=cb, st=st):
                            if cb == 0:
                                st[m] = [None] * MB if m == 0 else list(st[0])
                            o = st[m]
                            sl = (lt * 3 + m) * NC
                            uu = [us[ft, sl + cb * MB + i] for i in range(MB)]
                            if z is not None:
                                uu = [t + z for t in uu]
                            base = (ab - cb) * MB
                            hh = {}
                            for i in range(MB):
                                for j in range(MB):
                                    d = base + i - j
                                    if d < 0:
                                        continue
                                    if d not in hh:
                                        hh[d] = hs[ft, sl + d]
                                    t = uu[j] * hh[d]
                                    o[i] = t if o[i] is None else (o[i] - t if m == 2 else o[i] + t)
                            if cb == ab and m > 0:
                                for i in range(MB):
                                    ys[ab * MB + i, pl.ds(f0 if m == 2 else f1, 8), ls] = o[i]
                        units.append(unit)
        return units

    def finish(p, hh, acc, cols):
        if hh == 0:
            ot[p, 0:24, cols] = acc * (1.0 / acc[20:21])
        else:
            b = acc * (1.0 / acc[0:1])
            ot[p, 20:24, cols] = b[4:8]
            ot[p, 24:40, cols] = b[8:24]

    def p2(p, carry):
        steps = [(j, hh, c) for j in range(S // TQ) for hh in range(2) for c in range(S // TK)]
        units = mac_units(p)
        accs, ps, tok = {}, {}, {}

        def qk(j, hh, c):
            h = 2 * p + hh
            q = q8[h, :, j * TQ:(j + 1) * TQ]
            w = sq[pl.ds(h, 1), j * TQ:(j + 1) * TQ] * jnp.concatenate(
                [sk[c * TK // TB, pl.ds(h, 1), :]] * (TQ // 128), axis=1)
            s = jnp.dot(k8[p, c * TK:(c + 1) * TK, :], q, preferred_element_type=I32)
            e = jnp.exp2(s.astype(F32) * w)
            parts = []
            for t in range(TK // 128):
                parts += [e[t * 128 + 16 * i:t * 128 + 16 * (i + 1)] for i in reversed(range(8))]
            ps[(j, hh, c)] = jnp.concatenate(parts, axis=0).astype(BF16)
            tok[0] = e[TOKR:TOKR + 8, TQ - 128:TQ]

        def pv(j, hh, c):
            h = 2 * p + hh
            o = lax.dot_general(vt[h, :, c * TK:(c + 1) * TK], ps.pop((j, hh, c)), NN, preferred_element_type=F32)
            accs[(j, hh)] = o if c == 0 else o + accs[(j, hh)]
            if c == S // TK - 1:
                finish(p, hh, accs.pop((j, hh)), slice(j * TQ, (j + 1) * TQ))

        n = len(steps)
        ui = 0
        for i in range(n + 1):
            if i < n:
                qk(*steps[i])
            if i >= 1:
                pv(*steps[i - 1])
            while ui < len(units) and ui * (n - 1) < i * len(units):
                units[ui](jnp.minimum(tok[0], 0.0))
                ui += 1
        assert ui == len(units)
        return carry

    @pl.when(fast)
    def _():
        lax.fori_loop(0, NP, p2, 0)

    @pl.when(jnp.logical_not(fast))
    def _():
        def fb1(tb, carry):
            t0 = pl.multiple_of(tb * TB, TB)
            qkt[:, pl.ds(t0, TB)] = lax.dot_general(wt[0:2 * D, :], x_v[pl.ds(t0, TB), :], NT,
                                                    preferred_element_type=F32)
            return carry

        lax.fori_loop(0, NB, fb1, 0)

        def fb2(p, carry):
            r0 = pl.multiple_of(40 * p, 8)

            def tr(kt, c2):
                c0 = pl.multiple_of(kt * 128, 128)
                blk = jnp.concatenate([qkt[pl.ds(D + r0, 40), pl.ds(c0, 128)], jnp.zeros((88, 128), F32)], axis=0)
                kn[pl.ds(c0, 128), :] = lax.dot_general(eye_bf, blk.astype(BF16), NT,
                                                        preferred_element_type=F32).astype(BF16)
                return c2

            lax.fori_loop(0, S // 128, tr, 0)
            rows = lax.broadcasted_iota(I32, (40, TQ), 0)
            for hh in range(2):
                def qtile(j, c2, hh=hh):
                    c0 = pl.multiple_of(j * TQ, TQ)
                    qm = jnp.where((rows >= DH * hh) & (rows < DH * hh + DH), qkt[pl.ds(r0, 40), pl.ds(c0, TQ)], 0.0)
                    qm = jnp.concatenate([qm, jnp.zeros((88, TQ), F32)], axis=0).astype(BF16)

                    def kchunk(c, st):
                        m, acc = st
                        k0 = pl.multiple_of(c * TK, TK)
                        s = jnp.dot(kn[pl.ds(k0, TK), :], qm, preferred_element_type=F32) * SCALE2
                        mn = jnp.maximum(m, jnp.max(s, axis=0, keepdims=True))
                        e = jnp.exp2(s - mn).astype(BF16)
                        o = lax.dot_general(vt[2 * p + hh, :, pl.ds(k0, TK)], e, NN, preferred_element_type=F32)
                        return mn, o + acc * jnp.exp2(m - mn)

                    m0 = jnp.full((1, TQ), -jnp.inf, F32)
                    _, acc = lax.fori_loop(0, S // TK, kchunk, (m0, jnp.zeros((24, TQ), F32)))
                    finish(p, hh, acc, pl.ds(c0, TQ))
                    return c2

                lax.fori_loop(0, S // TQ, qtile, 0)
            for u in mac_units(p):
                u()
            return carry

        lax.fori_loop(0, NP, fb2, 0)

    cp_o.wait()
    gw = gw_ref[...].astype(F32)
    dv = dvec_ref[...].astype(F32)

    def p4(tb, carry):
        t0 = pl.multiple_of(tb * TB, TB)
        ob = jnp.concatenate([ot[:, :, pl.ds(pl.multiple_of(t0 + i * C, C), C)].reshape(D, C) for i in range(CB)], axis=0)
        o = lax.dot_general(eye_bf, ob.astype(BF16), NT, preferred_element_type=F32).astype(BF16)
        yb = jnp.concatenate([ys[tb * CB + i] for i in range(CB)], axis=1).astype(BF16)
        y = jnp.dot(inv_ref[...], yb, preferred_element_type=F32)
        o = jnp.concatenate([o[:, i * D:(i + 1) * D] for i in range(CB)], axis=0)
        y = jnp.concatenate([y[:, i * D:(i + 1) * D] for i in range(CB)], axis=0)
        a = jnp.dot(o, wo_v[...], preferred_element_type=F32)
        xf = x_v[pl.ds(t0, TB), :].astype(F32)
        g = jax.nn.sigmoid(jnp.sum(xf * gw, axis=-1, keepdims=True))
        b = xf * (y + kvb[pl.ds(t0, TB), :].astype(F32) * dv)
        out_v[pl.ds(t0, TB), :] = (b + g * (a - b)).astype(BF16)
        cp_out(tb).start()
        return carry

    lax.fori_loop(0, NB, p4, 0)
    for i in range(NB):
        cp_out(i).wait()


@jax.jit
def pallas_gated_mix__mha_block__ssm_conv_h3__prompt_kernel(A_x, A_wqkv, A_wo, B_q, B_k, B_v, B_shift_k, B_ssm_k, B_ssm_D, gate_w):
    fwd, inv = _dft_tables()
    vm = pl.BlockSpec(memory_space=pltpu.VMEM)
    hbm = pl.BlockSpec(memory_space=pl.ANY)
    return pl.pallas_call(
        _kernel,
        out_shape=jax.ShapeDtypeStruct((1, S, D), BF16),
        in_specs=[hbm] * 6 + [vm] * 5,
        out_specs=hbm,
        scratch_shapes=[
            pltpu.VMEM((S, D), BF16),
            pltpu.VMEM((D, 3 * D), BF16),
            pltpu.VMEM((D, D), BF16),
            pltpu.VMEM((S, D), BF16),
            pltpu.VMEM((S, D), BF16),
            pltpu.VMEM((D, S), BF16),
            pltpu.VMEM((S, D), BF16),
            pltpu.VMEM((3 * D, D), BF16),
            pltpu.VMEM((H, 128, S), I8),
            pltpu.VMEM((NP * 128, TB), I8),
            pltpu.VMEM((NP, S, 128), I8),
            pltpu.VMEM((H, 24, S), F32),
            pltpu.VMEM((H, S), F32),
            pltpu.VMEM((NB, H, 128), F32),
            pltpu.VMEM((H, S), F32),
            pltpu.VMEM((8, S), F32),
            pltpu.VMEM((NP, 40, S), F32),
            pltpu.VMEM((S + 8, D), F32),
            pltpu.VMEM((S, D), BF16),
            pltpu.VMEM((16, LT * 3 * NC, 8, 128), F32),
            pltpu.VMEM((16, LT * 3 * NC, 8, 128), F32),
            pltpu.VMEM((256, D), F32),
            pltpu.VMEM((NC, 256, D), F32),
            pltpu.VMEM((2 * D, S), F32),
            pltpu.VMEM((S, 128), BF16),
            pltpu.SemaphoreType.DMA((15,)),
        ],
        compiler_params=pltpu.CompilerParams(vmem_limit_bytes=120 * 1024 * 1024),
        name="gmix",
    )(A_x, A_wqkv, A_wo, B_k, B_v, B_ssm_k, B_shift_k.T, B_ssm_D.reshape(1, D), gate_w.reshape(1, D),
      jnp.asarray(fwd, BF16), jnp.asarray(inv, BF16))
```

```python
import numpy as np
import jax
import jax.numpy as jnp
from jax import lax
import jax.experimental.pallas as pl
import jax.experimental.pallas.tpu as pltpu

S, D, H, DH = 2048, 640, 32, 20
NP = H // 2
TB = 512
NB = S // TB
C = 128
NC = S // C
LT = D // 128
NKT = S // 128
TQ = 512
JL = S // TQ - 1
MB = 4
PU = 2
OB = 256
OC = OB // C
OU = 4
W_FIN = 0.3
PEEL = "qxQQvQQVkVKKKKVV"

F32, BF16, I32, I16, I8 = jnp.float32, jnp.bfloat16, jnp.int32, jnp.int16, jnp.int8
NT = (((1,), (1,)), ((), ()))
NN = (((1,), (0,)), ((), ()))
QMAX = 2038.0
MAGIC = 12582912.0
MAGIC_BITS = 0x4B400000
SCALE2 = (DH ** -0.5) * 1.4426950408889634
DEQ = 256.0 / (QMAX * QMAX) * SCALE2


def _dft_tables():
    r = np.arange(64, dtype=np.float64)
    f = np.concatenate([2 * r, 127 - 2 * r])
    n = np.arange(128, dtype=np.float64)
    ang = 2.0 * np.pi * (f[:, None] + 0.5) * n[None, :] / 256.0
    fwd = np.concatenate([np.cos(ang), -np.sin(ang)], axis=0)
    inv = np.concatenate([np.cos(ang[:64]).T, -np.sin(ang[:64]).T], axis=1) / 128.0
    inv = np.concatenate([inv[0::2], inv[1::2]], axis=0)
    return np.concatenate([fwd, inv], axis=0).astype(np.float32)


def _limbs(r, inv):
    t = lax.bitcast_convert_type(r * inv + MAGIC, I32) - (MAGIC_BITS - 8)
    return t >> 4, (t & 15) - 8, (t + 120) >> 8


def _kernel(x_hbm, wqkv_hbm, wo_hbm, k_hbm, v_hbm, ssm_hbm, shift_hbm, dvec_hbm, gw_hbm, dft_hbm, out_hbm,
            x_v, wqkv_v, wo_v, k_v, v_v, ssm_v, out_v, shift_v, dvec_v, gw_v, dft_v,
            wt, q8, k8, vt, sq, sk, kn2, vmx, ot, kvb, us, hs, ys, ysc, qkt, kn, pcar, acar, sems):
    def cp_w(i):
        return pltpu.make_async_copy(wqkv_hbm.at[:, i * D:(i + 1) * D], wqkv_v.at[:, i * D:(i + 1) * D],
                                     sems.at[i])

    def cp_x(i):
        return pltpu.make_async_copy(x_hbm.at[0, pl.ds(i * TB, TB), :], x_v.at[pl.ds(i * TB, TB), :],
                                     sems.at[3 + i])

    late = [
        pltpu.make_async_copy(ssm_hbm, ssm_v, sems.at[7]),
        pltpu.make_async_copy(k_hbm.at[0], k_v.at[pl.ds(16, S), :], sems.at[7]),
        pltpu.make_async_copy(v_hbm.at[0], v_v, sems.at[7]),
        pltpu.make_async_copy(wo_hbm, wo_v, sems.at[7]),
        pltpu.make_async_copy(shift_hbm, shift_v, sems.at[7]),
        pltpu.make_async_copy(dvec_hbm, dvec_v, sems.at[7]),
        pltpu.make_async_copy(gw_hbm, gw_v, sems.at[7]),
        pltpu.make_async_copy(dft_hbm, dft_v, sems.at[7]),
    ]

    def cp_out(i):
        r0 = pl.multiple_of(i * OB, OB)
        return pltpu.make_async_copy(out_v.at[pl.ds(r0, OB), :], out_hbm.at[0, pl.ds(r0, OB), :], sems.at[8])

    widx = {"q": 0, "k": 1, "v": 2}
    for ch in PEEL:
        if ch in widx:
            cp_w(widx[ch]).start()
        elif ch == "x":
            cp_x(0).start()
    for i in range(1, NB):
        cp_x(i).start()
    for cp in late:
        cp.start()

    k_v[0:16, :] = jnp.zeros((16, D), BF16)

    low4 = lax.broadcasted_iota(I32, (8, TB), 0) < 4
    zero8 = jnp.zeros((8, TB), I32)

    def headred(a, op, red):
        mid = a[16:24]
        ma = op(op(a[0:8], a[8:16]), jnp.where(low4, mid, 0.0))
        mb = op(op(a[24:32], a[32:40]), jnp.where(low4, 0.0, mid))
        return red(ma, axis=0, keepdims=True), red(mb, axis=0, keepdims=True)

    def pairscale(ia, ib):
        a8 = jnp.broadcast_to(ia, (8, TB))
        b8 = jnp.broadcast_to(ib, (8, TB))
        return jnp.concatenate([a8, a8, jnp.where(low4, a8, b8), b8, b8], axis=0)

    def proj(part, g, t0):
        return lax.dot_general(wt[part * D + 160 * g:part * D + 160 * (g + 1), :], x_v[pl.ds(t0, TB), :], NT,
                               preferred_element_type=F32)

    def kgrp(g, tb, t0):
        rk = proj(1, g, t0)
        for j in range(4):
            p = 4 * g + j
            r = rk[40 * j:40 * (j + 1)]
            ma, mb = headred(jnp.abs(r), jnp.maximum, jnp.max)
            na, nb = headred(r * r, jnp.add, jnp.sum)
            kn2[2 * p:2 * p + 1, pl.ds(t0, TB)] = na
            kn2[2 * p + 1:2 * p + 2, pl.ds(t0, TB)] = nb
            ma = jnp.maximum(jnp.max(ma, axis=1, keepdims=True), 1e-30)
            mb = jnp.maximum(jnp.max(mb, axis=1, keepdims=True), 1e-30)
            hi, lo, top = _limbs(r, pairscale(QMAX / ma, QMAX / mb))
            sk[tb, 2 * p:2 * p + 1, :] = jnp.broadcast_to(ma, (1, 128))
            sk[tb, 2 * p + 1:2 * p + 2, :] = jnp.broadcast_to(mb, (1, 128))
            kk = jnp.concatenate([hi, lo, top, zero8], axis=0).astype(I16).T
            kk = jnp.concatenate([kk[kt * 128 + 16 * i:kt * 128 + 16 * (i + 1)]
                                  for kt in range(TB // 128) for i in reversed(range(8))], axis=0)
            k8[p, pl.ds(t0, TB), :] = kk.astype(I8)

    def qgrp(g, tb, t0):
        rq = proj(0, g, t0)
        for j in range(4):
            p = 4 * g + j
            r = rq[40 * j:40 * (j + 1)]
            ma, mb = headred(jnp.abs(r), jnp.maximum, jnp.max)
            ma = jnp.maximum(ma, 1e-30)
            mb = jnp.maximum(mb, 1e-30)
            hi, lo, top = _limbs(r, pairscale(QMAX / ma, QMAX / mb))
            sq[2 * p:2 * p + 1, pl.ds(t0, TB)] = ma * DEQ
            sq[2 * p + 1:2 * p + 2, pl.ds(t0, TB)] = mb * DEQ
            pa, pb = [], []
            for l in (hi, top, lo):
                pa += [l[0:16], jnp.where(low4, l[16:24], 0), zero8, zero8]
                pb += [zero8, zero8, jnp.where(low4, 0, l[16:24]), l[24:40]]
            q8[2 * p, :, pl.ds(t0, TB)] = jnp.concatenate(pa + [zero8], axis=0).astype(I8)
            q8[2 * p + 1, :, pl.ds(t0, TB)] = jnp.concatenate(pb + [zero8], axis=0).astype(I8)

    def vgrp(g, tb, t0):
        rv = proj(2, g, t0)
        vmx[8 * g:8 * (g + 1), pl.ds(t0, TB)] = jnp.max(jnp.abs(rv).reshape(20, 8, TB), axis=0)
        for j in range(4):
            p = 4 * g + j
            r = rv[40 * j:40 * (j + 1)]
            mid = r[16:24]
            vt[2 * p, :, pl.ds(t0, TB)] = jnp.concatenate([r[0:16], jnp.where(low4, mid, 1.0)], axis=0)
            vt[2 * p + 1, :, pl.ds(t0, TB)] = jnp.concatenate([jnp.where(low4, 1.0, mid), r[24:40]], axis=0)

    grp = {"K": kgrp, "Q": qgrp, "V": vgrp}
    cnt = {"K": 0, "Q": 0, "V": 0}
    for ch in PEEL:
        if ch in widx:
            i = widx[ch]
            cp_w(i).wait()
            wt[i * D:(i + 1) * D, :] = wqkv_v[:, i * D:(i + 1) * D].T
        elif ch == "x":
            cp_x(0).wait()
        else:
            grp[ch](cnt[ch], 0, 0)
            cnt[ch] += 1

    def p1(tb, carry):
        t0 = pl.multiple_of(tb * TB, TB)
        cp_x(tb).wait()
        for ch in "QKV":
            for g in range(4):
                grp[ch](g, tb, t0)
        return carry

    lax.fori_loop(1, NB, p1, 0)

    for cp in late:
        cp.wait()

    qinf = jnp.max(sq[...], axis=1, keepdims=True) * (SCALE2 / DEQ)
    kl2 = jnp.max(kn2[...], axis=1, keepdims=True)
    bad = jnp.where(qinf * qinf * kl2 * DH <= 60.0 * 60.0, 0.0, 1.0)
    for tb in range(NB):
        ksum = jnp.sum(kn2[:, tb * TB:(tb + 1) * TB], axis=1, keepdims=True)
        kinf = sk[tb][:, 0:1]
        bad = bad + jnp.where(kinf * kinf * (DH * TB) <= 64.0 * ksum, 0.0, 1.0)
    bad = bad + jnp.where(jnp.max(vmx[...], axis=1, keepdims=True) <= 2.0 ** 50, 0.0, 1.0)
    fast = jnp.sum(bad) == 0.0

    def put(ref, m, c, val):
        for ft in range(16):
            for lt in range(LT):
                ref[ft, (lt * 2 + m) * NC + c] = val[8 * ft:8 * (ft + 1), 128 * lt:128 * (lt + 1)]

    sh = shift_v[...].astype(F32)
    prev = None
    for c in range(NC):
        r0 = c * C
        cur = lax.dot_general(dft_v[0:256, :], ssm_v[:, r0:r0 + C], NT, preferred_element_type=F32)
        if prev is None:
            put(hs, 0, c, cur[0:128])
            put(hs, 1, c, cur[128:256])
        else:
            put(hs, 0, c, jnp.concatenate([cur[0:64] - prev[128:192], cur[64:128] + prev[192:256]], axis=0))
            put(hs, 1, c, jnp.concatenate([cur[128:192] + prev[0:64], cur[192:256] - prev[64:128]], axis=0))
        prev = cur
        win = k_v[r0:r0 + C + 16, :].astype(F32)
        ks = (win[16:] * sh[0:1] + win[15:C + 15] * sh[1:2]
              + win[14:C + 14] * sh[2:3] + win[13:C + 13] * sh[3:4])
        kv = (ks * v_v[r0:r0 + C, :].astype(F32)).astype(BF16)
        kvb[r0:r0 + C, :] = kv
        u = jnp.dot(dft_v[0:256, :], kv, preferred_element_type=F32)
        put(us, 0, c, u[:128])
        put(us, 1, c, u[128:])

    def mac_tasks(ft, lts):
        f0 = pl.multiple_of(ft * 8, 8)
        f1 = pl.multiple_of(128 + ft * 8, 8)
        tasks = []
        for li, lt in enumerate(lts):
            for ab in range(NC // MB):
                st = {"r": [None] * MB, "i": [None] * MB, "id": (len(tasks), li, ab)}
                for cb in range(ab + 1):
                    for m in range(2):
                        for i in range(MB):
                            js = [j for j in range(MB) if (ab - cb) * MB + i - j >= 0]

                            def task(cache, z, lt=lt, ab=ab, m=m, cb=cb, i=i, js=js, st=st):
                                yr, yi = st["r"], st["i"]

                                def ld(ref, name, slot, pin):
                                    key = (st["id"], name, slot)
                                    if key not in cache:
                                        val = ref[ft, lt * 2 * NC + slot]
                                        cache[key] = val + z if (pin and z is not None) else val
                                    return cache[key]

                                for j in js:
                                    hv = ld(hs, "h", m * NC + (ab - cb) * MB + i - j, True)
                                    ta = ld(us, "u", cb * MB + j, False) * hv
                                    tb_ = ld(us, "u", NC + cb * MB + j, False) * hv
                                    if m == 0:
                                        yr[i] = ta if yr[i] is None else yr[i] + ta
                                        yi[i] = tb_ if yi[i] is None else yi[i] + tb_
                                    else:
                                        yr[i] = yr[i] - tb_
                                        yi[i] = yi[i] + ta
                                if cb == ab and m == 1:
                                    ys[ab * MB + i, lt, pl.ds(f0, 8), :] = yr[i]
                                    ys[ab * MB + i, lt, pl.ds(f1, 8), :] = yi[i]

                            tasks.append((4 * len(js), task))
        return tasks

    def finish(p, hh, acc, cols):
        if hh == 0:
            ot[p, 0:24, cols] = acc * (1.0 / acc[20:21])
        else:
            b = acc * (1.0 / acc[0:1])
            ot[p, 20:24, cols] = b[4:8]
            ot[p, 24:40, cols] = b[8:24]

    def pv_tile(h, t, pt, acc):
        o = lax.dot_general(vt[h, :, t * 128:(t + 1) * 128], pt, NN, preferred_element_type=F32)
        return o if acc is None else o + acc

    def drain(p):
        acc = acar[...]
        for i in range(2):
            acc = pv_tile(2 * p + 1, NKT - 2 + i, pcar[i], acc)
        finish(p, 1, acc, slice(JL * TQ, (JL + 1) * TQ))

    def p2(pb, carry):
        steps = [(pi, j, hh, t0) for pi in range(PU) for j in range(S // TQ) for hh in range(2)
                 for t0 in range(0, NKT, 2)]
        tasks = [(c, t, pi) for pi in range(PU) for c, t in mac_tasks(pb * PU + pi, range(LT))]
        accs, pend = {}, []

        def qk(pi, j, hh, t0):
            p = pb * PU + pi
            h = 2 * p + hh
            w = sq[pl.ds(h, 1), j * TQ:(j + 1) * TQ] * jnp.concatenate(
                [sk[t0 * 128 // TB, pl.ds(h, 1), :]] * (TQ // 128), axis=1)
            s = jnp.dot(k8[p, t0 * 128:(t0 + 2) * 128, :], q8[h, :, j * TQ:(j + 1) * TQ],
                        preferred_element_type=I32)
            for t in range(2):
                e = jnp.exp2(s[t * 128:(t + 1) * 128].astype(F32) * w)
                pt = jnp.concatenate([e[16 * i:16 * (i + 1)] for i in reversed(range(8))], axis=0).astype(BF16)
                pend.append((pi, j, hh, t0 + t, pt))
            return e[120:128, TQ - 128:TQ]

        def pv(pi, j, hh, t, pt):
            p = pb * PU + pi
            accs[(j, hh)] = pv_tile(2 * p + hh, t, pt, accs.get((j, hh)))
            if t == NKT - 1:
                finish(p, hh, accs.pop((j, hh)), slice(j * TQ, (j + 1) * TQ))

        n = len(steps)
        wts = [W_FIN if steps[i][3] == 0 else 1.0 for i in range(n - 1)]
        total = float(sum(t[0] for t in tasks))
        ti, done, cum = 0, 0.0, 0.0
        for i in range(n):
            last_e = qk(*steps[i])
            if i == 0:
                drain(jnp.maximum(pb * PU - 1, 0))
            while len(pend) > 2:
                pv(*pend.pop(0))
            if i < n - 1:
                z = jnp.minimum(last_e, 0.0)
                cum += wts[i] / sum(wts) * total
                caches = {}
                while ti < len(tasks) and (done + tasks[ti][0] / 2 <= cum or i == n - 2):
                    tasks[ti][1](caches.setdefault(tasks[ti][2], {}), z)
                    done += tasks[ti][0]
                    ti += 1
        for i in range(2):
            pcar[i] = pend[i][4]
        acar[...] = accs.pop((JL, 1))
        return carry

    pcar[...] = jnp.zeros((2, 128, TQ), BF16)
    acar[...] = jnp.ones((24, TQ), F32)

    @pl.when(fast)
    def _():
        lax.fori_loop(0, NP // PU, p2, 0)
        drain(NP - 1)

    @pl.when(jnp.logical_not(fast))
    def _():
        def fb1(i, carry):
            r0 = pl.multiple_of((i // NB) * 160, 32)
            t0 = pl.multiple_of((i % NB) * TB, TB)
            qkt[pl.ds(r0, 160), pl.ds(t0, TB)] = lax.dot_general(
                wt[pl.ds(r0, 160), :], x_v[pl.ds(t0, TB), :], NT, preferred_element_type=F32)
            return carry

        lax.fori_loop(0, 8 * NB, fb1, 0)

        def fb2(p, carry):
            r0 = pl.multiple_of(40 * p, 8)

            def tr(kt, c2):
                c0 = pl.multiple_of(kt * 128, 128)
                blk = jnp.concatenate([qkt[pl.ds(D + r0, 40), pl.ds(c0, 128)], jnp.zeros((88, 128), F32)], axis=0)
                kn[pl.ds(c0, 128), :] = blk.T.astype(BF16)
                return c2

            lax.fori_loop(0, NKT, tr, 0)
            rows = lax.broadcasted_iota(I32, (40, TQ), 0)
            for hh in range(2):
                def qtile(j, c2, hh=hh):
                    c0 = pl.multiple_of(j * TQ, TQ)
                    qm = jnp.where((rows >= DH * hh) & (rows < DH * hh + DH),
                                   qkt[pl.ds(r0, 40), pl.ds(c0, TQ)], 0.0)
                    qm = jnp.concatenate([qm, jnp.zeros((88, TQ), F32)], axis=0).astype(BF16)

                    def kchunk(c, st):
                        m, acc = st
                        k0 = pl.multiple_of(c * 128, 128)
                        s = jnp.dot(kn[pl.ds(k0, 128), :], qm, preferred_element_type=F32) * SCALE2
                        mn = jnp.maximum(m, jnp.max(s, axis=0, keepdims=True))
                        e = jnp.exp2(s - mn).astype(BF16)
                        o = lax.dot_general(vt[2 * p + hh, :, pl.ds(k0, 128)], e, NN, preferred_element_type=F32)
                        return mn, o + acc * jnp.exp2(m - mn)

                    m0 = jnp.full((1, TQ), -jnp.inf, F32)
                    _, acc = lax.fori_loop(0, NKT, kchunk, (m0, jnp.zeros((24, TQ), F32)))
                    finish(p, hh, acc, pl.ds(c0, TQ))
                    return c2

                lax.fori_loop(0, S // TQ, qtile, 0)

            def mac(lt, c2):
                cache = {}
                for _, task in mac_tasks(p, [lt]):
                    task(cache, None)
                return c2

            lax.fori_loop(0, LT, mac, 0)
            return carry

        lax.fori_loop(0, NP, fb2, 0)

    gw = gw_v[...].astype(F32).reshape(1, D)
    dv = dvec_v[...].astype(F32).reshape(1, D)

    def p4(it, carry):
        for sb in range(OU):
            ob = it * OU + sb
            t0 = pl.multiple_of(ob * OB, OB)
            s0 = (sb % 2) * OC * LT
            yv = jnp.concatenate([ys[ob * OC + i, lt] for i in range(OC) for lt in range(LT)], axis=1)
            ar, br, ai, bi = yv[0:64], yv[64:128], yv[128:192], yv[192:256]
            ye = jnp.dot(dft_v[256:320, :], jnp.concatenate([ar + br, ai - bi], axis=0).astype(BF16),
                         preferred_element_type=F32)
            yo = jnp.dot(dft_v[320:384, :], jnp.concatenate([ar - br, ai + bi], axis=0).astype(BF16),
                         preferred_element_type=F32)
            for i in range(OC * LT):
                ysc[s0 + i, pl.ds(0, 64, stride=2), :] = ye[:, i * 128:(i + 1) * 128]
                ysc[s0 + i, pl.ds(1, 64, stride=2), :] = yo[:, i * 128:(i + 1) * 128]
            y = jnp.concatenate(
                [jnp.concatenate([ysc[s0 + i * LT + lt] for lt in range(LT)], axis=1) for i in range(OC)], axis=0)
            o = ot[:, :, pl.ds(t0, OB)].reshape(D, OB).astype(BF16).T
            a = jnp.dot(o, wo_v[...], preferred_element_type=F32)
            xf = x_v[pl.ds(t0, OB), :].astype(F32)
            g = jax.nn.sigmoid(jnp.sum(xf * gw, axis=-1, keepdims=True))
            b = xf * (y + kvb[pl.ds(t0, OB), :].astype(F32) * dv)
            out_v[pl.ds(t0, OB), :] = (b + g * (a - b)).astype(BF16)
            cp_out(ob).start()
        return carry

    lax.fori_loop(0, S // (OB * OU), p4, 0)
    for i in range(S // OB):
        cp_out(i).wait()


@jax.jit
def pallas_gated_mix__mha_block__ssm_conv_h3__prompt_kernel(A_x, A_wqkv, A_wo, B_q, B_k, B_v, B_shift_k, B_ssm_k, B_ssm_D, gate_w):
    del B_q
    hbm = pl.BlockSpec(memory_space=pl.ANY)
    return pl.pallas_call(
        _kernel,
        out_shape=jax.ShapeDtypeStruct((1, S, D), BF16),
        in_specs=[hbm] * 10,
        out_specs=hbm,
        scratch_shapes=[
            pltpu.VMEM((S, D), BF16),
            pltpu.VMEM((D, 3 * D), BF16),
            pltpu.VMEM((D, D), BF16),
            pltpu.VMEM((S + 16, D), BF16),
            pltpu.VMEM((S, D), BF16),
            pltpu.VMEM((D, S), BF16),
            pltpu.VMEM((S, D), BF16),
            pltpu.VMEM((4, D), BF16),
            pltpu.VMEM((D,), BF16),
            pltpu.VMEM((D,), BF16),
            pltpu.VMEM((384, 128), BF16),
            pltpu.VMEM((3 * D, D), BF16),
            pltpu.VMEM((H, 128, S), I8),
            pltpu.VMEM((NP, S, 128), I8),
            pltpu.VMEM((H, 24, S), F32),
            pltpu.VMEM((H, S), F32),
            pltpu.VMEM((NB, H, 128), F32),
            pltpu.VMEM((H, S), F32),
            pltpu.VMEM((32, S), F32),
            pltpu.VMEM((NP, 40, S), F32),
            pltpu.VMEM((S, D), BF16),
            pltpu.VMEM((16, LT * 2 * NC, 8, 128), F32),
            pltpu.VMEM((16, LT * 2 * NC, 8, 128), F32),
            pltpu.VMEM((NC, LT, 256, 128), F32),
            pltpu.VMEM((2 * OC * LT, 128, 128), F32),
            pltpu.VMEM((2 * D, S), F32),
            pltpu.VMEM((S, 128), BF16),
            pltpu.VMEM((2, 128, TQ), BF16),
            pltpu.VMEM((24, TQ), F32),
            pltpu.SemaphoreType.DMA((9,)),
        ],
        compiler_params=pltpu.CompilerParams(vmem_limit_bytes=120 * 1024 * 1024),
        name="gmix",
    )(A_x, A_wqkv, A_wo, B_k, B_v, B_ssm_k, B_shift_k.T, B_ssm_D, gate_w, jnp.asarray(_dft_tables(), BF16))
```

```python
import numpy as np
import jax
import jax.numpy as jnp
from jax import lax
import jax.experimental.pallas as pl
import jax.experimental.pallas.tpu as pltpu

S, D, H, DH = 2048, 640, 32, 20
NP = H // 2
TB = 512
NB = S // TB
C = 128
NC = S // C
LT = D // 128
NKT = S // 128
TQ = 512
JL = S // TQ - 1
MB = 4
PU = 2
OBS = (4, 2, 1, 1)
W_FIN = 0.3
PEEL = "aaaqaaxQQQvQVkVKKKKVV"
KA = 128

F32, BF16, I32, I16, I8 = jnp.float32, jnp.bfloat16, jnp.int32, jnp.int16, jnp.int8
NT = (((1,), (1,)), ((), ()))
NN = (((1,), (0,)), ((), ()))
QMAX = 2038.0
MAGIC = 12582912.0
MAGIC_BITS = 0x4B400000
SCALE2 = (DH ** -0.5) * 1.4426950408889634
DEQ = 256.0 / (QMAX * QMAX) * SCALE2


def _dft_tables():
    r = np.arange(64, dtype=np.float64)
    f = np.concatenate([2 * r, 127 - 2 * r])
    n = np.arange(128, dtype=np.float64)
    ang = 2.0 * np.pi * (f[:, None] + 0.5) * n[None, :] / 256.0
    fwd = np.concatenate([np.cos(ang), -np.sin(ang)], axis=0)
    inv = np.concatenate([np.cos(ang[:64]).T, -np.sin(ang[:64]).T], axis=1) / 128.0
    inv = np.concatenate([inv[0::2], inv[1::2]], axis=0)
    fwd = fwd.reshape(2, 16, 8, 128).transpose(1, 0, 2, 3).reshape(256, 128)
    return np.concatenate([fwd, inv], axis=0).astype(np.float32)


def _limbs(r, inv):
    t = lax.bitcast_convert_type(r * inv + MAGIC, I32) - (MAGIC_BITS - 8)
    return t >> 4, (t & 15) - 8, (t + 120) >> 8


def _qscale(m):
    r = pl.reciprocal(m, approx=True)
    return (r * QMAX) * (2.0 - m * r)


def _kernel(x_hbm, wqkv_hbm, wo_hbm, k_hbm, v_hbm, ssm_hbm, shift_hbm, dvec_hbm, gw_hbm, dft_hbm, out_hbm,
            x_v, wqkv_v, wo_v, k_v, v_v, ssm_v, out_v, shift_v, dvec_v, gw_v, dft_v,
            wt, q8, k8, vt, sq, sk, kst, vmx, ot, kvb, us, hs, ys, ysc, qkt, kn, pcar, acar, part0, sems):
    def cp_w(i):
        return pltpu.make_async_copy(wqkv_hbm.at[KA:D, i * D:(i + 1) * D], wqkv_v.at[KA:D, i * D:(i + 1) * D],
                                     sems.at[i])

    cp_wa = pltpu.make_async_copy(wqkv_hbm.at[0:KA, :], wqkv_v.at[0:KA, :], sems.at[9])
    cp_xa = pltpu.make_async_copy(x_hbm.at[0, 0:TB, 0:KA], x_v.at[0:TB, 0:KA], sems.at[9])
    cp_xb = pltpu.make_async_copy(x_hbm.at[0, 0:TB, KA:D], x_v.at[0:TB, KA:D], sems.at[3])

    def cp_x(i):
        return pltpu.make_async_copy(x_hbm.at[0, pl.ds(i * TB, TB), :], x_v.at[pl.ds(i * TB, TB), :],
                                     sems.at[3 + i])

    late = [
        pltpu.make_async_copy(ssm_hbm, ssm_v, sems.at[7]),
        pltpu.make_async_copy(k_hbm.at[0], k_v.at[pl.ds(16, S), :], sems.at[7]),
        pltpu.make_async_copy(v_hbm.at[0], v_v, sems.at[7]),
        pltpu.make_async_copy(wo_hbm, wo_v, sems.at[7]),
        pltpu.make_async_copy(shift_hbm, shift_v, sems.at[7]),
        pltpu.make_async_copy(dvec_hbm, dvec_v, sems.at[7]),
        pltpu.make_async_copy(gw_hbm, gw_v, sems.at[7]),
        pltpu.make_async_copy(dft_hbm, dft_v, sems.at[7]),
    ]

    def cp_out(c0, oc):
        r0 = pl.multiple_of(c0 * C, C)
        return pltpu.make_async_copy(out_v.at[pl.ds(r0, oc * C), :], out_hbm.at[0, pl.ds(r0, oc * C), :], sems.at[8])

    widx = {"q": 0, "k": 1, "v": 2}
    cp_wa.start()
    cp_xa.start()
    for ch in PEEL:
        if ch in widx:
            cp_w(widx[ch]).start()
        elif ch == "x":
            cp_xb.start()
    for i in range(1, NB):
        cp_x(i).start()
    for cp in late:
        cp.start()

    k_v[0:16, :] = jnp.zeros((16, D), BF16)

    low4 = lax.broadcasted_iota(I32, (8, TB), 0) < 4
    zero8 = jnp.zeros((8, TB), I32)

    def headred(a, op, red):
        mid = a[16:24]
        ma = op(op(a[0:8], a[8:16]), jnp.where(low4, mid, 0.0))
        mb = op(op(a[24:32], a[32:40]), jnp.where(low4, 0.0, mid))
        return red(ma, axis=0, keepdims=True), red(mb, axis=0, keepdims=True)

    def pairscale(ia, ib):
        a8 = jnp.broadcast_to(ia, (8, TB))
        b8 = jnp.broadcast_to(ib, (8, TB))
        return jnp.concatenate([a8, a8, jnp.where(low4, a8, b8), b8, b8], axis=0)

    def lanefold(a, op):
        return op(op(a[:, 0:128], a[:, 128:256]), op(a[:, 256:384], a[:, 384:512]))

    memo = {}

    def proj(part, g, t0):
        r0 = part * D + 160 * g
        if memo["peel"]:
            return lax.dot_general(wt[r0:r0 + 160, KA:D], x_v[0:TB, KA:D], NT,
                                   preferred_element_type=F32) + part0[r0:r0 + 160, :]
        if g % 2 == 0:
            memo["wide"] = lax.dot_general(wt[r0:r0 + 320, :], x_v[pl.ds(t0, TB), :], NT,
                                           preferred_element_type=F32)
        return memo["wide"][160 * (g % 2):160 * (g % 2 + 1)]

    def kgrp(g, tb, t0):
        rk = proj(1, g, t0)
        for j in range(4):
            p = 4 * g + j
            r = rk[40 * j:40 * (j + 1)]
            ab = jnp.abs(r)
            mida, midb = jnp.where(low4, ab[16:24], 0.0), jnp.where(low4, 0.0, ab[16:24])
            ms = []
            for hh, (u0, u1, u2) in enumerate(((ab[0:8], ab[8:16], mida), (ab[24:32], ab[32:40], midb))):
                l1 = u0 + u1 + u2
                l1m = jnp.sum(jnp.max(lanefold(l1, jnp.maximum), axis=1, keepdims=True), axis=0, keepdims=True)
                l1s = jnp.sum(jnp.sum(lanefold(l1, jnp.add), axis=1, keepdims=True), axis=0, keepdims=True)
                kst[0, tb, 2 * p + hh:2 * p + hh + 1, :] = jnp.broadcast_to(l1m, (1, 128))
                kst[1, tb, 2 * p + hh:2 * p + hh + 1, :] = jnp.broadcast_to(l1s, (1, 128))
                m = lanefold(jnp.maximum(jnp.maximum(u0, u1), u2), jnp.maximum)
                m = jnp.max(jnp.max(m, axis=0, keepdims=True), axis=1, keepdims=True)
                ms.append(jnp.maximum(m, 1e-30))
            ma, mb = ms
            hi, lo, top = _limbs(r, pairscale(_qscale(ma), _qscale(mb)))
            sk[tb, 2 * p:2 * p + 1, :] = jnp.broadcast_to(ma, (1, 128))
            sk[tb, 2 * p + 1:2 * p + 2, :] = jnp.broadcast_to(mb, (1, 128))
            kk = jnp.concatenate([hi, lo, top, zero8], axis=0).astype(I16).T
            kk = jnp.concatenate([kk[kt * 128 + 16 * i:kt * 128 + 16 * (i + 1)]
                                  for kt in range(TB // 128) for i in reversed(range(8))], axis=0)
            k8[p, pl.ds(t0, TB), :] = kk.astype(I8)

    def qgrp(g, tb, t0):
        rq = proj(0, g, t0)
        for j in range(4):
            p = 4 * g + j
            r = rq[40 * j:40 * (j + 1)]
            ma, mb = headred(jnp.abs(r), jnp.maximum, jnp.max)
            ma = jnp.maximum(ma, 1e-30)
            mb = jnp.maximum(mb, 1e-30)
            hi, lo, top = _limbs(r, pairscale(_qscale(ma), _qscale(mb)))
            sq[2 * p:2 * p + 1, pl.ds(t0, TB)] = ma * DEQ
            sq[2 * p + 1:2 * p + 2, pl.ds(t0, TB)] = mb * DEQ
            pa, pb = [], []
            for l in (hi, top, lo):
                pa += [l[0:16], jnp.where(low4, l[16:24], 0), zero8, zero8]
                pb += [zero8, zero8, jnp.where(low4, 0, l[16:24]), l[24:40]]
            q8[2 * p, :, pl.ds(t0, TB)] = jnp.concatenate(pa + [zero8], axis=0).astype(I8)
            q8[2 * p + 1, :, pl.ds(t0, TB)] = jnp.concatenate(pb + [zero8], axis=0).astype(I8)

    def vgrp(g, tb, t0):
        rv = proj(2, g, t0)
        vmx[8 * g:8 * (g + 1), pl.ds(t0, TB)] = jnp.max(jnp.abs(rv).reshape(20, 8, TB), axis=0)
        for j in range(4):
            p = 4 * g + j
            r = rv[40 * j:40 * (j + 1)]
            mid = r[16:24]
            vt[2 * p, :, pl.ds(t0, TB)] = jnp.concatenate([r[0:16], jnp.where(low4, mid, 1.0)], axis=0)
            vt[2 * p + 1, :, pl.ds(t0, TB)] = jnp.concatenate([jnp.where(low4, 1.0, mid), r[24:40]], axis=0)

    grp = {"K": kgrp, "Q": qgrp, "V": vgrp}
    cnt = {"K": 0, "Q": 0, "V": 0}
    memo["peel"] = True
    cp_wa.wait()
    cp_xa.wait()
    na = PEEL.count("a")
    ra = 3 * D // na
    ia = 0
    for ch in PEEL:
        if ch in widx:
            i = widx[ch]
            cp_w(i).wait()
            wt[i * D:(i + 1) * D, KA:D] = wqkv_v[KA:D, i * D:(i + 1) * D].T
        elif ch == "x":
            cp_xb.wait()
        elif ch == "a":
            rows = slice(ia * ra, (ia + 1) * ra)
            wa = wqkv_v[0:KA, rows].T
            wt[rows, 0:KA] = wa
            part0[rows, :] = lax.dot_general(wa, x_v[0:TB, 0:KA], NT, preferred_element_type=F32)
            ia += 1
        else:
            grp[ch](cnt[ch], 0, 0)
            cnt[ch] += 1
    memo["peel"] = False

    def p1(tb, carry):
        t0 = pl.multiple_of(tb * TB, TB)
        cp_x(tb).wait()
        for ch in "QKV":
            for g in range(4):
                grp[ch](g, tb, t0)
        return carry

    lax.fori_loop(1, NB, p1, 0)

    for cp in late:
        cp.wait()

    qinf = jnp.max(sq[...], axis=1, keepdims=True) * (SCALE2 / DEQ)
    bad = jnp.where(jnp.max(vmx[...], axis=1, keepdims=True) <= 2.0 ** 50, 0.0, 1.0)
    for tb in range(NB):
        bad = bad + jnp.where(qinf * kst[0, tb] <= 60.0, 0.0, 1.0)
        bad = bad + jnp.where(qinf + kst[0, tb] <= 1e15, 0.0, 1.0)
        bad = bad + jnp.where(sk[tb] * (DH * TB) <= 10.0 * kst[1, tb] + 1e-25, 0.0, 1.0)
    fast = jnp.sum(bad) == 0.0

    def reim(val):
        n = val.shape[1]
        val = val.reshape(16, 16, n)
        return val[:, 0:8], val[:, 8:16]

    sh = shift_v[...].astype(F32)
    hprev = [None] * LT

    def hdft(cg, lt):
        ls = slice(lt * 128, (lt + 1) * 128)
        hb = jnp.concatenate([ssm_v[ls, (cg * 4 + i) * C:(cg * 4 + i + 1) * C] for i in range(4)], axis=0)
        hr, hi = reim(lax.dot_general(dft_v[0:256, :], hb, NT, preferred_element_type=F32))
        for i in range(4):
            cr, ci = hr[:, :, i * 128:(i + 1) * 128], hi[:, :, i * 128:(i + 1) * 128]
            if hprev[lt] is None:
                hs[:, cg * 4 + i, :, ls] = cr
                hs[:, NC + cg * 4 + i, :, ls] = ci
            else:
                pr, pi = hprev[lt]
                hs[:, cg * 4 + i, :, ls] = jnp.concatenate([cr[0:8] - pi[0:8], cr[8:] + pi[8:]], axis=0)
                hs[:, NC + cg * 4 + i, :, ls] = jnp.concatenate([ci[0:8] + pr[0:8], ci[8:] - pr[8:]], axis=0)
            hprev[lt] = (cr, ci)

    def udft(c):
        r0 = c * C
        win = k_v[r0:r0 + C + 16, :].astype(F32)
        ks = (win[16:] * sh[0:1] + win[15:C + 15] * sh[1:2]
              + win[14:C + 14] * sh[2:3] + win[13:C + 13] * sh[3:4])
        kv = (ks * v_v[r0:r0 + C, :].astype(F32)).astype(BF16)
        kvb[r0:r0 + C, :] = kv
        ur, ui = reim(jnp.dot(dft_v[0:256, :], kv, preferred_element_type=F32))
        us[:, c] = ur
        us[:, NC + c] = ui

    hjobs = [(cg, lt) for cg in range(NC // 4) for lt in range(LT)]
    for c in range(NC):
        while len(hjobs) * NC > (NC - 1 - c) * LT * NC // 4 and hjobs:
            hdft(*hjobs.pop(0))
        udft(c)

    def mac_tasks(ft, lts):
        tasks = []

        def lanes(lt):
            return slice(lt * 128, (lt + 1) * 128) if isinstance(lt, int) else pl.ds(pl.multiple_of(lt * 128, 128), 128)

        for li, lt in enumerate(lts):
            for ab in range(NC // MB):
                st = {"r": [None] * MB, "i": [None] * MB, "id": (len(tasks), li, ab)}
                for cb in range(ab + 1):
                    for m in range(2):
                        for i in range(MB):
                            js = [j for j in range(MB) if (ab - cb) * MB + i - j >= 0]

                            def task(cache, z, lt=lt, ab=ab, m=m, cb=cb, i=i, js=js, st=st):
                                yr, yi = st["r"], st["i"]

                                def ld(ref, name, slot, pin):
                                    key = (st["id"], name, slot)
                                    if key not in cache:
                                        val = ref[ft, slot, :, lanes(lt)]
                                        cache[key] = val + z if (pin and z is not None) else val
                                    return cache[key]

                                for j in js:
                                    hv = ld(hs, "h", m * NC + (ab - cb) * MB + i - j, True)
                                    ta = ld(us, "u", cb * MB + j, False) * hv
                                    tb_ = ld(us, "u", NC + cb * MB + j, False) * hv
                                    if m == 0:
                                        yr[i] = ta if yr[i] is None else yr[i] + ta
                                        yi[i] = tb_ if yi[i] is None else yi[i] + tb_
                                    else:
                                        yr[i] = yr[i] - tb_
                                        yi[i] = yi[i] + ta
                                if cb == ab and m == 1:
                                    ys[ft, ab * MB + i, :, lanes(lt)] = yr[i]
                                    ys[ft, NC + ab * MB + i, :, lanes(lt)] = yi[i]

                            tasks.append((4 * len(js), task))
        return tasks

    def finish(p, hh, acc, cols):
        if hh == 0:
            ot[p, 0:24, cols] = acc * (1.0 / acc[20:21])
        else:
            b = acc * (1.0 / acc[0:1])
            ot[p, 20:24, cols] = b[4:8]
            ot[p, 24:40, cols] = b[8:24]

    def pv_tile(h, t, pt, acc):
        o = lax.dot_general(vt[h, :, t * 128:(t + 1) * 128], pt, NN, preferred_element_type=F32)
        return o if acc is None else o + acc

    def drain(p):
        acc = acar[...]
        for i in range(2):
            acc = pv_tile(2 * p + 1, NKT - 2 + i, pcar[i], acc)
        finish(p, 1, acc, slice(JL * TQ, (JL + 1) * TQ))

    def p2(pb, carry):
        steps = [(pi, j, hh, t0) for pi in range(PU) for j in range(S // TQ) for hh in range(2)
                 for t0 in range(0, NKT, 2)]
        tasks = [(c, t, pi) for pi in range(PU) for c, t in mac_tasks(pb * PU + pi, range(LT))]
        accs, pend = {}, []

        def qk(pi, j, hh, t0):
            p = pb * PU + pi
            h = 2 * p + hh
            w = sq[pl.ds(h, 1), j * TQ:(j + 1) * TQ] * jnp.concatenate(
                [sk[t0 * 128 // TB, pl.ds(h, 1), :]] * (TQ // 128), axis=1)
            s = jnp.dot(k8[p, t0 * 128:(t0 + 2) * 128, :], q8[h, :, j * TQ:(j + 1) * TQ],
                        preferred_element_type=I32)
            for t in range(2):
                e = jnp.exp2(s[t * 128:(t + 1) * 128].astype(F32) * w)
                pt = jnp.concatenate([e[16 * i:16 * (i + 1)] for i in reversed(range(8))], axis=0).astype(BF16)
                pend.append((pi, j, hh, t0 + t, pt))
            return e[120:128, TQ - 128:TQ]

        def pv(pi, j, hh, t, pt):
            p = pb * PU + pi
            accs[(j, hh)] = pv_tile(2 * p + hh, t, pt, accs.get((j, hh)))
            if t == NKT - 1:
                finish(p, hh, accs.pop((j, hh)), slice(j * TQ, (j + 1) * TQ))

        n = len(steps)
        wts = [W_FIN if steps[i][3] == 0 else 1.0 for i in range(n - 1)]
        total = float(sum(t[0] for t in tasks))
        ti, done, cum = 0, 0.0, 0.0
        for i in range(n):
            last_e = qk(*steps[i])
            if i == 0:
                drain(jnp.maximum(pb * PU - 1, 0))
            while len(pend) > 2:
                pv(*pend.pop(0))
            if i < n - 1:
                z = jnp.minimum(last_e, 0.0)
                cum += wts[i] / sum(wts) * total
                caches = {}
                while ti < len(tasks) and (done + tasks[ti][0] / 2 <= cum or i == n - 2):
                    tasks[ti][1](caches.setdefault(tasks[ti][2], {}), z)
                    done += tasks[ti][0]
                    ti += 1
        for i in range(2):
            pcar[i] = pend[i][4]
        acar[...] = accs.pop((JL, 1))
        return carry

    pcar[...] = jnp.zeros((2, 128, TQ), BF16)
    acar[...] = jnp.ones((24, TQ), F32)

    def attn_fast():
        lax.fori_loop(0, NP // PU, p2, 0)
        drain(NP - 1)

    def attn_general():
        def fb1(i, carry):
            r0 = pl.multiple_of((i // NB) * 160, 32)
            t0 = pl.multiple_of((i % NB) * TB, TB)
            qkt[pl.ds(r0, 160), pl.ds(t0, TB)] = lax.dot_general(
                wt[pl.ds(r0, 160), :], x_v[pl.ds(t0, TB), :], NT, preferred_element_type=F32)
            return carry

        lax.fori_loop(0, 8 * NB, fb1, 0)

        def fb2(p, carry):
            r0 = pl.multiple_of(40 * p, 8)

            def tr(kt, c2):
                c0 = pl.multiple_of(kt * 128, 128)
                blk = jnp.concatenate([qkt[pl.ds(D + r0, 40), pl.ds(c0, 128)], jnp.zeros((88, 128), F32)], axis=0)
                kn[pl.ds(c0, 128), :] = blk.T.astype(BF16)
                return c2

            lax.fori_loop(0, NKT, tr, 0)
            rows = lax.broadcasted_iota(I32, (40, TQ), 0)
            for hh in range(2):
                def qtile(j, c2, hh=hh):
                    c0 = pl.multiple_of(j * TQ, TQ)
                    qm = jnp.where((rows >= DH * hh) & (rows < DH * hh + DH),
                                   qkt[pl.ds(r0, 40), pl.ds(c0, TQ)], 0.0)
                    qm = jnp.concatenate([qm, jnp.zeros((88, TQ), F32)], axis=0).astype(BF16)

                    def kchunk(c, st):
                        m, acc = st
                        k0 = pl.multiple_of(c * 128, 128)
                        s = jnp.dot(kn[pl.ds(k0, 128), :], qm, preferred_element_type=F32) * SCALE2
                        mn = jnp.maximum(m, jnp.max(s, axis=0, keepdims=True))
                        e = jnp.exp2(s - mn).astype(BF16)
                        o = lax.dot_general(vt[2 * p + hh, :, pl.ds(k0, 128)], e, NN, preferred_element_type=F32)
                        return mn, o + acc * jnp.exp2(m - mn)

                    m0 = jnp.full((1, TQ), -jnp.inf, F32)
                    _, acc = lax.fori_loop(0, NKT, kchunk, (m0, jnp.zeros((24, TQ), F32)))
                    finish(p, hh, acc, pl.ds(c0, TQ))
                    return c2

                lax.fori_loop(0, S // TQ, qtile, 0)

            def mac(lt, c2):
                cache = {}
                for _, task in mac_tasks(p, [lt]):
                    task(cache, None)
                return c2

            lax.fori_loop(0, LT, mac, 0)
            return carry

        lax.fori_loop(0, NP, fb2, 0)

    lax.cond(fast, attn_fast, attn_general)

    gw = gw_v[...].astype(F32).reshape(1, D)
    dv = dvec_v[...].astype(F32).reshape(1, D)

    def p4(it, carry):
        off = 0
        for sb, oc in enumerate(OBS):
            c0 = it * sum(OBS) + off
            off += oc
            ob = oc * C
            t0 = pl.multiple_of(c0 * C, C)
            s0 = (sb % 2) * max(OBS) * LT
            yr = jnp.concatenate([ys[:, c0 + i].reshape(128, D) for i in range(oc)], axis=1)
            yi = jnp.concatenate([ys[:, NC + c0 + i].reshape(128, D) for i in range(oc)], axis=1)
            ar, br, ai, bi = yr[0:64], yr[64:128], yi[0:64], yi[64:128]
            ye = jnp.dot(dft_v[256:320, :], jnp.concatenate([ar + br, ai - bi], axis=0).astype(BF16),
                         preferred_element_type=F32)
            yo = jnp.dot(dft_v[320:384, :], jnp.concatenate([ar - br, ai + bi], axis=0).astype(BF16),
                         preferred_element_type=F32)
            for i in range(oc * LT):
                ysc[s0 + i, pl.ds(0, 64, stride=2), :] = ye[:, i * 128:(i + 1) * 128]
                ysc[s0 + i, pl.ds(1, 64, stride=2), :] = yo[:, i * 128:(i + 1) * 128]
            y = jnp.concatenate(
                [jnp.concatenate([ysc[s0 + i * LT + lt] for lt in range(LT)], axis=1) for i in range(oc)], axis=0)
            o = ot[:, :, pl.ds(t0, ob)].reshape(D, ob).astype(BF16).T
            a = jnp.dot(o, wo_v[...], preferred_element_type=F32)
            xf = x_v[pl.ds(t0, ob), :].astype(F32)
            g = jax.nn.sigmoid(jnp.sum(xf * gw, axis=-1, keepdims=True))
            b = xf * (y + kvb[pl.ds(t0, ob), :].astype(F32) * dv)
            out_v[pl.ds(t0, ob), :] = (b + g * (a - b)).astype(BF16)
            cp_out(c0, oc).start()
        return carry

    lax.fori_loop(0, NC // sum(OBS), p4, 0)
    cp_out(0, NC).wait()


@jax.jit
def pallas_gated_mix__mha_block__ssm_conv_h3__prompt_kernel(A_x, A_wqkv, A_wo, B_q, B_k, B_v, B_shift_k, B_ssm_k, B_ssm_D, gate_w):
    del B_q
    hbm = pl.BlockSpec(memory_space=pl.ANY)
    return pl.pallas_call(
        _kernel,
        out_shape=jax.ShapeDtypeStruct((1, S, D), BF16),
        in_specs=[hbm] * 10,
        out_specs=hbm,
        scratch_shapes=[
            pltpu.VMEM((S, D), BF16),
            pltpu.VMEM((D, 3 * D), BF16),
            pltpu.VMEM((D, D), BF16),
            pltpu.VMEM((S + 16, D), BF16),
            pltpu.VMEM((S, D), BF16),
            pltpu.VMEM((D, S), BF16),
            pltpu.VMEM((S, D), BF16),
            pltpu.VMEM((4, D), BF16),
            pltpu.VMEM((D,), BF16),
            pltpu.VMEM((D,), BF16),
            pltpu.VMEM((384, 128), BF16),
            pltpu.VMEM((3 * D, D), BF16),
            pltpu.VMEM((H, 128, S), I8),
            pltpu.VMEM((NP, S, 128), I8),
            pltpu.VMEM((H, 24, S), F32),
            pltpu.VMEM((H, S), F32),
            pltpu.VMEM((NB, H, 128), F32),
            pltpu.VMEM((2, NB, H, 128), F32),
            pltpu.VMEM((32, S), F32),
            pltpu.VMEM((NP, 40, S), F32),
            pltpu.VMEM((S, D), BF16),
            pltpu.VMEM((16, 2 * NC, 8, D), F32),
            pltpu.VMEM((16, 2 * NC, 8, D), F32),
            pltpu.VMEM((16, 2 * NC, 8, D), F32),
            pltpu.VMEM((2 * max(OBS) * LT, 128, 128), F32),
            pltpu.VMEM((2 * D, S), F32),
            pltpu.VMEM((S, 128), BF16),
            pltpu.VMEM((2, 128, TQ), BF16),
            pltpu.VMEM((24, TQ), F32),
            pltpu.VMEM((3 * D, TB), F32),
            pltpu.SemaphoreType.DMA((10,)),
        ],
        compiler_params=pltpu.CompilerParams(vmem_limit_bytes=120 * 1024 * 1024),
        name="gmix",
    )(A_x, A_wqkv, A_wo, B_k, B_v, B_ssm_k, B_shift_k.T, B_ssm_D, gate_w, jnp.asarray(_dft_tables(), BF16))
```

```python
import numpy as np
import jax
import jax.numpy as jnp
from jax import lax
import jax.experimental.pallas as pl
import jax.experimental.pallas.tpu as pltpu

S, D, H, DH = 2048, 640, 32, 20
NP = H // 2
TB = 512
NB = S // TB
C = 128
NC = S // C
LT = D // 128
NKT = S // 128
TQ = 512
JL = S // TQ - 1
MB = 4
PU = 2
OBS = (4, 2, 1, 1)
SPLIT = 0.7
W_FIN = 0.6
PEEL = "aaaqaaxQQQvQVkVKKKKVV"
KA = 128

F32, BF16, I32, I16, I8 = jnp.float32, jnp.bfloat16, jnp.int32, jnp.int16, jnp.int8
NT = (((1,), (1,)), ((), ()))
NN = (((1,), (0,)), ((), ()))
QMAX = 2038.0
MAGIC = 12582912.0
MAGIC_BITS = 0x4B400000
SCALE2 = (DH ** -0.5) * 1.4426950408889634
DEQ = 256.0 / (QMAX * QMAX) * SCALE2


def _dft_tables():
    r = np.arange(64, dtype=np.float64)
    f = np.concatenate([2 * r, 127 - 2 * r])
    n = np.arange(128, dtype=np.float64)
    ang = 2.0 * np.pi * (f[:, None] + 0.5) * n[None, :] / 256.0
    fwd = np.concatenate([np.cos(ang), -np.sin(ang)], axis=0)
    inv = np.concatenate([np.cos(ang[:64]).T, -np.sin(ang[:64]).T], axis=1) / 128.0
    inv = np.concatenate([inv[0::2], inv[1::2]], axis=0)
    fwd = fwd.reshape(2, 16, 8, 128).transpose(1, 0, 2, 3).reshape(256, 128)
    return np.concatenate([fwd, inv], axis=0).astype(np.float32)


def _limbs(r, inv):
    t = lax.bitcast_convert_type(r * inv + MAGIC, I32) - (MAGIC_BITS - 8)
    return t >> 4, (t & 15) - 8, (t + 120) >> 8


def _recip(m):
    r = pl.reciprocal(m, approx=True)
    return r * (2.0 - m * r)


def _qscale(m):
    r = pl.reciprocal(m, approx=True)
    return (r * QMAX) * (2.0 - m * r)


def _kernel(x_hbm, wqkv_hbm, wo_hbm, k_hbm, v_hbm, ssm_hbm, shift_hbm, dvec_hbm, gw_hbm, dft_hbm, out_hbm,
            x_v, wqkv_v, wo_v, k_v, v_v, ssm_v, out_v, shift_v, dvec_v, gw_v, dft_v,
            wt, q8, k8, vt, sq, sk, kst, vmx, ot, kvb, us, hs, ys, ysc, qkt, kn, pcar, acar, part0, sems):
    def cp_w(i):
        return pltpu.make_async_copy(wqkv_hbm.at[KA:D, i * D:(i + 1) * D], wqkv_v.at[KA:D, i * D:(i + 1) * D],
                                     sems.at[i])

    cp_wa = pltpu.make_async_copy(wqkv_hbm.at[0:KA, :], wqkv_v.at[0:KA, :], sems.at[9])
    cp_xa = pltpu.make_async_copy(x_hbm.at[0, 0:TB, 0:KA], x_v.at[0:TB, 0:KA], sems.at[9])
    cp_xb = pltpu.make_async_copy(x_hbm.at[0, 0:TB, KA:D], x_v.at[0:TB, KA:D], sems.at[3])

    def cp_x(i):
        return pltpu.make_async_copy(x_hbm.at[0, pl.ds(i * TB, TB), :], x_v.at[pl.ds(i * TB, TB), :],
                                     sems.at[3 + i])

    late = [
        pltpu.make_async_copy(ssm_hbm, ssm_v, sems.at[7]),
        pltpu.make_async_copy(k_hbm.at[0], k_v.at[pl.ds(16, S), :], sems.at[7]),
        pltpu.make_async_copy(v_hbm.at[0], v_v, sems.at[7]),
        pltpu.make_async_copy(wo_hbm, wo_v, sems.at[7]),
        pltpu.make_async_copy(shift_hbm, shift_v, sems.at[7]),
        pltpu.make_async_copy(dvec_hbm, dvec_v, sems.at[7]),
        pltpu.make_async_copy(gw_hbm, gw_v, sems.at[7]),
        pltpu.make_async_copy(dft_hbm, dft_v, sems.at[7]),
    ]

    def cp_out(c0, oc):
        r0 = pl.multiple_of(c0 * C, C)
        return pltpu.make_async_copy(out_v.at[pl.ds(r0, oc * C), :], out_hbm.at[0, pl.ds(r0, oc * C), :], sems.at[8])

    widx = {"q": 0, "k": 1, "v": 2}
    cp_wa.start()
    cp_xa.start()
    for ch in PEEL:
        if ch in widx:
            cp_w(widx[ch]).start()
        elif ch == "x":
            cp_xb.start()
    for i in range(1, NB):
        cp_x(i).start()
    for cp in late:
        cp.start()

    k_v[0:16, :] = jnp.zeros((16, D), BF16)

    low4 = lax.broadcasted_iota(I32, (8, TB), 0) < 4

    def headred(a, op, red):
        mid = a[16:24]
        ma = op(op(a[0:8], a[8:16]), jnp.where(low4, mid, 0.0))
        mb = op(op(a[24:32], a[32:40]), jnp.where(low4, 0.0, mid))
        return red(ma, axis=0, keepdims=True), red(mb, axis=0, keepdims=True)

    def pairscale(ia, ib):
        a8 = jnp.broadcast_to(ia, (8, TB))
        b8 = jnp.broadcast_to(ib, (8, TB))
        return jnp.concatenate([a8, a8, jnp.where(low4, a8, b8), b8, b8], axis=0)

    def slots(l1, l2, l3, mask):
        r2 = pltpu.roll(l2[16:24], 4, 0)
        m3 = l3[16:24]
        a = [l1[0:16], l2[0:16], l3[0:16], jnp.where(low4, l1[16:24], r2), jnp.where(low4, m3, 0) if mask else m3]
        b = [l1[24:40], l2[24:40], l3[24:40], jnp.where(low4, r2, l1[16:24]), jnp.where(low4, 0, m3) if mask else m3]
        return a, b

    def lanefold(a, op):
        return op(op(a[:, 0:128], a[:, 128:256]), op(a[:, 256:384], a[:, 384:512]))

    memo = {}

    def proj(part, g, t0):
        r0 = part * D + 160 * g
        if memo["peel"]:
            return lax.dot_general(wt[r0:r0 + 160, KA:D], x_v[0:TB, KA:D], NT,
                                   preferred_element_type=F32) + part0[r0:r0 + 160, :]
        if g % 2 == 0:
            memo["wide"] = lax.dot_general(wt[r0:r0 + 320, :], x_v[pl.ds(t0, TB), :], NT,
                                           preferred_element_type=F32)
        return memo["wide"][160 * (g % 2):160 * (g % 2 + 1)]

    def kgrp(g, tb, t0):
        rk = proj(1, g, t0)
        for j in range(4):
            p = 4 * g + j
            r = rk[40 * j:40 * (j + 1)]
            ab = jnp.abs(r)
            mida, midb = jnp.where(low4, ab[16:24], 0.0), jnp.where(low4, 0.0, ab[16:24])
            ms = []
            for hh, (u0, u1, u2) in enumerate(((ab[0:8], ab[8:16], mida), (ab[24:32], ab[32:40], midb))):
                l1 = u0 + u1 + u2
                l1m = jnp.sum(jnp.max(lanefold(l1, jnp.maximum), axis=1, keepdims=True), axis=0, keepdims=True)
                l1s = jnp.sum(jnp.sum(lanefold(l1, jnp.add), axis=1, keepdims=True), axis=0, keepdims=True)
                kst[0, tb, 2 * p + hh:2 * p + hh + 1, :] = jnp.broadcast_to(l1m, (1, 128))
                kst[1, tb, 2 * p + hh:2 * p + hh + 1, :] = jnp.broadcast_to(l1s, (1, 128))
                m = lanefold(jnp.maximum(jnp.maximum(u0, u1), u2), jnp.maximum)
                m = jnp.max(jnp.max(m, axis=0, keepdims=True), axis=1, keepdims=True)
                ms.append(jnp.maximum(m, 1e-30))
            ma, mb = ms
            hi, lo, top = _limbs(r, pairscale(_qscale(ma), _qscale(mb)))
            sk[tb, 2 * p:2 * p + 1, :] = jnp.broadcast_to(ma, (1, 128))
            sk[tb, 2 * p + 1:2 * p + 2, :] = jnp.broadcast_to(mb, (1, 128))
            ka, kb = slots(hi, lo, top, False)
            kk = jnp.concatenate(ka + kb, axis=0).astype(I16).T
            kk = jnp.concatenate([kk[kt * 128 + 16 * i:kt * 128 + 16 * (i + 1)]
                                  for kt in range(TB // 128) for i in reversed(range(8))], axis=0)
            k8[p, pl.ds(t0, TB), :] = kk.astype(I8)

    def qgrp(g, tb, t0):
        rq = proj(0, g, t0)
        for j in range(4):
            p = 4 * g + j
            r = rq[40 * j:40 * (j + 1)]
            ma, mb = headred(jnp.abs(r), jnp.maximum, jnp.max)
            ma = jnp.maximum(ma, 1e-30)
            mb = jnp.maximum(mb, 1e-30)
            hi, lo, top = _limbs(r, pairscale(_qscale(ma), _qscale(mb)))
            sq[2 * p:2 * p + 1, pl.ds(t0, TB)] = ma * DEQ
            sq[2 * p + 1:2 * p + 2, pl.ds(t0, TB)] = mb * DEQ
            pa, pb = slots(hi, top, lo, True)
            q8[2 * p, :, pl.ds(t0, TB)] = jnp.concatenate(pa, axis=0).astype(I8)
            q8[2 * p + 1, :, pl.ds(t0, TB)] = jnp.concatenate(pb, axis=0).astype(I8)

    def vgrp(g, tb, t0):
        rv = proj(2, g, t0)
        vmx[8 * g:8 * (g + 1), pl.ds(t0, TB)] = jnp.max(jnp.abs(rv).reshape(20, 8, TB), axis=0)
        for j in range(4):
            p = 4 * g + j
            r = rv[40 * j:40 * (j + 1)]
            mid = r[16:24]
            vt[2 * p, :, pl.ds(t0, TB)] = jnp.concatenate([r[0:16], jnp.where(low4, mid, 1.0)], axis=0)
            vt[2 * p + 1, :, pl.ds(t0, TB)] = jnp.concatenate([jnp.where(low4, 1.0, mid), r[24:40]], axis=0)

    grp = {"K": kgrp, "Q": qgrp, "V": vgrp}
    cnt = {"K": 0, "Q": 0, "V": 0}
    memo["peel"] = True
    cp_wa.wait()
    cp_xa.wait()
    na = PEEL.count("a")
    ra = 3 * D // na
    ia = 0
    for ch in PEEL:
        if ch in widx:
            i = widx[ch]
            cp_w(i).wait()
            wt[i * D:(i + 1) * D, KA:D] = wqkv_v[KA:D, i * D:(i + 1) * D].T
        elif ch == "x":
            cp_xb.wait()
        elif ch == "a":
            rows = slice(ia * ra, (ia + 1) * ra)
            wa = wqkv_v[0:KA, rows].T
            wt[rows, 0:KA] = wa
            part0[rows, :] = lax.dot_general(wa, x_v[0:TB, 0:KA], NT, preferred_element_type=F32)
            ia += 1
        else:
            grp[ch](cnt[ch], 0, 0)
            cnt[ch] += 1
    memo["peel"] = False

    def p1(tb, carry):
        t0 = pl.multiple_of(tb * TB, TB)
        cp_x(tb).wait()
        for ch in "QKV":
            for g in range(4):
                grp[ch](g, tb, t0)
        return carry

    lax.fori_loop(1, NB, p1, 0)

    for cp in late:
        cp.wait()

    qinf = jnp.max(sq[...], axis=1, keepdims=True) * (SCALE2 / DEQ)
    bad = jnp.where(jnp.max(vmx[...], axis=1, keepdims=True) <= 2.0 ** 50, 0.0, 1.0)
    for tb in range(NB):
        bad = bad + jnp.where(qinf * kst[0, tb] <= 60.0, 0.0, 1.0)
        bad = bad + jnp.where(qinf + kst[0, tb] <= 1e15, 0.0, 1.0)
        bad = bad + jnp.where(sk[tb] * (DH * TB) <= 10.0 * kst[1, tb] + 1e-25, 0.0, 1.0)
    fast = jnp.sum(bad) == 0.0

    def reim(val):
        n = val.shape[1]
        val = val.reshape(16, 16, n)
        return val[:, 0:8], val[:, 8:16]

    sh = shift_v[...].astype(F32)
    hprev = [None] * LT

    def hdft(cg, lt):
        ls = slice(lt * 128, (lt + 1) * 128)
        hb = jnp.concatenate([ssm_v[ls, (cg * 4 + i) * C:(cg * 4 + i + 1) * C] for i in range(4)], axis=0)
        hr, hi = reim(lax.dot_general(dft_v[0:256, :], hb, NT, preferred_element_type=F32))
        for i in range(4):
            cr, ci = hr[:, :, i * 128:(i + 1) * 128], hi[:, :, i * 128:(i + 1) * 128]
            if hprev[lt] is None:
                hs[:, cg * 4 + i, :, ls] = cr
                hs[:, NC + cg * 4 + i, :, ls] = ci
            else:
                pr, pi = hprev[lt]
                hs[:, cg * 4 + i, :, ls] = jnp.concatenate([cr[0:8] - pi[0:8], cr[8:] + pi[8:]], axis=0)
                hs[:, NC + cg * 4 + i, :, ls] = jnp.concatenate([ci[0:8] + pr[0:8], ci[8:] - pr[8:]], axis=0)
            hprev[lt] = (cr, ci)

    def udft(c):
        r0 = c * C
        win = k_v[r0:r0 + C + 16, :].astype(F32)
        ks = (win[16:] * sh[0:1] + win[15:C + 15] * sh[1:2]
              + win[14:C + 14] * sh[2:3] + win[13:C + 13] * sh[3:4])
        kv = (ks * v_v[r0:r0 + C, :].astype(F32)).astype(BF16)
        kvb[r0:r0 + C, :] = kv
        ur, ui = reim(jnp.dot(dft_v[0:256, :], kv, preferred_element_type=F32))
        us[:, c] = ur
        us[:, NC + c] = ui

    hjobs = [(cg, lt) for cg in range(NC // 4) for lt in range(LT)]
    for c in range(NC):
        while len(hjobs) * NC > (NC - 1 - c) * LT * NC // 4 and hjobs:
            hdft(*hjobs.pop(0))
        udft(c)

    def mac_tasks(ft, lts):
        tasks = []

        def lanes(lt):
            return slice(lt * 128, (lt + 1) * 128) if isinstance(lt, int) else pl.ds(pl.multiple_of(lt * 128, 128), 128)

        for li, lt in enumerate(lts):
            for ab in range(NC // MB):
                st = {"r": [None] * MB, "i": [None] * MB, "id": (len(tasks), li, ab)}
                for cb in range(ab + 1):
                    for m in range(2):
                        for i in range(MB):
                            js = [j for j in range(MB) if (ab - cb) * MB + i - j >= 0]

                            def task(cache, z, lt=lt, ab=ab, m=m, cb=cb, i=i, js=js, st=st):
                                yr, yi = st["r"], st["i"]

                                def ld(ref, name, slot, pin):
                                    key = (st["id"], name, slot)
                                    if key not in cache:
                                        val = ref[ft, slot, :, lanes(lt)]
                                        cache[key] = val + z if (pin and z is not None) else val
                                    return cache[key]

                                for j in js:
                                    hv = ld(hs, "h", m * NC + (ab - cb) * MB + i - j, True)
                                    ta = ld(us, "u", cb * MB + j, False) * hv
                                    tb_ = ld(us, "u", NC + cb * MB + j, False) * hv
                                    if m == 0:
                                        yr[i] = ta if yr[i] is None else yr[i] + ta
                                        yi[i] = tb_ if yi[i] is None else yi[i] + tb_
                                    else:
                                        yr[i] = yr[i] - tb_
                                        yi[i] = yi[i] + ta
                                if cb == ab and m == 1:
                                    ys[ft, ab * MB + i, :, lanes(lt)] = yr[i]
                                    ys[ft, NC + ab * MB + i, :, lanes(lt)] = yi[i]

                            tasks.append((4 * len(js), task))
        return tasks

    def finish(p, hh, acc, cols):
        if hh == 0:
            ot[p, 0:24, cols] = acc * _recip(acc[20:21])
        else:
            b = acc * _recip(acc[0:1])
            ot[p, 20:24, cols] = b[4:8]
            ot[p, 24:40, cols] = b[8:24]

    def pv_tile(h, t, pt, acc):
        o = lax.dot_general(vt[h, :, t * 128:(t + 1) * 128], pt, NN, preferred_element_type=F32)
        return o if acc is None else o + acc

    def drain(p):
        acc = acar[...]
        for i in range(2):
            acc = pv_tile(2 * p + 1, NKT - 2 + i, pcar[i], acc)
        finish(p, 1, acc, slice(JL * TQ, (JL + 1) * TQ))

    def p2(pb, carry):
        steps = [(pi, j, hh, t0) for pi in range(PU) for j in range(S // TQ) for hh in range(2)
                 for t0 in range(0, NKT, 2)]
        tasks = [(c, t, pi) for pi in range(PU) for c, t in mac_tasks(pb * PU + pi, range(LT))]
        accs, pend = {}, []

        def qk(pi, j, hh, t0):
            p = pb * PU + pi
            h = 2 * p + hh
            w = sq[pl.ds(h, 1), j * TQ:(j + 1) * TQ] * jnp.concatenate(
                [sk[t0 * 128 // TB, pl.ds(h, 1), :]] * (TQ // 128), axis=1)
            qh = [q8[h, :, j * TQ:(j + 1) * TQ], jnp.zeros((64, TQ), I8)]
            s = jnp.dot(k8[p, t0 * 128:(t0 + 2) * 128, :], jnp.concatenate(qh if hh == 0 else qh[::-1], axis=0),
                        preferred_element_type=I32)
            for t in range(2):
                e = jnp.exp2(s[t * 128:(t + 1) * 128].astype(F32) * w)
                pt = jnp.concatenate([e[16 * i:16 * (i + 1)] for i in reversed(range(8))], axis=0).astype(BF16)
                pend.append((pi, j, hh, t0 + t, pt))
            return e[120:128, TQ - 128:TQ]

        def pv(pi, j, hh, t, pt):
            p = pb * PU + pi
            acc = pv_tile(2 * p + hh, t, pt, accs.get((j, hh)))
            accs[(j, hh)] = acc
            if t == NKT - 1:
                finish(p, hh, accs.pop((j, hh)), slice(j * TQ, (j + 1) * TQ))
            return acc

        n = len(steps)
        wts = [W_FIN if steps[i][3] == 0 else 1.0 for i in range(n - 1)]
        total = float(sum(t[0] for t in tasks))
        ti, done, cum = 0, 0.0, 0.0
        for i in range(n):
            last_e = qk(*steps[i])
            if i == 0:
                drain(jnp.maximum(pb * PU - 1, 0))
            outs = []
            while len(pend) > 2:
                outs.append(pv(*pend.pop(0)))
            if i < n - 1:
                tok2 = last_e
                if outs:
                    m = jnp.maximum(jnp.maximum(outs[0][0:8], outs[0][8:16]), outs[0][16:24])
                    tok2 = jnp.abs(lanefold(m, jnp.maximum))
                toks = [(last_e, SPLIT), (tok2, 1.0 - SPLIT)]
                for ui, (tk, fr) in enumerate(toks):
                    z = jnp.minimum(tk, 0.0)
                    cum += wts[i] / sum(wts) * total * fr
                    caches = {}
                    while ti < len(tasks) and (done + tasks[ti][0] / 2 <= cum or (i == n - 2 and ui == len(toks) - 1)):
                        tasks[ti][1](caches.setdefault(tasks[ti][2], {}), z)
                        done += tasks[ti][0]
                        ti += 1
        for i in range(2):
            pcar[i] = pend[i][4]
        acar[...] = accs.pop((JL, 1))
        return carry

    pcar[...] = jnp.zeros((2, 128, TQ), BF16)
    acar[...] = jnp.ones((24, TQ), F32)

    def attn_fast():
        lax.fori_loop(0, NP // PU, p2, 0)
        drain(NP - 1)

    def attn_general():
        def fb1(i, carry):
            r0 = pl.multiple_of((i // NB) * 160, 32)
            t0 = pl.multiple_of((i % NB) * TB, TB)
            qkt[pl.ds(r0, 160), pl.ds(t0, TB)] = lax.dot_general(
                wt[pl.ds(r0, 160), :], x_v[pl.ds(t0, TB), :], NT, preferred_element_type=F32)
            return carry

        lax.fori_loop(0, 8 * NB, fb1, 0)

        def fb2(p, carry):
            r0 = pl.multiple_of(40 * p, 8)

            def tr(kt, c2):
                c0 = pl.multiple_of(kt * 128, 128)
                blk = jnp.concatenate([qkt[pl.ds(D + r0, 40), pl.ds(c0, 128)], jnp.zeros((88, 128), F32)], axis=0)
                kn[pl.ds(c0, 128), :] = blk.T.astype(BF16)
                return c2

            lax.fori_loop(0, NKT, tr, 0)
            rows = lax.broadcasted_iota(I32, (40, TQ), 0)
            for hh in range(2):
                def qtile(j, c2, hh=hh):
                    c0 = pl.multiple_of(j * TQ, TQ)
                    qm = jnp.where((rows >= DH * hh) & (rows < DH * hh + DH),
                                   qkt[pl.ds(r0, 40), pl.ds(c0, TQ)], 0.0)
                    qm = jnp.concatenate([qm, jnp.zeros((88, TQ), F32)], axis=0).astype(BF16)

                    def kchunk(c, st):
                        m, acc = st
                        k0 = pl.multiple_of(c * 128, 128)
                        s = jnp.dot(kn[pl.ds(k0, 128), :], qm, preferred_element_type=F32) * SCALE2
                        mn = jnp.maximum(m, jnp.max(s, axis=0, keepdims=True))
                        e = jnp.exp2(s - mn).astype(BF16)
                        o = lax.dot_general(vt[2 * p + hh, :, pl.ds(k0, 128)], e, NN, preferred_element_type=F32)
                        return mn, o + acc * jnp.exp2(m - mn)

                    m0 = jnp.full((1, TQ), -jnp.inf, F32)
                    _, acc = lax.fori_loop(0, NKT, kchunk, (m0, jnp.zeros((24, TQ), F32)))
                    finish(p, hh, acc, pl.ds(c0, TQ))
                    return c2

                lax.fori_loop(0, S // TQ, qtile, 0)

            def mac(lt, c2):
                cache = {}
                for _, task in mac_tasks(p, [lt]):
                    task(cache, None)
                return c2

            lax.fori_loop(0, LT, mac, 0)
            return carry

        lax.fori_loop(0, NP, fb2, 0)

    lax.cond(fast, attn_fast, attn_general)

    gw = gw_v[...].astype(F32).reshape(1, D)
    dv = dvec_v[...].astype(F32).reshape(1, D)

    def p4(it, carry):
        off = 0
        for sb, oc in enumerate(OBS):
            c0 = it * sum(OBS) + off
            off += oc
            ob = oc * C
            t0 = pl.multiple_of(c0 * C, C)
            s0 = (sb % 2) * max(OBS) * LT
            yr = jnp.concatenate([ys[:, c0 + i].reshape(128, D) for i in range(oc)], axis=1)
            yi = jnp.concatenate([ys[:, NC + c0 + i].reshape(128, D) for i in range(oc)], axis=1)
            ar, br, ai, bi = yr[0:64], yr[64:128], yi[0:64], yi[64:128]
            ye = jnp.dot(dft_v[256:320, :], jnp.concatenate([ar + br, ai - bi], axis=0).astype(BF16),
                         preferred_element_type=F32)
            yo = jnp.dot(dft_v[320:384, :], jnp.concatenate([ar - br, ai + bi], axis=0).astype(BF16),
                         preferred_element_type=F32)
            for i in range(oc * LT):
                ysc[s0 + i, pl.ds(0, 64, stride=2), :] = ye[:, i * 128:(i + 1) * 128]
                ysc[s0 + i, pl.ds(1, 64, stride=2), :] = yo[:, i * 128:(i + 1) * 128]
            y = jnp.concatenate(
                [jnp.concatenate([ysc[s0 + i * LT + lt] for lt in range(LT)], axis=1) for i in range(oc)], axis=0)
            o = ot[:, :, pl.ds(t0, ob)].reshape(D, ob).astype(BF16).T
            a = jnp.dot(o, wo_v[...], preferred_element_type=F32)
            xf = x_v[pl.ds(t0, ob), :].astype(F32)
            g = jax.nn.sigmoid(jnp.sum(xf * gw, axis=-1, keepdims=True))
            b = xf * (y + kvb[pl.ds(t0, ob), :].astype(F32) * dv)
            out_v[pl.ds(t0, ob), :] = (b + g * (a - b)).astype(BF16)
            cp_out(c0, oc).start()
        return carry

    lax.fori_loop(0, NC // sum(OBS), p4, 0)
    cp_out(0, NC).wait()


@jax.jit
def pallas_gated_mix__mha_block__ssm_conv_h3__prompt_kernel(A_x, A_wqkv, A_wo, B_q, B_k, B_v, B_shift_k, B_ssm_k, B_ssm_D, gate_w):
    del B_q
    hbm = pl.BlockSpec(memory_space=pl.ANY)
    return pl.pallas_call(
        _kernel,
        out_shape=jax.ShapeDtypeStruct((1, S, D), BF16),
        in_specs=[hbm] * 10,
        out_specs=hbm,
        scratch_shapes=[
            pltpu.VMEM((S, D), BF16),
            pltpu.VMEM((D, 3 * D), BF16),
            pltpu.VMEM((D, D), BF16),
            pltpu.VMEM((S + 16, D), BF16),
            pltpu.VMEM((S, D), BF16),
            pltpu.VMEM((D, S), BF16),
            pltpu.VMEM((S, D), BF16),
            pltpu.VMEM((4, D), BF16),
            pltpu.VMEM((D,), BF16),
            pltpu.VMEM((D,), BF16),
            pltpu.VMEM((384, 128), BF16),
            pltpu.VMEM((3 * D, D), BF16),
            pltpu.VMEM((H, 64, S), I8),
            pltpu.VMEM((NP, S, 128), I8),
            pltpu.VMEM((H, 24, S), F32),
            pltpu.VMEM((H, S), F32),
            pltpu.VMEM((NB, H, 128), F32),
            pltpu.VMEM((2, NB, H, 128), F32),
            pltpu.VMEM((32, S), F32),
            pltpu.VMEM((NP, 40, S), F32),
            pltpu.VMEM((S, D), BF16),
            pltpu.VMEM((16, 2 * NC, 8, D), F32),
            pltpu.VMEM((16, 2 * NC, 8, D), F32),
            pltpu.VMEM((16, 2 * NC, 8, D), F32),
            pltpu.VMEM((2 * max(OBS) * LT, 128, 128), F32),
            pltpu.VMEM((2 * D, S), F32),
            pltpu.VMEM((S, 128), BF16),
            pltpu.VMEM((2, 128, TQ), BF16),
            pltpu.VMEM((24, TQ), F32),
            pltpu.VMEM((3 * D, TB), F32),
            pltpu.SemaphoreType.DMA((10,)),
        ],
        compiler_params=pltpu.CompilerParams(vmem_limit_bytes=120 * 1024 * 1024),
        name="gmix",
    )(A_x, A_wqkv, A_wo, B_k, B_v, B_ssm_k, B_shift_k.T, B_ssm_D, gate_w, jnp.asarray(_dft_tables(), BF16))
```

```python
import numpy as np
import jax
import jax.numpy as jnp
from jax import lax
import jax.experimental.pallas as pl
import jax.experimental.pallas.tpu as pltpu

S, D, H, DH = 2048, 640, 32, 20
NP = H // 2
TB = 512
NB = S // TB
C = 128
NC = S // C
LT = D // 128
NKT = S // 128
TQ = 512
JL = S // TQ - 1
MB = 4
PU = 2
OBS = (4, 2, 1, 1)
G, FIRST, STEP, LAST, LAG = 64, 5, 6, 4, 3
W_FIN, W_STR = 0.4, 0.5
PEEL = "aaaqaaxQQQvQVkVKKKKVV"
KA = 128

F32, BF16, I32, I16, I8 = jnp.float32, jnp.bfloat16, jnp.int32, jnp.int16, jnp.int8
NT = (((1,), (1,)), ((), ()))
NN = (((1,), (0,)), ((), ()))
QMAX = 2038.0
MAGIC = 12582912.0
MAGIC_BITS = 0x4B400000
SCALE2 = (DH ** -0.5) * 1.4426950408889634
DEQ = 256.0 / (QMAX * QMAX) * SCALE2


def _dft_tables():
    r = np.arange(64, dtype=np.float64)
    f = np.concatenate([2 * r, 127 - 2 * r])
    n = np.arange(128, dtype=np.float64)
    ang = 2.0 * np.pi * (f[:, None] + 0.5) * n[None, :] / 256.0
    fwd = np.concatenate([np.cos(ang), -np.sin(ang)], axis=0)
    inv = np.concatenate([np.cos(ang[:64]).T, -np.sin(ang[:64]).T], axis=1) / 128.0
    inv = np.concatenate([inv[0::2], inv[1::2]], axis=0)
    fwd = fwd.reshape(2, 16, 8, 128).transpose(1, 0, 2, 3).reshape(256, 128)
    return np.concatenate([fwd, inv], axis=0).astype(np.float32)


def _limbs(r, inv):
    t = lax.bitcast_convert_type(r * inv + MAGIC, I32) - (MAGIC_BITS - 8)
    return t >> 4, (t & 15) - 8, (t + 120) >> 8


def _recip(m):
    r = pl.reciprocal(m, approx=True)
    return r * (2.0 - m * r)


def _qscale(m):
    r = pl.reciprocal(m, approx=True)
    return (r * QMAX) * (2.0 - m * r)


def _kernel(x_hbm, wqkv_hbm, wo_hbm, k_hbm, v_hbm, ssm_hbm, shift_hbm, dvec_hbm, gw_hbm, dft_hbm, out_hbm,
            x_v, wqkv_v, wo_v, k_v, v_v, ssm_v, out_v, shift_v, dvec_v, gw_v, dft_v,
            wt, q8, k8, vt, sq, sk, kst, vmx, ot, kvb, us, hs, ys, ysc, qkt, kn, pcar, acar, part0, sems):
    def cp_w(i):
        return pltpu.make_async_copy(wqkv_hbm.at[KA:D, i * D:(i + 1) * D], wqkv_v.at[KA:D, i * D:(i + 1) * D],
                                     sems.at[i])

    cp_wa = pltpu.make_async_copy(wqkv_hbm.at[0:KA, :], wqkv_v.at[0:KA, :], sems.at[9])
    cp_xa = pltpu.make_async_copy(x_hbm.at[0, 0:TB, 0:KA], x_v.at[0:TB, 0:KA], sems.at[9])
    cp_xb = pltpu.make_async_copy(x_hbm.at[0, 0:TB, KA:D], x_v.at[0:TB, KA:D], sems.at[3])

    def cp_x(i):
        return pltpu.make_async_copy(x_hbm.at[0, pl.ds(i * TB, TB), :], x_v.at[pl.ds(i * TB, TB), :],
                                     sems.at[3 + i])

    late = [
        pltpu.make_async_copy(ssm_hbm, ssm_v, sems.at[7]),
        pltpu.make_async_copy(k_hbm.at[0], k_v.at[pl.ds(16, S), :], sems.at[7]),
        pltpu.make_async_copy(v_hbm.at[0], v_v, sems.at[7]),
        pltpu.make_async_copy(wo_hbm, wo_v, sems.at[7]),
        pltpu.make_async_copy(shift_hbm, shift_v, sems.at[7]),
        pltpu.make_async_copy(dvec_hbm, dvec_v, sems.at[7]),
        pltpu.make_async_copy(gw_hbm, gw_v, sems.at[7]),
        pltpu.make_async_copy(dft_hbm, dft_v, sems.at[7]),
    ]

    def cp_out(c0, oc):
        r0 = pl.multiple_of(c0 * C, C)
        return pltpu.make_async_copy(out_v.at[pl.ds(r0, oc * C), :], out_hbm.at[0, pl.ds(r0, oc * C), :], sems.at[8])

    widx = {"q": 0, "k": 1, "v": 2}
    cp_wa.start()
    cp_xa.start()
    for ch in PEEL:
        if ch in widx:
            cp_w(widx[ch]).start()
        elif ch == "x":
            cp_xb.start()
    for i in range(1, NB):
        cp_x(i).start()
    for cp in late:
        cp.start()

    k_v[0:16, :] = jnp.zeros((16, D), BF16)

    low4 = lax.broadcasted_iota(I32, (8, TB), 0) < 4

    def headred(a, op, red):
        mid = a[16:24]
        ma = op(op(a[0:8], a[8:16]), jnp.where(low4, mid, 0.0))
        mb = op(op(a[24:32], a[32:40]), jnp.where(low4, 0.0, mid))
        return red(ma, axis=0, keepdims=True), red(mb, axis=0, keepdims=True)

    def pairscale(ia, ib):
        a8 = jnp.broadcast_to(ia, (8, TB))
        b8 = jnp.broadcast_to(ib, (8, TB))
        return jnp.concatenate([a8, a8, jnp.where(low4, a8, b8), b8, b8], axis=0)

    def slots(l1, l2, l3, mask):
        r2 = pltpu.roll(l2[16:24], 4, 0)
        m3 = l3[16:24]
        a = [l1[0:16], l2[0:16], l3[0:16], jnp.where(low4, l1[16:24], r2), jnp.where(low4, m3, 0) if mask else m3]
        b = [l1[24:40], l2[24:40], l3[24:40], jnp.where(low4, r2, l1[16:24]), jnp.where(low4, 0, m3) if mask else m3]
        return a, b

    def lanefold(a, op):
        return op(op(a[:, 0:128], a[:, 128:256]), op(a[:, 256:384], a[:, 384:512]))

    memo = {}

    def proj(part, g, t0):
        r0 = part * D + 160 * g
        if memo["peel"]:
            return lax.dot_general(wt[r0:r0 + 160, KA:D], x_v[0:TB, KA:D], NT,
                                   preferred_element_type=F32) + part0[r0:r0 + 160, :]
        if g % 2 == 0:
            memo["wide"] = lax.dot_general(wt[r0:r0 + 320, :], x_v[pl.ds(t0, TB), :], NT,
                                           preferred_element_type=F32)
        return memo["wide"][160 * (g % 2):160 * (g % 2 + 1)]

    def kgrp(g, tb, t0):
        rk = proj(1, g, t0)
        for j in range(4):
            p = 4 * g + j
            r = rk[40 * j:40 * (j + 1)]
            ab = jnp.abs(r)
            mida, midb = jnp.where(low4, ab[16:24], 0.0), jnp.where(low4, 0.0, ab[16:24])
            ms = []
            for hh, (u0, u1, u2) in enumerate(((ab[0:8], ab[8:16], mida), (ab[24:32], ab[32:40], midb))):
                l1 = u0 + u1 + u2
                l1m = jnp.sum(jnp.max(lanefold(l1, jnp.maximum), axis=1, keepdims=True), axis=0, keepdims=True)
                l1s = jnp.sum(jnp.sum(lanefold(l1, jnp.add), axis=1, keepdims=True), axis=0, keepdims=True)
                kst[0, tb, 2 * p + hh:2 * p + hh + 1, :] = jnp.broadcast_to(l1m, (1, 128))
                kst[1, tb, 2 * p + hh:2 * p + hh + 1, :] = jnp.broadcast_to(l1s, (1, 128))
                m = lanefold(jnp.maximum(jnp.maximum(u0, u1), u2), jnp.maximum)
                m = jnp.max(jnp.max(m, axis=0, keepdims=True), axis=1, keepdims=True)
                ms.append(jnp.maximum(m, 1e-30))
            ma, mb = ms
            hi, lo, top = _limbs(r, pairscale(_qscale(ma), _qscale(mb)))
            sk[tb, 2 * p:2 * p + 1, :] = jnp.broadcast_to(ma, (1, 128))
            sk[tb, 2 * p + 1:2 * p + 2, :] = jnp.broadcast_to(mb, (1, 128))
            ka, kb = slots(hi, lo, top, False)
            kk = jnp.concatenate(ka + kb, axis=0).astype(I16).T
            kk = jnp.concatenate([kk[kt * 128 + 16 * i:kt * 128 + 16 * (i + 1)]
                                  for kt in range(TB // 128) for i in reversed(range(8))], axis=0)
            k8[p, pl.ds(t0, TB), :] = kk.astype(I8)

    def qgrp(g, tb, t0):
        rq = proj(0, g, t0)
        for j in range(4):
            p = 4 * g + j
            r = rq[40 * j:40 * (j + 1)]
            ma, mb = headred(jnp.abs(r), jnp.maximum, jnp.max)
            ma = jnp.maximum(ma, 1e-30)
            mb = jnp.maximum(mb, 1e-30)
            hi, lo, top = _limbs(r, pairscale(_qscale(ma), _qscale(mb)))
            sq[2 * p:2 * p + 1, pl.ds(t0, TB)] = ma * DEQ
            sq[2 * p + 1:2 * p + 2, pl.ds(t0, TB)] = mb * DEQ
            pa, pb = slots(hi, top, lo, True)
            q8[2 * p, :, pl.ds(t0, TB)] = jnp.concatenate(pa, axis=0).astype(I8)
            q8[2 * p + 1, :, pl.ds(t0, TB)] = jnp.concatenate(pb, axis=0).astype(I8)

    def vgrp(g, tb, t0):
        rv = proj(2, g, t0)
        vmx[8 * g:8 * (g + 1), pl.ds(t0, TB)] = jnp.max(jnp.abs(rv).reshape(20, 8, TB), axis=0)
        for j in range(4):
            p = 4 * g + j
            r = rv[40 * j:40 * (j + 1)]
            mid = r[16:24]
            vt[2 * p, :, pl.ds(t0, TB)] = jnp.concatenate([r[0:16], jnp.where(low4, mid, 1.0)], axis=0)
            vt[2 * p + 1, :, pl.ds(t0, TB)] = jnp.concatenate([jnp.where(low4, 1.0, mid), r[24:40]], axis=0)

    grp = {"K": kgrp, "Q": qgrp, "V": vgrp}
    cnt = {"K": 0, "Q": 0, "V": 0}
    memo["peel"] = True
    cp_wa.wait()
    cp_xa.wait()
    na = PEEL.count("a")
    ra = 3 * D // na
    ia = 0
    for ch in PEEL:
        if ch in widx:
            i = widx[ch]
            cp_w(i).wait()
            wt[i * D:(i + 1) * D, KA:D] = wqkv_v[KA:D, i * D:(i + 1) * D].T
        elif ch == "x":
            cp_xb.wait()
        elif ch == "a":
            rows = slice(ia * ra, (ia + 1) * ra)
            wa = wqkv_v[0:KA, rows].T
            wt[rows, 0:KA] = wa
            part0[rows, :] = lax.dot_general(wa, x_v[0:TB, 0:KA], NT, preferred_element_type=F32)
            ia += 1
        else:
            grp[ch](cnt[ch], 0, 0)
            cnt[ch] += 1
    memo["peel"] = False

    def p1(tb, carry):
        t0 = pl.multiple_of(tb * TB, TB)
        cp_x(tb).wait()
        for ch in "QKV":
            for g in range(4):
                grp[ch](g, tb, t0)
        return carry

    lax.fori_loop(1, NB, p1, 0)

    for cp in late:
        cp.wait()

    qinf = jnp.max(sq[...], axis=1, keepdims=True) * (SCALE2 / DEQ)
    bad = jnp.where(jnp.max(vmx[...], axis=1, keepdims=True) <= 2.0 ** 50, 0.0, 1.0)
    for tb in range(NB):
        bad = bad + jnp.where(qinf * kst[0, tb] <= 60.0, 0.0, 1.0)
        bad = bad + jnp.where(qinf + kst[0, tb] <= 1e15, 0.0, 1.0)
        bad = bad + jnp.where(sk[tb] * (DH * TB) <= 10.0 * kst[1, tb] + 1e-25, 0.0, 1.0)
    fast = jnp.sum(bad) == 0.0

    def reim(val):
        n = val.shape[1]
        val = val.reshape(16, 16, n)
        return val[:, 0:8], val[:, 8:16]

    sh = shift_v[...].astype(F32)
    hprev = [None] * LT

    def hdft(cg, lt):
        ls = slice(lt * 128, (lt + 1) * 128)
        hb = jnp.concatenate([ssm_v[ls, (cg * 4 + i) * C:(cg * 4 + i + 1) * C] for i in range(4)], axis=0)
        hr, hi = reim(lax.dot_general(dft_v[0:256, :], hb, NT, preferred_element_type=F32))
        for i in range(4):
            cr, ci = hr[:, :, i * 128:(i + 1) * 128], hi[:, :, i * 128:(i + 1) * 128]
            if hprev[lt] is None:
                hs[:, cg * 4 + i, :, ls] = cr
                hs[:, NC + cg * 4 + i, :, ls] = ci
            else:
                pr, pi = hprev[lt]
                hs[:, cg * 4 + i, :, ls] = jnp.concatenate([cr[0:8] - pi[0:8], cr[8:] + pi[8:]], axis=0)
                hs[:, NC + cg * 4 + i, :, ls] = jnp.concatenate([ci[0:8] + pr[0:8], ci[8:] - pr[8:]], axis=0)
            hprev[lt] = (cr, ci)

    def udft(c):
        r0 = c * C
        win = k_v[r0:r0 + C + 16, :].astype(F32)
        ks = (win[16:] * sh[0:1] + win[15:C + 15] * sh[1:2]
              + win[14:C + 14] * sh[2:3] + win[13:C + 13] * sh[3:4])
        kv = (ks * v_v[r0:r0 + C, :].astype(F32)).astype(BF16)
        kvb[r0:r0 + C, :] = kv
        ur, ui = reim(jnp.dot(dft_v[0:256, :], kv, preferred_element_type=F32))
        us[:, c] = ur
        us[:, NC + c] = ui

    hjobs = [(cg, lt) for cg in range(NC // 4) for lt in range(LT)]
    for c in range(NC):
        while len(hjobs) * NC > (NC - 1 - c) * LT * NC // 4 and hjobs:
            hdft(*hjobs.pop(0))
        udft(c)

    def mac_tasks(ft, lts):
        tasks = []

        def lanes(lt):
            return slice(lt * 128, (lt + 1) * 128) if isinstance(lt, int) else pl.ds(pl.multiple_of(lt * 128, 128), 128)

        for li, lt in enumerate(lts):
            for ab in range(NC // MB):
                st = {"r": [None] * MB, "i": [None] * MB, "id": (len(tasks), li, ab)}
                for cb in range(ab + 1):
                    for m in range(2):
                        for i in range(MB):
                            js = [j for j in range(MB) if (ab - cb) * MB + i - j >= 0]

                            def task(cache, z, lt=lt, ab=ab, m=m, cb=cb, i=i, js=js, st=st):
                                yr, yi = st["r"], st["i"]

                                def ld(ref, name, slot, pin):
                                    key = (st["id"], name, slot)
                                    if key not in cache:
                                        val = ref[ft, slot, :, lanes(lt)]
                                        cache[key] = val + z if (pin and z is not None) else val
                                    return cache[key]

                                for j in js:
                                    hv = ld(hs, "h", m * NC + (ab - cb) * MB + i - j, True)
                                    ta = ld(us, "u", cb * MB + j, False) * hv
                                    tb_ = ld(us, "u", NC + cb * MB + j, False) * hv
                                    if m == 0:
                                        yr[i] = ta if yr[i] is None else yr[i] + ta
                                        yi[i] = tb_ if yi[i] is None else yi[i] + tb_
                                    else:
                                        yr[i] = yr[i] - tb_
                                        yi[i] = yi[i] + ta
                                if cb == ab and m == 1:
                                    ys[ft, ab * MB + i, :, lanes(lt)] = yr[i]
                                    ys[ft, NC + ab * MB + i, :, lanes(lt)] = yi[i]

                            tasks.append((4 * len(js), task))
        return tasks

    def finish(p, hh, acc, cols):
        if hh == 0:
            ot[p, 0:24, cols] = acc * _recip(acc[20:21])
        else:
            b = acc * _recip(acc[0:1])
            ot[p, 20:24, cols] = b[4:8]
            ot[p, 24:40, cols] = b[8:24]

    def pv_tile(h, t, pt, acc):
        o = lax.dot_general(vt[h, :, t * 128:(t + 1) * 128], pt, NN, preferred_element_type=F32)
        return o if acc is None else o + acc

    def drain(p):
        acc = acar[...]
        for i in range(2):
            acc = pv_tile(2 * p + 1, NKT - 2 + i, pcar[i], acc)
        finish(p, 1, acc, slice(JL * TQ, (JL + 1) * TQ))

    def p2(pb, carry):
        heads = [(pi, j, hh) for pi in range(PU) for j in range(S // TQ) for hh in range(2)]
        hu = S // G
        sizes = [FIRST]
        while len(heads) * hu - sum(sizes) - LAST > STEP:
            sizes.append(STEP)
        sizes += [len(heads) * hu - sum(sizes) - LAST, LAST]
        steps, g0 = [], 0
        for left in sizes:
            segs = []
            while left:
                u, h0 = divmod(g0, hu)
                nh = min(left, hu - h0)
                segs.append(heads[u] + (h0, nh))
                g0 += nh
                left -= nh
            steps.append(segs)
        tasks = [(c, t, pi) for pi in range(PU) for c, t in mac_tasks(pb * PU + pi, range(LT))]
        accs, pend, part, pos = {}, [], [], [0]

        def qk(pi, j, hh, h0, nh):
            p = pb * PU + pi
            h = 2 * p + hh
            wq = sq[pl.ds(h, 1), j * TQ:(j + 1) * TQ]
            qh = [q8[h, :, j * TQ:(j + 1) * TQ], jnp.zeros((64, TQ), I8)]
            s = jnp.dot(k8[p, h0 * G:(h0 + nh) * G, :], jnp.concatenate(qh if hh == 0 else qh[::-1], axis=0),
                        preferred_element_type=I32)
            ws = {}
            for t in range(nh):
                kb = (h0 + t) * G // TB
                if kb not in ws:
                    ws[kb] = wq * jnp.concatenate([sk[kb, pl.ds(h, 1), :]] * (TQ // 128), axis=1)
                e = jnp.exp2(s[t * G:(t + 1) * G].astype(F32) * ws[kb])
                part.extend(e[16 * i:16 * (i + 1)] for i in range(G // 16))
                pos[0] += 1
                if len(part) == 8:
                    pt = jnp.concatenate(part[::-1], axis=0).astype(BF16)
                    pend.append((pos[0], pi, j, hh, (h0 + t) * G // 128, pt))
                    part.clear()

        def pv(_, pi, j, hh, t, pt):
            p = pb * PU + pi
            acc = pv_tile(2 * p + hh, t, pt, accs.get((j, hh)))
            accs[(j, hh)] = acc
            if t == NKT - 1:
                finish(p, hh, accs.pop((j, hh)), slice(j * TQ, (j + 1) * TQ))
            return acc

        n = len(steps)
        wts, issued, tiles = [], 0, -2
        for i in range(n - 1):
            issued += sizes[i]
            nd = (issued - LAG) * G // 128
            wts.append(nd - tiles - (W_FIN if nd // NKT != tiles // NKT else 0.0)
                       - (W_STR if len(steps[i + 1]) > 1 else 0.0))
            tiles = nd
        total = float(sum(t[0] for t in tasks))
        ti, done, cum = 0, 0.0, 0.0
        for i in range(n):
            for seg in steps[i]:
                qk(*seg)
            if i == 0:
                drain(jnp.maximum(pb * PU - 1, 0))
            outs = []
            while pend and (pend[0][0] <= pos[0] - LAG if i < n - 1 else len(pend) > 2):
                outs.append(pv(*pend.pop(0)))
            if i < n - 1:
                for ui in range(2):
                    z = jnp.minimum(jnp.abs(outs[min(ui, len(outs) - 1)][0:8, 0:128]), 0.0)
                    cum += wts[i] / sum(wts) * total / 2
                    caches = {}
                    while ti < len(tasks) and (done + tasks[ti][0] / 2 <= cum or (i == n - 2 and ui == 1)):
                        tasks[ti][1](caches.setdefault(tasks[ti][2], {}), z)
                        done += tasks[ti][0]
                        ti += 1
        for i in range(2):
            pcar[i] = pend[i][5]
        acar[...] = accs.pop((JL, 1))
        return carry

    pcar[...] = jnp.zeros((2, 128, TQ), BF16)
    acar[...] = jnp.ones((24, TQ), F32)

    def attn_fast():
        lax.fori_loop(0, NP // PU, p2, 0)
        drain(NP - 1)

    def attn_general():
        def fb1(i, carry):
            r0 = pl.multiple_of((i // NB) * 160, 32)
            t0 = pl.multiple_of((i % NB) * TB, TB)
            qkt[pl.ds(r0, 160), pl.ds(t0, TB)] = lax.dot_general(
                wt[pl.ds(r0, 160), :], x_v[pl.ds(t0, TB), :], NT, preferred_element_type=F32)
            return carry

        lax.fori_loop(0, 8 * NB, fb1, 0)

        def fb2(p, carry):
            r0 = pl.multiple_of(40 * p, 8)

            def tr(kt, c2):
                c0 = pl.multiple_of(kt * 128, 128)
                blk = jnp.concatenate([qkt[pl.ds(D + r0, 40), pl.ds(c0, 128)], jnp.zeros((88, 128), F32)], axis=0)
                kn[pl.ds(c0, 128), :] = blk.T.astype(BF16)
                return c2

            lax.fori_loop(0, NKT, tr, 0)
            rows = lax.broadcasted_iota(I32, (40, TQ), 0)
            for hh in range(2):
                def qtile(j, c2, hh=hh):
                    c0 = pl.multiple_of(j * TQ, TQ)
                    qm = jnp.where((rows >= DH * hh) & (rows < DH * hh + DH),
                                   qkt[pl.ds(r0, 40), pl.ds(c0, TQ)], 0.0)
                    qm = jnp.concatenate([qm, jnp.zeros((88, TQ), F32)], axis=0).astype(BF16)

                    def kchunk(c, st):
                        m, acc = st
                        k0 = pl.multiple_of(c * 128, 128)
                        s = jnp.dot(kn[pl.ds(k0, 128), :], qm, preferred_element_type=F32) * SCALE2
                        mn = jnp.maximum(m, jnp.max(s, axis=0, keepdims=True))
                        e = jnp.exp2(s - mn).astype(BF16)
                        o = lax.dot_general(vt[2 * p + hh, :, pl.ds(k0, 128)], e, NN, preferred_element_type=F32)
                        return mn, o + acc * jnp.exp2(m - mn)

                    m0 = jnp.full((1, TQ), -jnp.inf, F32)
                    _, acc = lax.fori_loop(0, NKT, kchunk, (m0, jnp.zeros((24, TQ), F32)))
                    finish(p, hh, acc, pl.ds(c0, TQ))
                    return c2

                lax.fori_loop(0, S // TQ, qtile, 0)

            def mac(lt, c2):
                cache = {}
                for _, task in mac_tasks(p, [lt]):
                    task(cache, None)
                return c2

            lax.fori_loop(0, LT, mac, 0)
            return carry

        lax.fori_loop(0, NP, fb2, 0)

    lax.cond(fast, attn_fast, attn_general)

    gw = gw_v[...].astype(F32).reshape(1, D)
    dv = dvec_v[...].astype(F32).reshape(1, D)

    def p4(it, carry):
        off = 0
        for sb, oc in enumerate(OBS):
            c0 = it * sum(OBS) + off
            off += oc
            ob = oc * C
            t0 = pl.multiple_of(c0 * C, C)
            s0 = (sb % 2) * max(OBS) * LT
            yr = jnp.concatenate([ys[:, c0 + i].reshape(128, D) for i in range(oc)], axis=1)
            yi = jnp.concatenate([ys[:, NC + c0 + i].reshape(128, D) for i in range(oc)], axis=1)
            ar, br, ai, bi = yr[0:64], yr[64:128], yi[0:64], yi[64:128]
            ye = jnp.dot(dft_v[256:320, :], jnp.concatenate([ar + br, ai - bi], axis=0).astype(BF16),
                         preferred_element_type=F32)
            yo = jnp.dot(dft_v[320:384, :], jnp.concatenate([ar - br, ai + bi], axis=0).astype(BF16),
                         preferred_element_type=F32)
            for i in range(oc * LT):
                ysc[s0 + i, pl.ds(0, 64, stride=2), :] = ye[:, i * 128:(i + 1) * 128]
                ysc[s0 + i, pl.ds(1, 64, stride=2), :] = yo[:, i * 128:(i + 1) * 128]
            y = jnp.concatenate(
                [jnp.concatenate([ysc[s0 + i * LT + lt] for lt in range(LT)], axis=1) for i in range(oc)], axis=0)
            o = ot[:, :, pl.ds(t0, ob)].reshape(D, ob).astype(BF16).T
            a = jnp.dot(o, wo_v[...], preferred_element_type=F32)
            xf = x_v[pl.ds(t0, ob), :].astype(F32)
            g = jax.nn.sigmoid(jnp.sum(xf * gw, axis=-1, keepdims=True))
            b = xf * (y + kvb[pl.ds(t0, ob), :].astype(F32) * dv)
            out_v[pl.ds(t0, ob), :] = (b + g * (a - b)).astype(BF16)
            cp_out(c0, oc).start()
        return carry

    lax.fori_loop(0, NC // sum(OBS), p4, 0)
    cp_out(0, NC).wait()


@jax.jit
def pallas_gated_mix__mha_block__ssm_conv_h3__prompt_kernel(A_x, A_wqkv, A_wo, B_q, B_k, B_v, B_shift_k, B_ssm_k, B_ssm_D, gate_w):
    del B_q
    hbm = pl.BlockSpec(memory_space=pl.ANY)
    return pl.pallas_call(
        _kernel,
        out_shape=jax.ShapeDtypeStruct((1, S, D), BF16),
        in_specs=[hbm] * 10,
        out_specs=hbm,
        scratch_shapes=[
            pltpu.VMEM((S, D), BF16),
            pltpu.VMEM((D, 3 * D), BF16),
            pltpu.VMEM((D, D), BF16),
            pltpu.VMEM((S + 16, D), BF16),
            pltpu.VMEM((S, D), BF16),
            pltpu.VMEM((D, S), BF16),
            pltpu.VMEM((S, D), BF16),
            pltpu.VMEM((4, D), BF16),
            pltpu.VMEM((D,), BF16),
            pltpu.VMEM((D,), BF16),
            pltpu.VMEM((384, 128), BF16),
            pltpu.VMEM((3 * D, D), BF16),
            pltpu.VMEM((H, 64, S), I8),
            pltpu.VMEM((NP, S, 128), I8),
            pltpu.VMEM((H, 24, S), F32),
            pltpu.VMEM((H, S), F32),
            pltpu.VMEM((NB, H, 128), F32),
            pltpu.VMEM((2, NB, H, 128), F32),
            pltpu.VMEM((32, S), F32),
            pltpu.VMEM((NP, 40, S), F32),
            pltpu.VMEM((S, D), BF16),
            pltpu.VMEM((16, 2 * NC, 8, D), F32),
            pltpu.VMEM((16, 2 * NC, 8, D), F32),
            pltpu.VMEM((16, 2 * NC, 8, D), F32),
            pltpu.VMEM((2 * max(OBS) * LT, 128, 128), F32),
            pltpu.VMEM((2 * D, S), F32),
            pltpu.VMEM((S, 128), BF16),
            pltpu.VMEM((2, 128, TQ), BF16),
            pltpu.VMEM((24, TQ), F32),
            pltpu.VMEM((3 * D, TB), F32),
            pltpu.SemaphoreType.DMA((10,)),
        ],
        compiler_params=pltpu.CompilerParams(vmem_limit_bytes=120 * 1024 * 1024),
        name="gmix",
    )(A_x, A_wqkv, A_wo, B_k, B_v, B_ssm_k, B_shift_k.T, B_ssm_D, gate_w, jnp.asarray(_dft_tables(), BF16))
```

```python
import numpy as np
import jax
import jax.numpy as jnp
from jax import lax
import jax.experimental.pallas as pl
import jax.experimental.pallas.tpu as pltpu

S, D, H, DH = 2048, 640, 32, 20
NP = H // 2
TB = 512
NB = S // TB
C = 128
NC = S // C
LT = D // 128
NKT = S // 128
TQ = 512
JL = S // TQ - 1
HN = 2
MB = 4
PU = 2
OBS = (4, 2, 1, 1)
G, FIRST, STEP, LAST, LAG = 64, 5, 6, 4, 3
W_FIN, W_STR = 0.4, 0.5
PEEL = "334q32xQQQQkvKKKKVVVV"
KA = 128

F32, BF16, I32, I16, I8 = jnp.float32, jnp.bfloat16, jnp.int32, jnp.int16, jnp.int8
NT = (((1,), (1,)), ((), ()))
NN = (((1,), (0,)), ((), ()))
QMAX = 2038.0
MAGIC = 12582912.0
MAGIC_BITS = 0x4B400000
SCALE2 = (DH ** -0.5) * 1.4426950408889634
DEQ = 256.0 / (QMAX * QMAX) * SCALE2


def _dft_tables():
    r = np.arange(64, dtype=np.float64)
    f = np.concatenate([2 * r, 127 - 2 * r])
    n = np.arange(128, dtype=np.float64)
    ang = 2.0 * np.pi * (f[:, None] + 0.5) * n[None, :] / 256.0
    fwd = np.concatenate([np.cos(ang), -np.sin(ang)], axis=0)
    inv = np.concatenate([np.cos(ang[:64]).T, -np.sin(ang[:64]).T], axis=1) / 128.0
    inv = np.concatenate([inv[0::2], inv[1::2]], axis=0)
    fwd = fwd.reshape(2, 16, 8, 128).transpose(1, 0, 2, 3).reshape(256, 128)
    return np.concatenate([fwd, inv], axis=0).astype(np.float32)


def _limbs(r, inv):
    t = lax.bitcast_convert_type(r * inv + MAGIC, I32) - (MAGIC_BITS - 8)
    return t >> 4, (t & 15) - 8, (t + 120) >> 8


def _recip(m):
    r = pl.reciprocal(m, approx=True)
    return r * (2.0 - m * r)


def _qscale(m):
    r = pl.reciprocal(m, approx=True)
    return (r * QMAX) * (2.0 - m * r)


def _kernel(x_hbm, wqkv_hbm, wo_hbm, k_hbm, v_hbm, ssm_hbm, shift_hbm, dvec_hbm, gw_hbm, dft_hbm, out_hbm,
            x_v, wqkv_v, wo_v, k_v, v_v, ssm_v, out_v, shift_v, dvec_v, gw_v, dft_v,
            wt, q8, k8, vt, sq, sk, kst, vmx, ot, kvb, us, hs, ys, ysc, qkt, kn, pcar, acar, part0, sems):
    def cp_w(i):
        return pltpu.make_async_copy(wqkv_hbm.at[KA:D, i * D:(i + 1) * D], wqkv_v.at[KA:D, i * D:(i + 1) * D],
                                     sems.at[i])

    cp_wa = pltpu.make_async_copy(wqkv_hbm.at[0:KA, :], wqkv_v.at[0:KA, :], sems.at[9])
    cp_xa = pltpu.make_async_copy(x_hbm.at[0, 0:TB, 0:KA], x_v.at[0:TB, 0:KA], sems.at[9])
    cp_xb = pltpu.make_async_copy(x_hbm.at[0, 0:TB, KA:D], x_v.at[0:TB, KA:D], sems.at[3])

    def cp_x(i):
        return pltpu.make_async_copy(x_hbm.at[0, pl.ds(i * TB, TB), :], x_v.at[pl.ds(i * TB, TB), :],
                                     sems.at[3 + i])

    late = [
        pltpu.make_async_copy(ssm_hbm, ssm_v, sems.at[7]),
        pltpu.make_async_copy(k_hbm.at[0], k_v.at[pl.ds(16, S), :], sems.at[7]),
        pltpu.make_async_copy(v_hbm.at[0], v_v, sems.at[7]),
        pltpu.make_async_copy(wo_hbm, wo_v, sems.at[7]),
        pltpu.make_async_copy(shift_hbm, shift_v, sems.at[7]),
        pltpu.make_async_copy(dvec_hbm, dvec_v, sems.at[7]),
        pltpu.make_async_copy(gw_hbm, gw_v, sems.at[7]),
        pltpu.make_async_copy(dft_hbm, dft_v, sems.at[7]),
    ]

    def cp_out(c0, oc):
        r0 = pl.multiple_of(c0 * C, C)
        return pltpu.make_async_copy(out_v.at[pl.ds(r0, oc * C), :], out_hbm.at[0, pl.ds(r0, oc * C), :], sems.at[8])

    widx = {"q": 0, "k": 1, "v": 2}
    cp_wa.start()
    cp_xa.start()
    for ch in PEEL:
        if ch in widx:
            cp_w(widx[ch]).start()
        elif ch == "x":
            cp_xb.start()
    for i in range(1, NB):
        cp_x(i).start()
    for cp in late:
        cp.start()

    k_v[0:16, :] = jnp.zeros((16, D), BF16)

    low4 = lax.broadcasted_iota(I32, (8, TB), 0) < 4

    def headred(a, op, red):
        mid = a[16:24]
        ma = op(op(a[0:8], a[8:16]), jnp.where(low4, mid, 0.0))
        mb = op(op(a[24:32], a[32:40]), jnp.where(low4, 0.0, mid))
        return red(ma, axis=0, keepdims=True), red(mb, axis=0, keepdims=True)

    def pairscale(ia, ib):
        a8 = jnp.broadcast_to(ia, (8, TB))
        b8 = jnp.broadcast_to(ib, (8, TB))
        return jnp.concatenate([a8, a8, jnp.where(low4, a8, b8), b8, b8], axis=0)

    def slots(l1, l2, l3, mask):
        r2 = pltpu.roll(l2[16:24], 4, 0)
        m3 = l3[16:24]
        a = [l1[0:16], l2[0:16], l3[0:16], jnp.where(low4, l1[16:24], r2), jnp.where(low4, m3, 0) if mask else m3]
        b = [l1[24:40], l2[24:40], l3[24:40], jnp.where(low4, r2, l1[16:24]), jnp.where(low4, 0, m3) if mask else m3]
        return a, b

    def lanefold(a, op):
        return op(op(a[:, 0:128], a[:, 128:256]), op(a[:, 256:384], a[:, 384:512]))

    memo = {}

    def proj(part, g, t0):
        r0 = part * D + 160 * g
        if memo["peel"]:
            return lax.dot_general(wt[r0:r0 + 160, KA:D], x_v[0:TB, KA:D], NT,
                                   preferred_element_type=F32) + part0[r0:r0 + 160, :]
        if g % 2 == 0:
            memo["wide"] = lax.dot_general(wt[r0:r0 + 320, :], x_v[pl.ds(t0, TB), :], NT,
                                           preferred_element_type=F32)
        return memo["wide"][160 * (g % 2):160 * (g % 2 + 1)]

    def kgrp(g, tb, t0):
        rk = proj(1, g, t0)
        for j in range(4):
            p = 4 * g + j
            r = rk[40 * j:40 * (j + 1)]
            ab = jnp.abs(r)
            mida, midb = jnp.where(low4, ab[16:24], 0.0), jnp.where(low4, 0.0, ab[16:24])
            ms = []
            for hh, (u0, u1, u2) in enumerate(((ab[0:8], ab[8:16], mida), (ab[24:32], ab[32:40], midb))):
                l1 = u0 + u1 + u2
                l1m = jnp.sum(jnp.max(lanefold(l1, jnp.maximum), axis=1, keepdims=True), axis=0, keepdims=True)
                l1s = jnp.sum(jnp.sum(lanefold(l1, jnp.add), axis=1, keepdims=True), axis=0, keepdims=True)
                kst[0, tb, 2 * p + hh:2 * p + hh + 1, :] = jnp.broadcast_to(l1m, (1, 128))
                kst[1, tb, 2 * p + hh:2 * p + hh + 1, :] = jnp.broadcast_to(l1s, (1, 128))
                m = lanefold(jnp.maximum(jnp.maximum(u0, u1), u2), jnp.maximum)
                m = jnp.max(jnp.max(m, axis=0, keepdims=True), axis=1, keepdims=True)
                ms.append(jnp.maximum(m, 1e-30))
            ma, mb = ms
            hi, lo, top = _limbs(r, pairscale(_qscale(ma), _qscale(mb)))
            sk[tb, 2 * p:2 * p + 1, :] = jnp.broadcast_to(ma, (1, 128))
            sk[tb, 2 * p + 1:2 * p + 2, :] = jnp.broadcast_to(mb, (1, 128))
            ka, kb = slots(hi, lo, top, False)
            kk = jnp.concatenate(ka + kb, axis=0).astype(I16).T
            kk = jnp.concatenate([kk[kt * 128 + 16 * i:kt * 128 + 16 * (i + 1)]
                                  for kt in range(TB // 128) for i in reversed(range(8))], axis=0)
            k8[p, pl.ds(t0, TB), :] = kk.astype(I8)

    def qgrp(g, tb, t0):
        rq = proj(0, g, t0)
        for j in range(4):
            p = 4 * g + j
            r = rq[40 * j:40 * (j + 1)]
            ma, mb = headred(jnp.abs(r), jnp.maximum, jnp.max)
            ma = jnp.maximum(ma, 1e-30)
            mb = jnp.maximum(mb, 1e-30)
            hi, lo, top = _limbs(r, pairscale(_qscale(ma), _qscale(mb)))
            sq[2 * p:2 * p + 1, pl.ds(t0, TB)] = ma * DEQ
            sq[2 * p + 1:2 * p + 2, pl.ds(t0, TB)] = mb * DEQ
            pa, pb = slots(hi, top, lo, True)
            q8[2 * p, :, pl.ds(t0, TB)] = jnp.concatenate(pa, axis=0).astype(I8)
            q8[2 * p + 1, :, pl.ds(t0, TB)] = jnp.concatenate(pb, axis=0).astype(I8)

    def vgrp(g, tb, t0):
        rv = proj(2, g, t0)
        vmx[8 * g:8 * (g + 1), pl.ds(t0, TB)] = jnp.max(jnp.abs(rv).reshape(20, 8, TB), axis=0)
        for j in range(4):
            p = 4 * g + j
            r = rv[40 * j:40 * (j + 1)]
            mid = r[16:24]
            vt[2 * p, :, pl.ds(t0, TB)] = jnp.concatenate([r[0:16], jnp.where(low4, mid, 1.0)], axis=0)
            vt[2 * p + 1, :, pl.ds(t0, TB)] = jnp.concatenate([jnp.where(low4, 1.0, mid), r[24:40]], axis=0)

    grp = {"K": kgrp, "Q": qgrp, "V": vgrp}
    cnt = {"K": 0, "Q": 0, "V": 0}
    memo["peel"] = True
    cp_wa.wait()
    cp_xa.wait()
    atiles = list(range(0, 5)) + list(range(10, 15)) + list(range(5, 10))
    for t in atiles:
        wt[t * 128:(t + 1) * 128, 0:KA] = wqkv_v[0:KA, t * 128:(t + 1) * 128].T
    todo = []
    for ch in PEEL:
        if ch in widx:
            cp_w(widx[ch]).wait()
            todo.append(widx[ch])
            continue
        elif ch == "x":
            cp_xb.wait()
            continue
        for i in todo:
            for t in range(LT):
                c0 = i * D + t * 128
                wt[c0:c0 + 128, KA:D] = wqkv_v[KA:D, c0:c0 + 128].T
        todo = []
        if ch.isdigit():
            ts = [atiles.pop(0) for _ in range(int(ch))]
            wa = jnp.concatenate([wt[t * 128:(t + 1) * 128, 0:KA] for t in ts], axis=0)
            pa = lax.dot_general(wa, x_v[0:TB, 0:KA], NT, preferred_element_type=F32)
            for i, t in enumerate(ts):
                part0[t * 128:(t + 1) * 128, :] = pa[i * 128:(i + 1) * 128]
        else:
            grp[ch](cnt[ch], 0, 0)
            cnt[ch] += 1
    assert not atiles
    memo["peel"] = False

    def p1(tb, carry):
        t0 = pl.multiple_of(tb * TB, TB)
        cp_x(tb).wait()
        for ch in "QKV":
            for g in range(4):
                grp[ch](g, tb, t0)
        return carry

    lax.fori_loop(1, NB, p1, 0)

    for cp in late:
        cp.wait()

    qinf = jnp.max(sq[...], axis=1, keepdims=True) * (SCALE2 / DEQ)
    bad = jnp.where(jnp.max(vmx[...], axis=1, keepdims=True) <= 2.0 ** 50, 0.0, 1.0)
    for tb in range(NB):
        bad = bad + jnp.where(qinf * kst[0, tb] <= 60.0, 0.0, 1.0)
        bad = bad + jnp.where(qinf + kst[0, tb] <= 1e15, 0.0, 1.0)
        bad = bad + jnp.where(sk[tb] * (DH * TB) <= 10.0 * kst[1, tb] + 1e-25, 0.0, 1.0)
    fast = jnp.sum(bad) == 0.0

    def reim(val):
        n = val.shape[1]
        val = val.reshape(16, 16, n)
        return val[:, 0:8], val[:, 8:16]

    sh = shift_v[...].astype(F32)
    hprev = [None] * LT

    def hdft(c0, lt):
        ls = slice(lt * 128, (lt + 1) * 128)
        hb = jnp.concatenate([ssm_v[ls, (c0 + i) * C:(c0 + i + 1) * C] for i in range(HN)], axis=0)
        hr, hi = reim(lax.dot_general(dft_v[0:256, :], hb, NT, preferred_element_type=F32))
        for i in range(HN):
            cr, ci = hr[:, :, i * 128:(i + 1) * 128], hi[:, :, i * 128:(i + 1) * 128]
            if hprev[lt] is None:
                hs[:, c0 + i, :, ls] = cr
                hs[:, NC + c0 + i, :, ls] = ci
            else:
                pr, pi = hprev[lt]
                hs[:, c0 + i, :, ls] = jnp.concatenate([cr[0:8] - pi[0:8], cr[8:] + pi[8:]], axis=0)
                hs[:, NC + c0 + i, :, ls] = jnp.concatenate([ci[0:8] + pr[0:8], ci[8:] - pr[8:]], axis=0)
            hprev[lt] = (cr, ci)

    def udft(c0, lt):
        ls = slice(lt * 128, (lt + 1) * 128)
        r0, n = c0 * C, HN * C
        win = k_v[r0:r0 + n + 16, ls].astype(F32)
        ks = (win[16:] * sh[0:1, ls] + win[15:n + 15] * sh[1:2, ls]
              + win[14:n + 14] * sh[2:3, ls] + win[13:n + 13] * sh[3:4, ls])
        kv = ks * v_v[r0:r0 + n, ls].astype(F32)
        kvb[r0:r0 + n, ls] = kv.astype(BF16)
        kw = jnp.concatenate([kv[i * C:(i + 1) * C] for i in range(HN)], axis=1).astype(BF16)
        ur, ui = reim(jnp.dot(dft_v[0:256, :], kw, preferred_element_type=F32))
        for i in range(HN):
            us[:, c0 + i, :, ls] = ur[:, :, i * 128:(i + 1) * 128]
            us[:, NC + c0 + i, :, ls] = ui[:, :, i * 128:(i + 1) * 128]

    for lt in range(LT):
        for c0 in range(0, NC, HN):
            hdft(c0, lt)
            udft(c0, lt)

    def mac_tasks(ft, lts):
        tasks = []

        def lanes(lt):
            return slice(lt * 128, (lt + 1) * 128) if isinstance(lt, int) else pl.ds(pl.multiple_of(lt * 128, 128), 128)

        for li, lt in enumerate(lts):
            for ab in range(NC // MB):
                st = {"r": [None] * MB, "i": [None] * MB, "id": (len(tasks), li, ab)}
                for cb in range(ab + 1):
                    for m in range(2):
                        for i in range(MB):
                            js = [j for j in range(MB) if (ab - cb) * MB + i - j >= 0]

                            def task(cache, z, lt=lt, ab=ab, m=m, cb=cb, i=i, js=js, st=st):
                                yr, yi = st["r"], st["i"]

                                def ld(ref, name, slot, pin):
                                    key = (st["id"], name, slot)
                                    if key not in cache:
                                        val = ref[ft, slot, :, lanes(lt)]
                                        cache[key] = val + z if (pin and z is not None) else val
                                    return cache[key]

                                for j in js:
                                    hv = ld(hs, "h", m * NC + (ab - cb) * MB + i - j, True)
                                    ta = ld(us, "u", cb * MB + j, False) * hv
                                    tb_ = ld(us, "u", NC + cb * MB + j, False) * hv
                                    if m == 0:
                                        yr[i] = ta if yr[i] is None else yr[i] + ta
                                        yi[i] = tb_ if yi[i] is None else yi[i] + tb_
                                    else:
                                        yr[i] = yr[i] - tb_
                                        yi[i] = yi[i] + ta
                                if cb == ab and m == 1:
                                    ys[ft, ab * MB + i, :, lanes(lt)] = yr[i]
                                    ys[ft, NC + ab * MB + i, :, lanes(lt)] = yi[i]

                            tasks.append((4 * len(js), task))
        return tasks

    def finish(p, hh, acc, cols):
        if hh == 0:
            ot[p, 0:24, cols] = acc * _recip(acc[20:21])
        else:
            b = acc * _recip(acc[0:1])
            ot[p, 20:24, cols] = b[4:8]
            ot[p, 24:40, cols] = b[8:24]

    def pv_tile(h, t, pt, acc):
        o = lax.dot_general(vt[h, :, t * 128:(t + 1) * 128], pt, NN, preferred_element_type=F32)
        return o if acc is None else o + acc

    def drain(p):
        acc = acar[...]
        for i in range(2):
            acc = pv_tile(2 * p + 1, NKT - 2 + i, pcar[i], acc)
        finish(p, 1, acc, slice(JL * TQ, (JL + 1) * TQ))

    def p2(pb, carry):
        heads = [(pi, j, hh) for pi in range(PU) for j in range(S // TQ) for hh in range(2)]
        hu = S // G
        sizes = [FIRST]
        while len(heads) * hu - sum(sizes) - LAST > STEP:
            sizes.append(STEP)
        sizes += [len(heads) * hu - sum(sizes) - LAST, LAST]
        steps, g0 = [], 0
        for left in sizes:
            segs = []
            while left:
                u, h0 = divmod(g0, hu)
                nh = min(left, hu - h0)
                segs.append(heads[u] + (h0, nh))
                g0 += nh
                left -= nh
            steps.append(segs)
        tasks = [(c, t, pi) for pi in range(PU) for c, t in mac_tasks(pb * PU + pi, range(LT))]
        accs, pend, part, pos = {}, [], [], [0]

        def qk(pi, j, hh, h0, nh):
            p = pb * PU + pi
            h = 2 * p + hh
            wq = sq[pl.ds(h, 1), j * TQ:(j + 1) * TQ]
            qh = [q8[h, :, j * TQ:(j + 1) * TQ], jnp.zeros((64, TQ), I8)]
            s = jnp.dot(k8[p, h0 * G:(h0 + nh) * G, :], jnp.concatenate(qh if hh == 0 else qh[::-1], axis=0),
                        preferred_element_type=I32)
            ws = {}
            for t in range(nh):
                kb = (h0 + t) * G // TB
                if kb not in ws:
                    ws[kb] = wq * jnp.concatenate([sk[kb, pl.ds(h, 1), :]] * (TQ // 128), axis=1)
                e = jnp.exp2(s[t * G:(t + 1) * G].astype(F32) * ws[kb])
                part.extend(e[16 * i:16 * (i + 1)] for i in range(G // 16))
                pos[0] += 1
                if len(part) == 8:
                    pt = jnp.concatenate(part[::-1], axis=0).astype(BF16)
                    pend.append((pos[0], pi, j, hh, (h0 + t) * G // 128, pt))
                    part.clear()

        def pv(_, pi, j, hh, t, pt):
            p = pb * PU + pi
            acc = pv_tile(2 * p + hh, t, pt, accs.get((j, hh)))
            accs[(j, hh)] = acc
            if t == NKT - 1:
                finish(p, hh, accs.pop((j, hh)), slice(j * TQ, (j + 1) * TQ))
            return acc

        n = len(steps)
        wts, issued, tiles = [], 0, -2
        for i in range(n - 1):
            issued += sizes[i]
            nd = (issued - LAG) * G // 128
            wts.append(nd - tiles - (W_FIN if nd // NKT != tiles // NKT else 0.0)
                       - (W_STR if len(steps[i + 1]) > 1 else 0.0))
            tiles = nd
        total = float(sum(t[0] for t in tasks))
        ti, done, cum = 0, 0.0, 0.0
        for i in range(n):
            for seg in steps[i]:
                qk(*seg)
            if i == 0:
                drain(jnp.maximum(pb * PU - 1, 0))
            outs = []
            while pend and (pend[0][0] <= pos[0] - LAG if i < n - 1 else len(pend) > 2):
                outs.append(pv(*pend.pop(0)))
            if i < n - 1:
                for ui in range(2):
                    z = jnp.minimum(jnp.abs(outs[min(ui, len(outs) - 1)][0:8, 0:128]), 0.0)
                    cum += wts[i] / sum(wts) * total / 2
                    caches = {}
                    while ti < len(tasks) and (done + tasks[ti][0] / 2 <= cum or (i == n - 2 and ui == 1)):
                        tasks[ti][1](caches.setdefault(tasks[ti][2], {}), z)
                        done += tasks[ti][0]
                        ti += 1
        for i in range(2):
            pcar[i] = pend[i][5]
        acar[...] = accs.pop((JL, 1))
        return carry

    pcar[...] = jnp.zeros((2, 128, TQ), BF16)
    acar[...] = jnp.ones((24, TQ), F32)

    def attn_fast():
        lax.fori_loop(0, NP // PU, p2, 0)
        drain(NP - 1)

    def attn_general():
        def fb1(i, carry):
            r0 = pl.multiple_of((i // NB) * 160, 32)
            t0 = pl.multiple_of((i % NB) * TB, TB)
            qkt[pl.ds(r0, 160), pl.ds(t0, TB)] = lax.dot_general(
                wt[pl.ds(r0, 160), :], x_v[pl.ds(t0, TB), :], NT, preferred_element_type=F32)
            return carry

        lax.fori_loop(0, 8 * NB, fb1, 0)

        def fb2(p, carry):
            r0 = pl.multiple_of(40 * p, 8)

            def tr(kt, c2):
                c0 = pl.multiple_of(kt * 128, 128)
                blk = jnp.concatenate([qkt[pl.ds(D + r0, 40), pl.ds(c0, 128)], jnp.zeros((88, 128), F32)], axis=0)
                kn[pl.ds(c0, 128), :] = blk.T.astype(BF16)
                return c2

            lax.fori_loop(0, NKT, tr, 0)
            rows = lax.broadcasted_iota(I32, (40, TQ), 0)
            for hh in range(2):
                def qtile(j, c2, hh=hh):
                    c0 = pl.multiple_of(j * TQ, TQ)
                    qm = jnp.where((rows >= DH * hh) & (rows < DH * hh + DH),
                                   qkt[pl.ds(r0, 40), pl.ds(c0, TQ)], 0.0)
                    qm = jnp.concatenate([qm, jnp.zeros((88, TQ), F32)], axis=0).astype(BF16)

                    def kchunk(c, st):
                        m, acc = st
                        k0 = pl.multiple_of(c * 128, 128)
                        s = jnp.dot(kn[pl.ds(k0, 128), :], qm, preferred_element_type=F32) * SCALE2
                        mn = jnp.maximum(m, jnp.max(s, axis=0, keepdims=True))
                        e = jnp.exp2(s - mn).astype(BF16)
                        o = lax.dot_general(vt[2 * p + hh, :, pl.ds(k0, 128)], e, NN, preferred_element_type=F32)
                        return mn, o + acc * jnp.exp2(m - mn)

                    m0 = jnp.full((1, TQ), -jnp.inf, F32)
                    _, acc = lax.fori_loop(0, NKT, kchunk, (m0, jnp.zeros((24, TQ), F32)))
                    finish(p, hh, acc, pl.ds(c0, TQ))
                    return c2

                lax.fori_loop(0, S // TQ, qtile, 0)

            def mac(lt, c2):
                cache = {}
                for _, task in mac_tasks(p, [lt]):
                    task(cache, None)
                return c2

            lax.fori_loop(0, LT, mac, 0)
            return carry

        lax.fori_loop(0, NP, fb2, 0)

    lax.cond(fast, attn_fast, attn_general)

    gw = gw_v[...].astype(F32).reshape(1, D)
    dv = dvec_v[...].astype(F32).reshape(1, D)

    def p4(it, carry):
        off = 0
        for sb, oc in enumerate(OBS):
            c0 = it * sum(OBS) + off
            off += oc
            ob = oc * C
            t0 = pl.multiple_of(c0 * C, C)
            s0 = (sb % 2) * max(OBS) * LT
            yr = jnp.concatenate([ys[:, c0 + i].reshape(128, D) for i in range(oc)], axis=1)
            yi = jnp.concatenate([ys[:, NC + c0 + i].reshape(128, D) for i in range(oc)], axis=1)
            ar, br, ai, bi = yr[0:64], yr[64:128], yi[0:64], yi[64:128]
            ye = jnp.dot(dft_v[256:320, :], jnp.concatenate([ar + br, ai - bi], axis=0).astype(BF16),
                         preferred_element_type=F32)
            yo = jnp.dot(dft_v[320:384, :], jnp.concatenate([ar - br, ai + bi], axis=0).astype(BF16),
                         preferred_element_type=F32)
            for i in range(oc * LT):
                ysc[s0 + i, pl.ds(0, 64, stride=2), :] = ye[:, i * 128:(i + 1) * 128]
                ysc[s0 + i, pl.ds(1, 64, stride=2), :] = yo[:, i * 128:(i + 1) * 128]
            y = jnp.concatenate(
                [jnp.concatenate([ysc[s0 + i * LT + lt] for lt in range(LT)], axis=1) for i in range(oc)], axis=0)
            o = ot[:, :, pl.ds(t0, ob)].reshape(D, ob).astype(BF16).T
            a = jnp.dot(o, wo_v[...], preferred_element_type=F32)
            xf = x_v[pl.ds(t0, ob), :].astype(F32)
            g = jax.nn.sigmoid(jnp.sum(xf * gw, axis=-1, keepdims=True))
            b = xf * (y + kvb[pl.ds(t0, ob), :].astype(F32) * dv)
            out_v[pl.ds(t0, ob), :] = (b + g * (a - b)).astype(BF16)
            cp_out(c0, oc).start()
        return carry

    lax.fori_loop(0, NC // sum(OBS), p4, 0)
    cp_out(0, NC).wait()


@jax.jit
def pallas_gated_mix__mha_block__ssm_conv_h3__prompt_kernel(A_x, A_wqkv, A_wo, B_q, B_k, B_v, B_shift_k, B_ssm_k, B_ssm_D, gate_w):
    del B_q
    hbm = pl.BlockSpec(memory_space=pl.ANY)
    return pl.pallas_call(
        _kernel,
        out_shape=jax.ShapeDtypeStruct((1, S, D), BF16),
        in_specs=[hbm] * 10,
        out_specs=hbm,
        scratch_shapes=[
            pltpu.VMEM((S, D), BF16),
            pltpu.VMEM((D, 3 * D), BF16),
            pltpu.VMEM((D, D), BF16),
            pltpu.VMEM((S + 16, D), BF16),
            pltpu.VMEM((S, D), BF16),
            pltpu.VMEM((D, S), BF16),
            pltpu.VMEM((S, D), BF16),
            pltpu.VMEM((4, D), BF16),
            pltpu.VMEM((D,), BF16),
            pltpu.VMEM((D,), BF16),
            pltpu.VMEM((384, 128), BF16),
            pltpu.VMEM((3 * D, D), BF16),
            pltpu.VMEM((H, 64, S), I8),
            pltpu.VMEM((NP, S, 128), I8),
            pltpu.VMEM((H, 24, S), F32),
            pltpu.VMEM((H, S), F32),
            pltpu.VMEM((NB, H, 128), F32),
            pltpu.VMEM((2, NB, H, 128), F32),
            pltpu.VMEM((32, S), F32),
            pltpu.VMEM((NP, 40, S), F32),
            pltpu.VMEM((S, D), BF16),
            pltpu.VMEM((16, 2 * NC, 8, D), F32),
            pltpu.VMEM((16, 2 * NC, 8, D), F32),
            pltpu.VMEM((16, 2 * NC, 8, D), F32),
            pltpu.VMEM((2 * max(OBS) * LT, 128, 128), F32),
            pltpu.VMEM((2 * D, S), F32),
            pltpu.VMEM((S, 128), BF16),
            pltpu.VMEM((2, 128, TQ), BF16),
            pltpu.VMEM((24, TQ), F32),
            pltpu.VMEM((3 * D, TB), F32),
            pltpu.SemaphoreType.DMA((10,)),
        ],
        compiler_params=pltpu.CompilerParams(vmem_limit_bytes=120 * 1024 * 1024),
        name="gmix",
    )(A_x, A_wqkv, A_wo, B_k, B_v, B_ssm_k, B_shift_k.T, B_ssm_D, gate_w, jnp.asarray(_dft_tables(), BF16))
```

```python
import numpy as np
import jax
import jax.numpy as jnp
from jax import lax
import jax.experimental.pallas as pl
import jax.experimental.pallas.tpu as pltpu

S, D, H, DH = 2048, 640, 32, 20
NP = H // 2
TB = 512
NB = S // TB
C = 128
NC = S // C
LT = D // 128
NKT = S // 128
TQ = 512
JL = S // TQ - 1
HN = 2
MB = 4
PU = 2
OBS = (4, 2, 1, 1)
G, FIRST, STEP, LAST, LAG = 64, 5, 6, 4, 3
W_FIN, W_STR = 0.4, 0.5
PEEL = "334q32xQQQQkvKKKKVVVV"
KA = 128

F32, BF16, I32, I16, I8 = jnp.float32, jnp.bfloat16, jnp.int32, jnp.int16, jnp.int8
NT = (((1,), (1,)), ((), ()))
NN = (((1,), (0,)), ((), ()))
QMAX = 2038.0
MAGIC = 12582912.0
MAGIC_BITS = 0x4B400000
SCALE2 = (DH ** -0.5) * 1.4426950408889634
DEQ = 256.0 / (QMAX * QMAX) * SCALE2


def _dft_tables():
    r = np.arange(64, dtype=np.float64)
    f = np.concatenate([2 * r, 127 - 2 * r])
    n = np.arange(128, dtype=np.float64)
    ang = 2.0 * np.pi * (f[:, None] + 0.5) * n[None, :] / 256.0
    fwd = np.concatenate([np.cos(ang), -np.sin(ang)], axis=0)
    inv = np.concatenate([np.cos(ang[:64]).T, -np.sin(ang[:64]).T], axis=1) / 128.0
    inv = np.concatenate([inv[0::2], inv[1::2]], axis=0)
    fwd = fwd.reshape(2, 16, 8, 128).transpose(1, 0, 2, 3).reshape(256, 128)
    return np.concatenate([fwd, inv], axis=0).astype(np.float32)


def _limbs(r, inv):
    t = lax.bitcast_convert_type(r * inv + MAGIC, I32) - (MAGIC_BITS - 8)
    return t >> 4, (t & 15) - 8, (t + 120) >> 8


def _recip(m):
    r = pl.reciprocal(m, approx=True)
    return r * (2.0 - m * r)


def _qscale(m):
    r = pl.reciprocal(m, approx=True)
    return (r * QMAX) * (2.0 - m * r)


def _kernel(x_hbm, wqkv_hbm, wo_hbm, k_hbm, v_hbm, ssm_hbm, shift_hbm, dvec_hbm, gw_hbm, dft_hbm, out_hbm,
            x_v, wqkv_v, wo_v, k_v, v_v, ssm_v, out_v, shift_v, dvec_v, gw_v, dft_v,
            wt, q8, k8, vt, sq, sk, kst, vmx, ot, kvb, us, hs, ys, ysc, qkt, kn, pcar, acar, part0, sems):
    def cp_w(i):
        return pltpu.make_async_copy(wqkv_hbm.at[KA:D, i * D:(i + 1) * D], wqkv_v.at[KA:D, i * D:(i + 1) * D],
                                     sems.at[i])

    cp_wa = pltpu.make_async_copy(wqkv_hbm.at[0:KA, :], wqkv_v.at[0:KA, :], sems.at[9])
    cp_xa = pltpu.make_async_copy(x_hbm.at[0, 0:TB, 0:KA], x_v.at[0:TB, 0:KA], sems.at[9])
    cp_xb = pltpu.make_async_copy(x_hbm.at[0, 0:TB, KA:D], x_v.at[0:TB, KA:D], sems.at[3])

    def cp_x(i):
        return pltpu.make_async_copy(x_hbm.at[0, pl.ds(i * TB, TB), :], x_v.at[pl.ds(i * TB, TB), :],
                                     sems.at[3 + i])

    late = [
        pltpu.make_async_copy(ssm_hbm, ssm_v, sems.at[7]),
        pltpu.make_async_copy(k_hbm.at[0], k_v.at[pl.ds(16, S), :], sems.at[7]),
        pltpu.make_async_copy(v_hbm.at[0], v_v, sems.at[7]),
        pltpu.make_async_copy(wo_hbm, wo_v, sems.at[7]),
        pltpu.make_async_copy(shift_hbm, shift_v, sems.at[7]),
        pltpu.make_async_copy(dvec_hbm, dvec_v, sems.at[7]),
        pltpu.make_async_copy(gw_hbm, gw_v, sems.at[7]),
        pltpu.make_async_copy(dft_hbm, dft_v, sems.at[7]),
    ]

    def cp_out(c0, oc):
        r0 = pl.multiple_of(c0 * C, C)
        return pltpu.make_async_copy(out_v.at[pl.ds(r0, oc * C), :], out_hbm.at[0, pl.ds(r0, oc * C), :], sems.at[8])

    widx = {"q": 0, "k": 1, "v": 2}
    cp_wa.start()
    cp_xa.start()
    for ch in PEEL:
        if ch in widx:
            cp_w(widx[ch]).start()
        elif ch == "x":
            cp_xb.start()
    for i in range(1, NB):
        cp_x(i).start()
    for cp in late:
        cp.start()

    k_v[0:16, :] = jnp.zeros((16, D), BF16)

    low4 = lax.broadcasted_iota(I32, (8, TB), 0) < 4

    def headred(a, op, red):
        mid = a[16:24]
        ma = op(op(a[0:8], a[8:16]), jnp.where(low4, mid, 0.0))
        mb = op(op(a[24:32], a[32:40]), jnp.where(low4, 0.0, mid))
        return red(ma, axis=0, keepdims=True), red(mb, axis=0, keepdims=True)

    def pairscale(ia, ib):
        a8 = jnp.broadcast_to(ia, (8, TB))
        b8 = jnp.broadcast_to(ib, (8, TB))
        return jnp.concatenate([a8, a8, jnp.where(low4, a8, b8), b8, b8], axis=0)

    def slots(l1, l2, l3, mask):
        r2 = pltpu.roll(l2[16:24], 4, 0)
        m3 = l3[16:24]
        a = [l1[0:16], l2[0:16], l3[0:16], jnp.where(low4, l1[16:24], r2), jnp.where(low4, m3, 0) if mask else m3]
        b = [l1[24:40], l2[24:40], l3[24:40], jnp.where(low4, r2, l1[16:24]), jnp.where(low4, 0, m3) if mask else m3]
        return a, b

    def lanefold(a, op):
        return op(op(a[:, 0:128], a[:, 128:256]), op(a[:, 256:384], a[:, 384:512]))

    memo = {}

    def proj(part, g, t0):
        r0 = part * D + 160 * g
        if memo["peel"]:
            return lax.dot_general(wt[r0:r0 + 160, KA:D], x_v[0:TB, KA:D], NT,
                                   preferred_element_type=F32) + part0[r0:r0 + 160, :]
        if g % 2 == 0:
            memo["wide"] = lax.dot_general(wt[r0:r0 + 320, :], x_v[pl.ds(t0, TB), :], NT,
                                           preferred_element_type=F32)
        return memo["wide"][160 * (g % 2):160 * (g % 2 + 1)]

    def kgrp(g, tb, t0):
        rk = proj(1, g, t0)
        for j in range(4):
            p = 4 * g + j
            r = rk[40 * j:40 * (j + 1)]
            ab = jnp.abs(r)
            mida, midb = jnp.where(low4, ab[16:24], 0.0), jnp.where(low4, 0.0, ab[16:24])
            ms = []
            for hh, (u0, u1, u2) in enumerate(((ab[0:8], ab[8:16], mida), (ab[24:32], ab[32:40], midb))):
                l1 = u0 + u1 + u2
                l1m = jnp.sum(jnp.max(lanefold(l1, jnp.maximum), axis=1, keepdims=True), axis=0, keepdims=True)
                l1s = jnp.sum(jnp.sum(lanefold(l1, jnp.add), axis=1, keepdims=True), axis=0, keepdims=True)
                kst[0, tb, 2 * p + hh:2 * p + hh + 1, :] = jnp.broadcast_to(l1m, (1, 128))
                kst[1, tb, 2 * p + hh:2 * p + hh + 1, :] = jnp.broadcast_to(l1s, (1, 128))
                m = lanefold(jnp.maximum(jnp.maximum(u0, u1), u2), jnp.maximum)
                m = jnp.max(jnp.max(m, axis=0, keepdims=True), axis=1, keepdims=True)
                ms.append(jnp.maximum(m, 1e-30))
            ma, mb = ms
            hi, lo, top = _limbs(r, pairscale(_qscale(ma), _qscale(mb)))
            sk[tb, 2 * p:2 * p + 1, :] = jnp.broadcast_to(ma, (1, 128))
            sk[tb, 2 * p + 1:2 * p + 2, :] = jnp.broadcast_to(mb, (1, 128))
            ka, kb = slots(hi, lo, top, False)
            kk = jnp.concatenate(ka + kb, axis=0).astype(I16).T
            kk = jnp.concatenate([kk[kt * 128 + 16 * i:kt * 128 + 16 * (i + 1)]
                                  for kt in range(TB // 128) for i in reversed(range(8))], axis=0)
            k8[p, pl.ds(t0, TB), :] = kk.astype(I8)

    def qgrp(g, tb, t0):
        rq = proj(0, g, t0)
        for j in range(4):
            p = 4 * g + j
            r = rq[40 * j:40 * (j + 1)]
            ma, mb = headred(jnp.abs(r), jnp.maximum, jnp.max)
            ma = jnp.maximum(ma, 1e-30)
            mb = jnp.maximum(mb, 1e-30)
            hi, lo, top = _limbs(r, pairscale(_qscale(ma), _qscale(mb)))
            sq[2 * p:2 * p + 1, pl.ds(t0, TB)] = ma * DEQ
            sq[2 * p + 1:2 * p + 2, pl.ds(t0, TB)] = mb * DEQ
            pa, pb = slots(hi, top, lo, True)
            q8[2 * p, :, pl.ds(t0, TB)] = jnp.concatenate(pa, axis=0).astype(I8)
            q8[2 * p + 1, :, pl.ds(t0, TB)] = jnp.concatenate(pb, axis=0).astype(I8)

    def vgrp(g, tb, t0):
        rv = proj(2, g, t0)
        vmx[8 * g:8 * (g + 1), pl.ds(t0, TB)] = jnp.max(jnp.abs(rv).reshape(20, 8, TB), axis=0)
        for j in range(4):
            p = 4 * g + j
            r = rv[40 * j:40 * (j + 1)]
            mid = r[16:24]
            vt[2 * p, :, pl.ds(t0, TB)] = jnp.concatenate([r[0:16], jnp.where(low4, mid, 1.0)], axis=0)
            vt[2 * p + 1, :, pl.ds(t0, TB)] = jnp.concatenate([jnp.where(low4, 1.0, mid), r[24:40]], axis=0)

    grp = {"K": kgrp, "Q": qgrp, "V": vgrp}
    cnt = {"K": 0, "Q": 0, "V": 0}
    memo["peel"] = True
    cp_wa.wait()
    cp_xa.wait()
    atiles = list(range(0, 5)) + list(range(10, 15)) + list(range(5, 10))
    for t in atiles:
        wt[t * 128:(t + 1) * 128, 0:KA] = wqkv_v[0:KA, t * 128:(t + 1) * 128].T
    todo = []
    for ch in PEEL:
        if ch in widx:
            cp_w(widx[ch]).wait()
            todo.append(widx[ch])
            continue
        elif ch == "x":
            cp_xb.wait()
            continue
        for i in todo:
            for t in range(LT):
                c0 = i * D + t * 128
                wt[c0:c0 + 128, KA:D] = wqkv_v[KA:D, c0:c0 + 128].T
        todo = []
        if ch.isdigit():
            ts = [atiles.pop(0) for _ in range(int(ch))]
            wa = jnp.concatenate([wt[t * 128:(t + 1) * 128, 0:KA] for t in ts], axis=0)
            pa = lax.dot_general(wa, x_v[0:TB, 0:KA], NT, preferred_element_type=F32)
            for i, t in enumerate(ts):
                part0[t * 128:(t + 1) * 128, :] = pa[i * 128:(i + 1) * 128]
        else:
            grp[ch](cnt[ch], 0, 0)
            cnt[ch] += 1
    assert not atiles
    memo["peel"] = False

    def p1(tb, carry):
        t0 = pl.multiple_of(tb * TB, TB)
        cp_x(tb).wait()
        for ch in "QKV":
            for g in range(4):
                grp[ch](g, tb, t0)
        return carry

    lax.fori_loop(1, NB, p1, 0)

    for cp in late:
        cp.wait()

    qinf = jnp.max(sq[...], axis=1, keepdims=True) * (SCALE2 / DEQ)
    bad = jnp.where(jnp.max(vmx[...], axis=1, keepdims=True) <= 2.0 ** 50, 0.0, 1.0)
    for tb in range(NB):
        bad = bad + jnp.where(qinf * kst[0, tb] <= 60.0, 0.0, 1.0)
        bad = bad + jnp.where(qinf + kst[0, tb] <= 1e15, 0.0, 1.0)
        bad = bad + jnp.where(sk[tb] * (DH * TB) <= 10.0 * kst[1, tb] + 1e-25, 0.0, 1.0)
    fast = jnp.sum(bad) == 0.0

    def reim(val):
        n = val.shape[1]
        val = val.reshape(16, 16, n)
        return val[:, 0:8], val[:, 8:16]

    sh = shift_v[...].astype(F32)
    hprev = [None] * LT

    def hdft(c0, lt):
        ls = slice(lt * 128, (lt + 1) * 128)
        hb = jnp.concatenate([ssm_v[ls, (c0 + i) * C:(c0 + i + 1) * C] for i in range(HN)], axis=0)
        hr, hi = reim(lax.dot_general(dft_v[0:256, :], hb, NT, preferred_element_type=F32))
        for i in range(HN):
            cr, ci = hr[:, :, i * 128:(i + 1) * 128], hi[:, :, i * 128:(i + 1) * 128]
            if hprev[lt] is None:
                hs[:, c0 + i, :, ls] = cr
                hs[:, NC + c0 + i, :, ls] = ci
            else:
                pr, pi = hprev[lt]
                hs[:, c0 + i, :, ls] = jnp.concatenate([cr[0:8] - pi[0:8], cr[8:] + pi[8:]], axis=0)
                hs[:, NC + c0 + i, :, ls] = jnp.concatenate([ci[0:8] + pr[0:8], ci[8:] - pr[8:]], axis=0)
            hprev[lt] = (cr, ci)

    def udft(c0, lt):
        ls = slice(lt * 128, (lt + 1) * 128)
        r0, n = c0 * C, HN * C
        win = k_v[r0:r0 + n + 16, ls].astype(F32)
        ks = (win[16:] * sh[0:1, ls] + win[15:n + 15] * sh[1:2, ls]
              + win[14:n + 14] * sh[2:3, ls] + win[13:n + 13] * sh[3:4, ls])
        kv = ks * v_v[r0:r0 + n, ls].astype(F32)
        kvb[r0:r0 + n, ls] = kv.astype(BF16)
        kw = jnp.concatenate([kv[i * C:(i + 1) * C] for i in range(HN)], axis=1).astype(BF16)
        ur, ui = reim(jnp.dot(dft_v[0:256, :], kw, preferred_element_type=F32))
        for i in range(HN):
            us[:, c0 + i, :, ls] = ur[:, :, i * 128:(i + 1) * 128]
            us[:, NC + c0 + i, :, ls] = ui[:, :, i * 128:(i + 1) * 128]

    for lt in range(LT):
        for c0 in range(0, NC, HN):
            hdft(c0, lt)
            udft(c0, lt)

    def mac_tasks(ft, lts):
        tasks = []

        def lanes(lt):
            return slice(lt * 128, (lt + 1) * 128) if isinstance(lt, int) else pl.ds(pl.multiple_of(lt * 128, 128), 128)

        for li, lt in enumerate(lts):
            for ab in range(NC // MB):
                st = {"r": [None] * MB, "i": [None] * MB, "id": (len(tasks), li, ab)}
                for cb in range(ab + 1):
                    for m in range(2):
                        for i in range(MB):
                            js = [j for j in range(MB) if (ab - cb) * MB + i - j >= 0]

                            def task(cache, z, lt=lt, ab=ab, m=m, cb=cb, i=i, js=js, st=st):
                                yr, yi = st["r"], st["i"]

                                def ld(ref, name, slot, pin):
                                    key = (st["id"], name, slot)
                                    if key not in cache:
                                        val = ref[ft, slot, :, lanes(lt)]
                                        cache[key] = val + z if (pin and z is not None) else val
                                    return cache[key]

                                for j in js:
                                    hv = ld(hs, "h", m * NC + (ab - cb) * MB + i - j, True)
                                    ta = ld(us, "u", cb * MB + j, False) * hv
                                    tb_ = ld(us, "u", NC + cb * MB + j, False) * hv
                                    if m == 0:
                                        yr[i] = ta if yr[i] is None else yr[i] + ta
                                        yi[i] = tb_ if yi[i] is None else yi[i] + tb_
                                    else:
                                        yr[i] = yr[i] - tb_
                                        yi[i] = yi[i] + ta
                                if cb == ab and m == 1:
                                    ys[ft, ab * MB + i, :, lanes(lt)] = yr[i]
                                    ys[ft, NC + ab * MB + i, :, lanes(lt)] = yi[i]

                            tasks.append((4 * len(js), task))
        return tasks

    def finish(p, hh, acc, cols):
        if hh == 0:
            ot[p, 0:24, cols] = acc * _recip(acc[20:21])
        else:
            b = acc * _recip(acc[0:1])
            ot[p, 20:24, cols] = b[4:8]
            ot[p, 24:40, cols] = b[8:24]

    def pv_tile(h, t, pt, acc):
        o = lax.dot_general(vt[h, :, t * 128:(t + 1) * 128], pt, NN, preferred_element_type=F32)
        return o if acc is None else o + acc

    def drain(p):
        acc = acar[...]
        for i in range(2):
            acc = pv_tile(2 * p + 1, NKT - 2 + i, pcar[i], acc)
        finish(p, 1, acc, slice(JL * TQ, (JL + 1) * TQ))

    def p2(pb, carry):
        heads = [(pi, j, hh) for pi in range(PU) for j in range(S // TQ) for hh in range(2)]
        hu = S // G
        sizes = [FIRST]
        while len(heads) * hu - sum(sizes) - LAST > STEP:
            sizes.append(STEP)
        sizes += [len(heads) * hu - sum(sizes) - LAST, LAST]
        steps, g0 = [], 0
        for left in sizes:
            segs = []
            while left:
                u, h0 = divmod(g0, hu)
                nh = min(left, hu - h0)
                segs.append(heads[u] + (h0, nh))
                g0 += nh
                left -= nh
            steps.append(segs)
        tasks = [(c, t, pi) for pi in range(PU) for c, t in mac_tasks(pb * PU + pi, range(LT))]
        accs, pend, part, pos = {}, [], [], [0]

        def qk(pi, j, hh, h0, nh):
            p = pb * PU + pi
            h = 2 * p + hh
            wq = sq[pl.ds(h, 1), j * TQ:(j + 1) * TQ]
            qh = [q8[h, :, j * TQ:(j + 1) * TQ], jnp.zeros((64, TQ), I8)]
            s = jnp.dot(k8[p, h0 * G:(h0 + nh) * G, :], jnp.concatenate(qh if hh == 0 else qh[::-1], axis=0),
                        preferred_element_type=I32)
            ws = {}
            for t in range(nh):
                kb = (h0 + t) * G // TB
                if kb not in ws:
                    ws[kb] = wq * jnp.concatenate([sk[kb, pl.ds(h, 1), :]] * (TQ // 128), axis=1)
                e = jnp.exp2(s[t * G:(t + 1) * G].astype(F32) * ws[kb])
                part.extend(e[16 * i:16 * (i + 1)] for i in range(G // 16))
                pos[0] += 1
                if len(part) == 8:
                    pt = jnp.concatenate(part[::-1], axis=0).astype(BF16)
                    pend.append((pos[0], pi, j, hh, (h0 + t) * G // 128, pt))
                    part.clear()

        def pv(_, pi, j, hh, t, pt):
            p = pb * PU + pi
            acc = pv_tile(2 * p + hh, t, pt, accs.get((j, hh)))
            accs[(j, hh)] = acc
            if t == NKT - 1:
                finish(p, hh, accs.pop((j, hh)), slice(j * TQ, (j + 1) * TQ))
            return acc

        n = len(steps)
        wts, issued, tiles = [], 0, -2
        for i in range(n - 1):
            issued += sizes[i]
            nd = (issued - LAG) * G // 128
            wts.append(nd - tiles - (W_FIN if nd // NKT != tiles // NKT else 0.0)
                       - (W_STR if len(steps[i + 1]) > 1 else 0.0))
            tiles = nd
        total = float(sum(t[0] for t in tasks))
        ti, done, cum = 0, 0.0, 0.0
        for i in range(n):
            for seg in steps[i]:
                qk(*seg)
            if i == 0:
                drain(jnp.maximum(pb * PU - 1, 0))
            outs = []
            while pend and (pend[0][0] <= pos[0] - LAG if i < n - 1 else len(pend) > 2):
                outs.append(pv(*pend.pop(0)))
            if i < n - 1:
                for ui in range(2):
                    z = jnp.minimum(jnp.abs(outs[min(ui, len(outs) - 1)][0:8, 0:128]), 0.0)
                    cum += wts[i] / sum(wts) * total / 2
                    caches = {}
                    while ti < len(tasks) and (done + tasks[ti][0] / 2 <= cum or (i == n - 2 and ui == 1)):
                        tasks[ti][1](caches.setdefault(tasks[ti][2], {}), z)
                        done += tasks[ti][0]
                        ti += 1
        for i in range(2):
            pcar[i] = pend[i][5]
        acar[...] = accs.pop((JL, 1))
        return carry

    pcar[...] = jnp.zeros((2, 128, TQ), BF16)
    acar[...] = jnp.ones((24, TQ), F32)

    def attn_fast():
        lax.fori_loop(0, NP // PU, p2, 0)
        drain(NP - 1)

    def attn_general():
        def fb1(i, carry):
            r0 = pl.multiple_of((i // NB) * 160, 32)
            t0 = pl.multiple_of((i % NB) * TB, TB)
            qkt[pl.ds(r0, 160), pl.ds(t0, TB)] = lax.dot_general(
                wt[pl.ds(r0, 160), :], x_v[pl.ds(t0, TB), :], NT, preferred_element_type=F32)
            return carry

        lax.fori_loop(0, 8 * NB, fb1, 0)

        def fb2(p, carry):
            r0 = pl.multiple_of(40 * p, 8)

            def tr(kt, c2):
                c0 = pl.multiple_of(kt * 128, 128)
                blk = jnp.concatenate([qkt[pl.ds(D + r0, 40), pl.ds(c0, 128)], jnp.zeros((88, 128), F32)], axis=0)
                kn[pl.ds(c0, 128), :] = blk.T.astype(BF16)
                return c2

            lax.fori_loop(0, NKT, tr, 0)
            rows = lax.broadcasted_iota(I32, (40, TQ), 0)
            for hh in range(2):
                def qtile(j, c2, hh=hh):
                    c0 = pl.multiple_of(j * TQ, TQ)
                    qm = jnp.where((rows >= DH * hh) & (rows < DH * hh + DH),
                                   qkt[pl.ds(r0, 40), pl.ds(c0, TQ)], 0.0)
                    qm = jnp.concatenate([qm, jnp.zeros((88, TQ), F32)], axis=0).astype(BF16)

                    def kchunk(c, st):
                        m, acc = st
                        k0 = pl.multiple_of(c * 128, 128)
                        s = jnp.dot(kn[pl.ds(k0, 128), :], qm, preferred_element_type=F32) * SCALE2
                        mn = jnp.maximum(m, jnp.max(s, axis=0, keepdims=True))
                        e = jnp.exp2(s - mn).astype(BF16)
                        o = lax.dot_general(vt[2 * p + hh, :, pl.ds(k0, 128)], e, NN, preferred_element_type=F32)
                        return mn, o + acc * jnp.exp2(m - mn)

                    m0 = jnp.full((1, TQ), -jnp.inf, F32)
                    _, acc = lax.fori_loop(0, NKT, kchunk, (m0, jnp.zeros((24, TQ), F32)))
                    finish(p, hh, acc, pl.ds(c0, TQ))
                    return c2

                lax.fori_loop(0, S // TQ, qtile, 0)

            def mac(lt, c2):
                cache = {}
                for _, task in mac_tasks(p, [lt]):
                    task(cache, None)
                return c2

            lax.fori_loop(0, LT, mac, 0)
            return carry

        lax.fori_loop(0, NP, fb2, 0)

    lax.cond(fast, attn_fast, attn_general)

    gw = gw_v[...].astype(F32).reshape(1, D)
    dv = dvec_v[...].astype(F32).reshape(1, D)

    def p4(it, carry):
        off = 0
        for sb, oc in enumerate(OBS):
            c0 = it * sum(OBS) + off
            off += oc
            ob = oc * C
            t0 = pl.multiple_of(c0 * C, C)
            s0 = (sb % 2) * max(OBS) * LT
            yr = jnp.concatenate([ys[:, c0 + i].reshape(128, D) for i in range(oc)], axis=1)
            yi = jnp.concatenate([ys[:, NC + c0 + i].reshape(128, D) for i in range(oc)], axis=1)
            ar, br, ai, bi = yr[0:64], yr[64:128], yi[0:64], yi[64:128]
            ye = jnp.dot(dft_v[256:320, :], jnp.concatenate([ar + br, ai - bi], axis=0).astype(BF16),
                         preferred_element_type=F32)
            yo = jnp.dot(dft_v[320:384, :], jnp.concatenate([ar - br, ai + bi], axis=0).astype(BF16),
                         preferred_element_type=F32)
            for i in range(oc * LT):
                ysc[s0 + i, pl.ds(0, 64, stride=2), :] = ye[:, i * 128:(i + 1) * 128]
                ysc[s0 + i, pl.ds(1, 64, stride=2), :] = yo[:, i * 128:(i + 1) * 128]
            y = jnp.concatenate(
                [jnp.concatenate([ysc[s0 + i * LT + lt] for lt in range(LT)], axis=1) for i in range(oc)], axis=0)
            if oc > 1:
                o = ot[:, :, pl.ds(t0, ob)].reshape(D, ob).astype(BF16).T
            elif "o2" not in memo:
                memo["o2"] = ot[:, :, pl.ds(t0, 2 * C)].reshape(D, 2 * C).astype(BF16).T
                o = memo["o2"][0:C]
            else:
                o = memo.pop("o2")[C:2 * C]
            a = jnp.dot(o, wo_v[...], preferred_element_type=F32)
            xf = x_v[pl.ds(t0, ob), :].astype(F32)
            g = jax.nn.sigmoid(jnp.sum(xf * gw, axis=-1, keepdims=True))
            b = xf * (y + kvb[pl.ds(t0, ob), :].astype(F32) * dv)
            out_v[pl.ds(t0, ob), :] = (b + g * (a - b)).astype(BF16)
            cp_out(c0, oc).start()
        return carry

    lax.fori_loop(0, NC // sum(OBS), p4, 0)
    cp_out(0, NC).wait()


@jax.jit
def pallas_gated_mix__mha_block__ssm_conv_h3__prompt_kernel(A_x, A_wqkv, A_wo, B_q, B_k, B_v, B_shift_k, B_ssm_k, B_ssm_D, gate_w):
    del B_q
    hbm = pl.BlockSpec(memory_space=pl.ANY)
    return pl.pallas_call(
        _kernel,
        out_shape=jax.ShapeDtypeStruct((1, S, D), BF16),
        in_specs=[hbm] * 10,
        out_specs=hbm,
        scratch_shapes=[
            pltpu.VMEM((S, D), BF16),
            pltpu.VMEM((D, 3 * D), BF16),
            pltpu.VMEM((D, D), BF16),
            pltpu.VMEM((S + 16, D), BF16),
            pltpu.VMEM((S, D), BF16),
            pltpu.VMEM((D, S), BF16),
            pltpu.VMEM((S, D), BF16),
            pltpu.VMEM((4, D), BF16),
            pltpu.VMEM((D,), BF16),
            pltpu.VMEM((D,), BF16),
            pltpu.VMEM((384, 128), BF16),
            pltpu.VMEM((3 * D, D), BF16),
            pltpu.VMEM((H, 64, S), I8),
            pltpu.VMEM((NP, S, 128), I8),
            pltpu.VMEM((H, 24, S), F32),
            pltpu.VMEM((H, S), F32),
            pltpu.VMEM((NB, H, 128), F32),
            pltpu.VMEM((2, NB, H, 128), F32),
            pltpu.VMEM((32, S), F32),
            pltpu.VMEM((NP, 40, S), F32),
            pltpu.VMEM((S, D), BF16),
            pltpu.VMEM((16, 2 * NC, 8, D), F32),
            pltpu.VMEM((16, 2 * NC, 8, D), F32),
            pltpu.VMEM((16, 2 * NC, 8, D), F32),
            pltpu.VMEM((2 * max(OBS) * LT, 128, 128), F32),
            pltpu.VMEM((2 * D, S), F32),
            pltpu.VMEM((S, 128), BF16),
            pltpu.VMEM((2, 128, TQ), BF16),
            pltpu.VMEM((24, TQ), F32),
            pltpu.VMEM((3 * D, TB), F32),
            pltpu.SemaphoreType.DMA((10,)),
        ],
        compiler_params=pltpu.CompilerParams(vmem_limit_bytes=120 * 1024 * 1024),
        name="gmix",
    )(A_x, A_wqkv, A_wo, B_k, B_v, B_ssm_k, B_shift_k.T, B_ssm_D, gate_w, jnp.asarray(_dft_tables(), BF16))
```

```python
import numpy as np
import jax
import jax.numpy as jnp
from jax import lax
import jax.experimental.pallas as pl
import jax.experimental.pallas.tpu as pltpu

S, D, H, DH = 2048, 640, 32, 20
NP = H // 2
TB = 512
NB = S // TB
C = 128
NC = S // C
LT = D // 128
NKT = S // 128
TQ = 512
JL = S // TQ - 1
HN = 2
MB = 4
PU = 2
OBS = (2, 2, 2, 2, 2, 2, 2, 1, 1)
G, FIRST, STEP, LAST, LAG = 64, 5, 6, 4, 3
W_FIN, W_STR = 0.4, 0.5
KA = 128

F32, BF16, I32, I16, I8 = jnp.float32, jnp.bfloat16, jnp.int32, jnp.int16, jnp.int8
NT = (((1,), (1,)), ((), ()))
NN = (((1,), (0,)), ((), ()))
QMAX = 2038.0
MAGIC = 12582912.0
MAGIC_BITS = 0x4B400000
SCALE2 = (DH ** -0.5) * 1.4426950408889634
DEQ = 256.0 / (QMAX * QMAX) * SCALE2


def _dft_tables():
    r = np.arange(64, dtype=np.float64)
    f = np.concatenate([2 * r, 127 - 2 * r])
    n = np.arange(128, dtype=np.float64)
    ang = 2.0 * np.pi * (f[:, None] + 0.5) * n[None, :] / 256.0
    fwd = np.concatenate([np.cos(ang), -np.sin(ang)], axis=0)
    inv = np.concatenate([np.cos(ang[:64]).T, -np.sin(ang[:64]).T], axis=1) / 128.0
    inv = np.concatenate([inv[0::2], inv[1::2]], axis=0)
    fwd = fwd.reshape(2, 16, 8, 128).transpose(1, 0, 2, 3).reshape(256, 128)
    return np.concatenate([fwd, inv], axis=0).astype(np.float32)


def _limbs(r, inv):
    t = lax.bitcast_convert_type(r * inv + MAGIC, I32) - (MAGIC_BITS - 8)
    return t >> 4, (t & 15) - 8, (t + 120) >> 8


def _recip(m):
    r = pl.reciprocal(m, approx=True)
    return r * (2.0 - m * r)


def _qscale(m):
    r = pl.reciprocal(m, approx=True)
    return (r * QMAX) * (2.0 - m * r)


def _kernel(x_hbm, wqkv_hbm, wo_hbm, k_hbm, v_hbm, ssm_hbm, shift_hbm, dvec_hbm, gw_hbm, dft_hbm, out_hbm,
            x_v, wqkv_v, wo_v, k_v, v_v, ssm_v, out_v, shift_v, dvec_v, gw_v, dft_v,
            wt, q8, k8, vt, sq, sk, kst, vmx, ot, kvb, us, hs, ys, ysc, kn, pcar, acar, part0, sems):
    qkt = part0
    def cp(src, dst, sem):
        return pltpu.make_async_copy(src, dst, sems.at[sem])

    cp_a1 = [cp(wqkv_hbm.at[0:KA, 0:D], wqkv_v.at[0:KA, 0:D], 0),
             cp(x_hbm.at[0, 0:2 * TB, 0:KA], x_v.at[0:2 * TB, 0:KA], 0)]
    cp_a2 = [cp(wqkv_hbm.at[0:KA, D:3 * D], wqkv_v.at[0:KA, D:3 * D], 1),
             cp(x_hbm.at[0, 2 * TB:S, 0:KA], x_v.at[2 * TB:S, 0:KA], 1)]
    cp_b = cp(wqkv_hbm.at[KA:D, :], wqkv_v.at[KA:D, :], 2)

    def cp_x(i):
        return cp(x_hbm.at[0, pl.ds(i * TB, TB), KA:D], x_v.at[pl.ds(i * TB, TB), KA:D], 3 + i)

    late = [
        cp(ssm_hbm, ssm_v, 7),
        cp(k_hbm.at[0], k_v.at[pl.ds(16, S), :], 7),
        cp(v_hbm.at[0], v_v, 7),
        cp(wo_hbm, wo_v, 7),
        cp(shift_hbm, shift_v, 7),
        cp(dvec_hbm, dvec_v, 7),
        cp(gw_hbm, gw_v, 7),
        cp(dft_hbm, dft_v, 7),
    ]

    def cp_out(r0, n):
        return cp(out_v.at[r0:r0 + n, :], out_hbm.at[0, r0:r0 + n, :], 8)

    for c in cp_a1 + cp_a2 + [cp_b] + [cp_x(i) for i in range(NB)] + late:
        c.start()

    k_v[0:16, :] = jnp.zeros((16, D), BF16)

    low4 = lax.broadcasted_iota(I32, (8, TB), 0) < 4

    def headred(a, op, red):
        mid = a[16:24]
        ma = op(op(a[0:8], a[8:16]), jnp.where(low4, mid, 0.0))
        mb = op(op(a[24:32], a[32:40]), jnp.where(low4, 0.0, mid))
        return red(ma, axis=0, keepdims=True), red(mb, axis=0, keepdims=True)

    def pairscale(ia, ib):
        a8 = jnp.broadcast_to(ia, (8, TB))
        b8 = jnp.broadcast_to(ib, (8, TB))
        return jnp.concatenate([a8, a8, jnp.where(low4, a8, b8), b8, b8], axis=0)

    def slots(l1, l2, l3, mask):
        r2 = pltpu.roll(l2[16:24], 4, 0)
        m3 = l3[16:24]
        a = [l1[0:16], l2[0:16], l3[0:16], jnp.where(low4, l1[16:24], r2), jnp.where(low4, m3, 0) if mask else m3]
        b = [l1[24:40], l2[24:40], l3[24:40], jnp.where(low4, r2, l1[16:24]), jnp.where(low4, 0, m3) if mask else m3]
        return a, b

    def lanefold(a, op):
        return op(op(a[:, 0:128], a[:, 128:256]), op(a[:, 256:384], a[:, 384:512]))

    memo = {}

    def proj(part, g, t0):
        r0 = part * D + 160 * g
        if g % 2 == 0:
            memo["wide"] = lax.dot_general(wt[r0:r0 + 320, KA:D], x_v[pl.ds(t0, TB), KA:D], NT,
                                           preferred_element_type=F32) + part0[r0:r0 + 320, pl.ds(t0, TB)]
        return memo["wide"][160 * (g % 2):160 * (g % 2 + 1)]

    def kgrp(g, tb, t0):
        rk = proj(1, g, t0)
        for j in range(4):
            p = 4 * g + j
            r = rk[40 * j:40 * (j + 1)]
            ab = jnp.abs(r)
            mida, midb = jnp.where(low4, ab[16:24], 0.0), jnp.where(low4, 0.0, ab[16:24])
            ms = []
            for hh, (u0, u1, u2) in enumerate(((ab[0:8], ab[8:16], mida), (ab[24:32], ab[32:40], midb))):
                l1 = u0 + u1 + u2
                l1m = jnp.sum(jnp.max(lanefold(l1, jnp.maximum), axis=1, keepdims=True), axis=0, keepdims=True)
                l1s = jnp.sum(jnp.sum(lanefold(l1, jnp.add), axis=1, keepdims=True), axis=0, keepdims=True)
                kst[0, tb, 2 * p + hh:2 * p + hh + 1, :] = jnp.broadcast_to(l1m, (1, 128))
                kst[1, tb, 2 * p + hh:2 * p + hh + 1, :] = jnp.broadcast_to(l1s, (1, 128))
                m = lanefold(jnp.maximum(jnp.maximum(u0, u1), u2), jnp.maximum)
                m = jnp.max(jnp.max(m, axis=0, keepdims=True), axis=1, keepdims=True)
                ms.append(jnp.maximum(m, 1e-30))
            ma, mb = ms
            hi, lo, top = _limbs(r, pairscale(_qscale(ma), _qscale(mb)))
            sk[tb, 2 * p:2 * p + 1, :] = jnp.broadcast_to(ma, (1, 128))
            sk[tb, 2 * p + 1:2 * p + 2, :] = jnp.broadcast_to(mb, (1, 128))
            ka, kb = slots(hi, lo, top, False)
            kk = jnp.concatenate(ka + kb, axis=0).astype(I16).T
            kk = jnp.concatenate([kk[kt * 128 + 16 * i:kt * 128 + 16 * (i + 1)]
                                  for kt in range(TB // 128) for i in reversed(range(8))], axis=0)
            k8[p, pl.ds(t0, TB), :] = kk.astype(I8)

    def qgrp(g, tb, t0):
        rq = proj(0, g, t0)
        for j in range(4):
            p = 4 * g + j
            r = rq[40 * j:40 * (j + 1)]
            ma, mb = headred(jnp.abs(r), jnp.maximum, jnp.max)
            ma = jnp.maximum(ma, 1e-30)
            mb = jnp.maximum(mb, 1e-30)
            hi, lo, top = _limbs(r, pairscale(_qscale(ma), _qscale(mb)))
            sq[2 * p:2 * p + 1, pl.ds(t0, TB)] = ma * DEQ
            sq[2 * p + 1:2 * p + 2, pl.ds(t0, TB)] = mb * DEQ
            pa, pb = slots(hi, top, lo, True)
            q8[2 * p, :, pl.ds(t0, TB)] = jnp.concatenate(pa, axis=0).astype(I8)
            q8[2 * p + 1, :, pl.ds(t0, TB)] = jnp.concatenate(pb, axis=0).astype(I8)

    def vgrp(g, tb, t0):
        rv = proj(2, g, t0)
        vmx[8 * g:8 * (g + 1), pl.ds(t0, TB)] = jnp.max(jnp.abs(rv).reshape(20, 8, TB), axis=0)
        for j in range(4):
            p = 4 * g + j
            r = rv[40 * j:40 * (j + 1)]
            mid = r[16:24]
            vt[2 * p, :, pl.ds(t0, TB)] = jnp.concatenate([r[0:16], jnp.where(low4, mid, 1.0)], axis=0)
            vt[2 * p + 1, :, pl.ds(t0, TB)] = jnp.concatenate([jnp.where(low4, 1.0, mid), r[24:40]], axis=0)

    grp = {"K": kgrp, "Q": qgrp, "V": vgrp}

    def wtr(rows, tiles):
        for t in tiles:
            wt[t * 128:(t + 1) * 128, rows] = wqkv_v[rows, t * 128:(t + 1) * 128].T

    def pa(part, tb):
        part0[part * D:(part + 1) * D, tb * TB:(tb + 1) * TB] = lax.dot_general(
            wt[part * D:(part + 1) * D, 0:KA], x_v[tb * TB:(tb + 1) * TB, 0:KA], NT, preferred_element_type=F32)

    for c in cp_a1:
        c.wait()
    wtr(slice(0, KA), range(0, LT))
    pa(0, 0)
    pa(0, 1)
    for c in cp_a2:
        c.wait()
    wtr(slice(0, KA), range(LT, 3 * LT))
    jobs = [(0, 2), (0, 3)] + [(part, tb) for part in (1, 2) for tb in range(NB)]
    for job in jobs[:5]:
        pa(*job)
    cp_b.wait()
    wtr(slice(KA, D), range(3 * LT))
    for job in jobs[5:]:
        pa(*job)

    def p1(tb, carry):
        t0 = pl.multiple_of(tb * TB, TB)
        cp_x(tb).wait()
        for ch in "QKV":
            for g in range(4):
                grp[ch](g, tb, t0)
        return carry

    lax.fori_loop(0, NB, p1, 0)

    for c in late:
        c.wait()

    qinf = jnp.max(sq[...], axis=1, keepdims=True) * (SCALE2 / DEQ)
    bad = jnp.where(jnp.max(vmx[...], axis=1, keepdims=True) <= 2.0 ** 50, 0.0, 1.0)
    for tb in range(NB):
        bad = bad + jnp.where(qinf * kst[0, tb] <= 60.0, 0.0, 1.0)
        bad = bad + jnp.where(qinf + kst[0, tb] <= 1e15, 0.0, 1.0)
        bad = bad + jnp.where(sk[tb] * (DH * TB) <= 10.0 * kst[1, tb] + 1e-25, 0.0, 1.0)
    fast = jnp.sum(bad) == 0.0

    def reim(val):
        n = val.shape[1]
        val = val.reshape(16, 16, n)
        return val[:, 0:8], val[:, 8:16]

    sh = shift_v[...].astype(F32)
    hprev = [None] * LT

    def hdft(c0, lt):
        ls = slice(lt * 128, (lt + 1) * 128)
        hb = jnp.concatenate([ssm_v[ls, (c0 + i) * C:(c0 + i + 1) * C] for i in range(HN)], axis=0)
        hr, hi = reim(lax.dot_general(dft_v[0:256, :], hb, NT, preferred_element_type=F32))
        for i in range(HN):
            cr, ci = hr[:, :, i * 128:(i + 1) * 128], hi[:, :, i * 128:(i + 1) * 128]
            if hprev[lt] is None:
                hs[:, c0 + i, :, ls] = cr
                hs[:, NC + c0 + i, :, ls] = ci
            else:
                pr, pi = hprev[lt]
                hs[:, c0 + i, :, ls] = jnp.concatenate([cr[0:8] - pi[0:8], cr[8:] + pi[8:]], axis=0)
                hs[:, NC + c0 + i, :, ls] = jnp.concatenate([ci[0:8] + pr[0:8], ci[8:] - pr[8:]], axis=0)
            hprev[lt] = (cr, ci)

    def udft(c0, lt):
        ls = slice(lt * 128, (lt + 1) * 128)
        r0, n = c0 * C, HN * C
        win = k_v[r0:r0 + n + 16, ls].astype(F32)
        ks = (win[16:] * sh[0:1, ls] + win[15:n + 15] * sh[1:2, ls]
              + win[14:n + 14] * sh[2:3, ls] + win[13:n + 13] * sh[3:4, ls])
        kv = ks * v_v[r0:r0 + n, ls].astype(F32)
        kvb[r0:r0 + n, ls] = kv.astype(BF16)
        kw = jnp.concatenate([kv[i * C:(i + 1) * C] for i in range(HN)], axis=1).astype(BF16)
        ur, ui = reim(jnp.dot(dft_v[0:256, :], kw, preferred_element_type=F32))
        for i in range(HN):
            us[:, c0 + i, :, ls] = ur[:, :, i * 128:(i + 1) * 128]
            us[:, NC + c0 + i, :, ls] = ui[:, :, i * 128:(i + 1) * 128]

    for lt in range(LT):
        for c0 in range(0, NC, HN):
            hdft(c0, lt)
            udft(c0, lt)

    def mac_tasks(ft, lts):
        tasks = []

        def lanes(lt):
            return slice(lt * 128, (lt + 1) * 128) if isinstance(lt, int) else pl.ds(pl.multiple_of(lt * 128, 128), 128)

        for li, lt in enumerate(lts):
            for ab in range(NC // MB):
                st = {"r": [None] * MB, "i": [None] * MB, "id": (len(tasks), li, ab)}
                for cb in range(ab + 1):
                    for m in range(2):
                        for i in range(MB):
                            js = [j for j in range(MB) if (ab - cb) * MB + i - j >= 0]

                            def task(cache, z, lt=lt, ab=ab, m=m, cb=cb, i=i, js=js, st=st):
                                yr, yi = st["r"], st["i"]

                                def ld(ref, name, slot, pin):
                                    key = (st["id"], name, slot)
                                    if key not in cache:
                                        val = ref[ft, slot, :, lanes(lt)]
                                        cache[key] = val + z if (pin and z is not None) else val
                                    return cache[key]

                                for j in js:
                                    hv = ld(hs, "h", m * NC + (ab - cb) * MB + i - j, True)
                                    ta = ld(us, "u", cb * MB + j, False) * hv
                                    tb_ = ld(us, "u", NC + cb * MB + j, False) * hv
                                    if m == 0:
                                        yr[i] = ta if yr[i] is None else yr[i] + ta
                                        yi[i] = tb_ if yi[i] is None else yi[i] + tb_
                                    else:
                                        yr[i] = yr[i] - tb_
                                        yi[i] = yi[i] + ta
                                if cb == ab and m == 1:
                                    ys[ft, ab * MB + i, :, lanes(lt)] = yr[i]
                                    ys[ft, NC + ab * MB + i, :, lanes(lt)] = yi[i]

                            tasks.append((4 * len(js), task))
        return tasks

    def finish(p, hh, acc, cols):
        if hh == 0:
            ot[p, 0:24, cols] = acc * _recip(acc[20:21])
        else:
            b = acc * _recip(acc[0:1])
            ot[p, 20:24, cols] = b[4:8]
            ot[p, 24:40, cols] = b[8:24]

    def pv_tile(h, t, pt, acc):
        o = lax.dot_general(vt[h, :, t * 128:(t + 1) * 128], pt, NN, preferred_element_type=F32)
        return o if acc is None else o + acc

    def drain(p):
        acc = acar[...]
        for i in range(2):
            acc = pv_tile(2 * p + 1, NKT - 2 + i, pcar[i], acc)
        finish(p, 1, acc, slice(JL * TQ, (JL + 1) * TQ))

    def p2(pb, carry):
        heads = [(pi, j, hh) for pi in range(PU) for j in range(S // TQ) for hh in range(2)]
        hu = S // G
        sizes = [FIRST]
        while len(heads) * hu - sum(sizes) - LAST > STEP:
            sizes.append(STEP)
        sizes += [len(heads) * hu - sum(sizes) - LAST, LAST]
        steps, g0 = [], 0
        for left in sizes:
            segs = []
            while left:
                u, h0 = divmod(g0, hu)
                nh = min(left, hu - h0)
                segs.append(heads[u] + (h0, nh))
                g0 += nh
                left -= nh
            steps.append(segs)
        tasks = [(c, t, pi) for pi in range(PU) for c, t in mac_tasks(pb * PU + pi, range(LT))]
        accs, pend, part, pos = {}, [], [], [0]

        def qk(pi, j, hh, h0, nh):
            p = pb * PU + pi
            h = 2 * p + hh
            wq = sq[pl.ds(h, 1), j * TQ:(j + 1) * TQ]
            qh = [q8[h, :, j * TQ:(j + 1) * TQ], jnp.zeros((64, TQ), I8)]
            s = jnp.dot(k8[p, h0 * G:(h0 + nh) * G, :], jnp.concatenate(qh if hh == 0 else qh[::-1], axis=0),
                        preferred_element_type=I32)
            ws = {}
            for t in range(nh):
                kb = (h0 + t) * G // TB
                if kb not in ws:
                    ws[kb] = wq * jnp.concatenate([sk[kb, pl.ds(h, 1), :]] * (TQ // 128), axis=1)
                e = jnp.exp2(s[t * G:(t + 1) * G].astype(F32) * ws[kb])
                part.extend(e[16 * i:16 * (i + 1)] for i in range(G // 16))
                pos[0] += 1
                if len(part) == 8:
                    pt = jnp.concatenate(part[::-1], axis=0).astype(BF16)
                    pend.append((pos[0], pi, j, hh, (h0 + t) * G // 128, pt))
                    part.clear()

        def pv(_, pi, j, hh, t, pt):
            p = pb * PU + pi
            acc = pv_tile(2 * p + hh, t, pt, accs.get((j, hh)))
            accs[(j, hh)] = acc
            if t == NKT - 1:
                finish(p, hh, accs.pop((j, hh)), slice(j * TQ, (j + 1) * TQ))
            return acc

        n = len(steps)
        wts, issued, tiles = [], 0, -2
        for i in range(n - 1):
            issued += sizes[i]
            nd = (issued - LAG) * G // 128
            wts.append(nd - tiles - (W_FIN if nd // NKT != tiles // NKT else 0.0)
                       - (W_STR if len(steps[i + 1]) > 1 else 0.0))
            tiles = nd
        total = float(sum(t[0] for t in tasks))
        ti, done, cum = 0, 0.0, 0.0
        for i in range(n):
            for seg in steps[i]:
                qk(*seg)
            if i == 0:
                drain(jnp.maximum(pb * PU - 1, 0))
            outs = []
            while pend and (pend[0][0] <= pos[0] - LAG if i < n - 1 else len(pend) > 2):
                outs.append(pv(*pend.pop(0)))
            if i < n - 1:
                for ui in range(2):
                    z = jnp.minimum(jnp.abs(outs[min(ui, len(outs) - 1)][0:8, 0:128]), 0.0)
                    cum += wts[i] / sum(wts) * total / 2
                    caches = {}
                    while ti < len(tasks) and (done + tasks[ti][0] / 2 <= cum or (i == n - 2 and ui == 1)):
                        tasks[ti][1](caches.setdefault(tasks[ti][2], {}), z)
                        done += tasks[ti][0]
                        ti += 1
        for i in range(2):
            pcar[i] = pend[i][5]
        acar[...] = accs.pop((JL, 1))
        return carry

    pcar[...] = jnp.zeros((2, 128, TQ), BF16)
    acar[...] = jnp.ones((24, TQ), F32)

    def attn_fast():
        lax.fori_loop(0, NP // PU, p2, 0)

    def attn_general():
        def fb1(i, carry):
            r0 = pl.multiple_of((i // NKT) * 64, 64)
            t0 = pl.multiple_of((i % NKT) * 128, 128)
            qkt[pl.ds(r0, 64), pl.ds(t0, 128)] = lax.dot_general(
                wt[pl.ds(r0, 64), :], x_v[pl.ds(t0, 128), :], NT, preferred_element_type=F32)
            return carry

        lax.fori_loop(0, 2 * D // 64 * NKT, fb1, 0)
        fq = 256

        def fb2(p, carry):
            r0 = pl.multiple_of(40 * p, 8)

            def tr(kt, c2):
                c0 = pl.multiple_of(kt * 128, 128)
                blk = jnp.concatenate([qkt[pl.ds(D + r0, 40), pl.ds(c0, 128)], jnp.zeros((88, 128), F32)], axis=0)
                kn[pl.ds(c0, 128), :] = blk.T.astype(BF16)
                return c2

            lax.fori_loop(0, NKT, tr, 0)
            rows = lax.broadcasted_iota(I32, (40, fq), 0)

            def qtile(i, c2):
                hh = i // (S // fq)
                c0 = pl.multiple_of((i % (S // fq)) * fq, fq)
                qm = jnp.where((rows >= DH * hh) & (rows < DH * hh + DH), qkt[pl.ds(r0, 40), pl.ds(c0, fq)], 0.0)
                qm = jnp.concatenate([qm, jnp.zeros((88, fq), F32)], axis=0).astype(BF16)

                def kchunk(c, st):
                    m, acc = st
                    k0 = pl.multiple_of(c * 128, 128)
                    s = jnp.dot(kn[pl.ds(k0, 128), :], qm, preferred_element_type=F32) * SCALE2
                    mn = jnp.maximum(m, jnp.max(s, axis=0, keepdims=True))
                    e = jnp.exp2(s - mn).astype(BF16)
                    o = lax.dot_general(vt[2 * p + hh, :, pl.ds(k0, 128)], e, NN, preferred_element_type=F32)
                    return mn, o + acc * jnp.exp2(m - mn)

                m0 = jnp.full((1, fq), -jnp.inf, F32)
                _, acc = lax.fori_loop(0, NKT, kchunk, (m0, jnp.zeros((24, fq), F32)))
                lax.cond(hh == 0, lambda: finish(p, 0, acc, pl.ds(c0, fq)), lambda: finish(p, 1, acc, pl.ds(c0, fq)))
                acar[:, pl.ds(pl.multiple_of(c0 % TQ, fq), fq)] = acc
                return c2

            lax.fori_loop(0, 2 * S // fq, qtile, 0)

            def mac(lt, c2):
                cache = {}
                for _, task in mac_tasks(p, [lt]):
                    task(cache, None)
                return c2

            lax.fori_loop(0, LT, mac, 0)
            return carry

        lax.fori_loop(0, NP, fb2, 0)

    lax.cond(fast, attn_fast, attn_general)

    gw = gw_v[...].astype(F32).reshape(1, D)
    dv = dvec_v[...].astype(F32).reshape(1, D)

    drain(NP - 1)
    c0, o2 = 0, None
    for sb, oc in enumerate(OBS):
        ob, t0 = oc * C, c0 * C
        s0 = (sb % 2) * max(OBS) * LT
        yr = jnp.concatenate([ys[:, c0 + i].reshape(128, D) for i in range(oc)], axis=1)
        yi = jnp.concatenate([ys[:, NC + c0 + i].reshape(128, D) for i in range(oc)], axis=1)
        ar, br, ai, bi = yr[0:64], yr[64:128], yi[0:64], yi[64:128]
        ye = jnp.dot(dft_v[256:320, :], jnp.concatenate([ar + br, ai - bi], axis=0).astype(BF16),
                     preferred_element_type=F32)
        yo = jnp.dot(dft_v[320:384, :], jnp.concatenate([ar - br, ai + bi], axis=0).astype(BF16),
                     preferred_element_type=F32)
        for i in range(oc * LT):
            ysc[s0 + i, pl.ds(0, 64, stride=2), :] = ye[:, i * 128:(i + 1) * 128]
            ysc[s0 + i, pl.ds(1, 64, stride=2), :] = yo[:, i * 128:(i + 1) * 128]
        y = jnp.concatenate(
            [jnp.concatenate([ysc[s0 + i * LT + lt] for lt in range(LT)], axis=1) for i in range(oc)], axis=0)
        if oc > 1:
            o = ot[:, :, t0:t0 + ob].reshape(D, ob).astype(BF16).T
        elif o2 is None:
            o2 = ot[:, :, t0:t0 + 2 * C].reshape(D, 2 * C).astype(BF16).T
            o = o2[0:C]
        else:
            o, o2 = o2[C:2 * C], None
        a = jnp.dot(o, wo_v[...], preferred_element_type=F32)
        xf = x_v[t0:t0 + ob, :].astype(F32)
        g = jax.nn.sigmoid(jnp.sum(xf * gw, axis=-1, keepdims=True))
        b = xf * (y + kvb[t0:t0 + ob, :].astype(F32) * dv)
        out_v[t0:t0 + ob, :] = (b + g * (a - b)).astype(BF16)
        cp_out(t0, ob).start()
        c0 += oc
    cp_out(0, S).wait()


@jax.jit
def pallas_gated_mix__mha_block__ssm_conv_h3__prompt_kernel(A_x, A_wqkv, A_wo, B_q, B_k, B_v, B_shift_k, B_ssm_k, B_ssm_D, gate_w):
    del B_q
    hbm = pl.BlockSpec(memory_space=pl.ANY)
    return pl.pallas_call(
        _kernel,
        out_shape=jax.ShapeDtypeStruct((1, S, D), BF16),
        in_specs=[hbm] * 10,
        out_specs=hbm,
        scratch_shapes=[
            pltpu.VMEM((S, D), BF16),
            pltpu.VMEM((D, 3 * D), BF16),
            pltpu.VMEM((D, D), BF16),
            pltpu.VMEM((S + 16, D), BF16),
            pltpu.VMEM((S, D), BF16),
            pltpu.VMEM((D, S), BF16),
            pltpu.VMEM((S, D), BF16),
            pltpu.VMEM((4, D), BF16),
            pltpu.VMEM((D,), BF16),
            pltpu.VMEM((D,), BF16),
            pltpu.VMEM((384, 128), BF16),
            pltpu.VMEM((3 * D, D), BF16),
            pltpu.VMEM((H, 64, S), I8),
            pltpu.VMEM((NP, S, 128), I8),
            pltpu.VMEM((H, 24, S), F32),
            pltpu.VMEM((H, S), F32),
            pltpu.VMEM((NB, H, 128), F32),
            pltpu.VMEM((2, NB, H, 128), F32),
            pltpu.VMEM((32, S), F32),
            pltpu.VMEM((NP, 40, S), F32),
            pltpu.VMEM((S, D), BF16),
            pltpu.VMEM((16, 2 * NC, 8, D), F32),
            pltpu.VMEM((16, 2 * NC, 8, D), F32),
            pltpu.VMEM((16, 2 * NC, 8, D), F32),
            pltpu.VMEM((2 * max(OBS) * LT, 128, 128), F32),
            pltpu.VMEM((S, 128), BF16),
            pltpu.VMEM((2, 128, TQ), BF16),
            pltpu.VMEM((24, TQ), F32),
            pltpu.VMEM((3 * D, S), F32),
            pltpu.SemaphoreType.DMA((9,)),
        ],
        compiler_params=pltpu.CompilerParams(vmem_limit_bytes=120 * 1024 * 1024),
        name="gmix",
    )(A_x, A_wqkv, A_wo, B_k, B_v, B_ssm_k, B_shift_k.T, B_ssm_D, gate_w, jnp.asarray(_dft_tables(), BF16))
```

```python
import numpy as np
import jax
import jax.numpy as jnp
from jax import lax
import jax.experimental.pallas as pl
import jax.experimental.pallas.tpu as pltpu

S, D, H, DH = 2048, 640, 32, 20
NP = H // 2
TB = 512
NB = S // TB
C = 128
NC = S // C
LT = D // 128
NKT = S // 128
TQ = 512
JL = S // TQ - 1
HN = 2
MB = 4
PU = 2
OBS = (2, 2, 2, 2, 2, 2, 2, 1, 1)
G, FIRST, STEP, LAST, LAG = 64, 5, 6, 4, 3
W_FIN, W_STR = 0.4, 0.5
KA = 128

F32, BF16, I32, I16, I8 = jnp.float32, jnp.bfloat16, jnp.int32, jnp.int16, jnp.int8
NT = (((1,), (1,)), ((), ()))
NN = (((1,), (0,)), ((), ()))
QMAX = 2038.0
MAGIC = 12582912.0
MAGIC_BITS = 0x4B400000
SCALE2 = (DH ** -0.5) * 1.4426950408889634
DEQ = 256.0 / (QMAX * QMAX) * SCALE2


def _dft_tables():
    r = np.arange(64, dtype=np.float64)
    f = np.concatenate([2 * r, 127 - 2 * r])
    n = np.arange(128, dtype=np.float64)
    ang = 2.0 * np.pi * (f[:, None] + 0.5) * n[None, :] / 256.0
    fwd = np.concatenate([np.cos(ang), -np.sin(ang)], axis=0)
    inv = np.concatenate([np.cos(ang[:64]).T, -np.sin(ang[:64]).T], axis=1) / 128.0
    inv = np.concatenate([inv[0::2], inv[1::2]], axis=0)
    fwd = fwd.reshape(2, 16, 8, 128).transpose(1, 0, 2, 3).reshape(256, 128)
    return np.concatenate([fwd, inv], axis=0).astype(np.float32)


def _limbs(r, inv):
    t = lax.bitcast_convert_type(r * inv + MAGIC, I32) - (MAGIC_BITS - 8)
    return t >> 4, (t & 15) - 8, (t + 120) >> 8


def _recip(m):
    r = pl.reciprocal(m, approx=True)
    return r * (2.0 - m * r)


def _qscale(m):
    r = pl.reciprocal(m, approx=True)
    return (r * QMAX) * (2.0 - m * r)


def _kernel(x_hbm, wqkv_hbm, wo_hbm, k_hbm, v_hbm, ssm_hbm, shift_hbm, dvec_hbm, gw_hbm, dft_hbm, out_hbm,
            x_v, wqkv_v, wo_v, k_v, v_v, ssm_v, out_v, shift_v, dvec_v, gw_v, dft_v,
            wt, q8, k8, vt, sq, sk, kst, vmx, ot, kvb, us, hs, ys, ysc, kn, pcar, acar, part0, sems):
    qkt = part0
    def cp(src, dst, sem):
        return pltpu.make_async_copy(src, dst, sems.at[sem])

    cp_a1 = [cp(wqkv_hbm.at[0:KA, 0:D], wqkv_v.at[0:KA, 0:D], 0),
             cp(x_hbm.at[0, 0:2 * TB, 0:KA], x_v.at[0:2 * TB, 0:KA], 0)]
    cp_a2 = [cp(wqkv_hbm.at[0:KA, D:3 * D], wqkv_v.at[0:KA, D:3 * D], 1),
             cp(x_hbm.at[0, 2 * TB:S, 0:KA], x_v.at[2 * TB:S, 0:KA], 1)]
    cp_b = cp(wqkv_hbm.at[KA:D, :], wqkv_v.at[KA:D, :], 2)

    def cp_x(i):
        return cp(x_hbm.at[0, pl.ds(i * TB, TB), KA:D], x_v.at[pl.ds(i * TB, TB), KA:D], 3 + i)

    late = [
        cp(ssm_hbm, ssm_v, 7),
        cp(k_hbm.at[0], k_v.at[pl.ds(16, S), :], 7),
        cp(v_hbm.at[0], v_v, 7),
        cp(wo_hbm, wo_v, 7),
        cp(shift_hbm, shift_v, 7),
        cp(dvec_hbm, dvec_v, 7),
        cp(gw_hbm, gw_v, 7),
        cp(dft_hbm, dft_v, 7),
    ]

    def cp_out(r0, n):
        return cp(out_v.at[r0:r0 + n, :], out_hbm.at[0, r0:r0 + n, :], 8)

    for c in cp_a1 + cp_a2 + [cp_b] + [cp_x(i) for i in range(NB)] + late:
        c.start()

    k_v[0:16, :] = jnp.zeros((16, D), BF16)

    low4 = lax.broadcasted_iota(I32, (8, TB), 0) < 4

    def headred(a, op, red):
        mid = a[16:24]
        ma = op(op(a[0:8], a[8:16]), jnp.where(low4, mid, 0.0))
        mb = op(op(a[24:32], a[32:40]), jnp.where(low4, 0.0, mid))
        return red(ma, axis=0, keepdims=True), red(mb, axis=0, keepdims=True)

    def pairscale(ia, ib):
        a8 = jnp.broadcast_to(ia, (8, TB))
        b8 = jnp.broadcast_to(ib, (8, TB))
        return jnp.concatenate([a8, a8, jnp.where(low4, a8, b8), b8, b8], axis=0)

    def slots(l1, l2, l3, mask):
        r2 = pltpu.roll(l2[16:24], 4, 0)
        m3 = l3[16:24]
        a = [l1[0:16], l2[0:16], l3[0:16], jnp.where(low4, l1[16:24], r2), jnp.where(low4, m3, 0) if mask else m3]
        b = [l1[24:40], l2[24:40], l3[24:40], jnp.where(low4, r2, l1[16:24]), jnp.where(low4, 0, m3) if mask else m3]
        return a, b

    def lanefold(a, op):
        return op(op(a[:, 0:128], a[:, 128:256]), op(a[:, 256:384], a[:, 384:512]))

    memo = {}

    def proj(part, g, t0):
        r0 = part * D + 160 * g
        if g % 2 == 0:
            memo["wide"] = lax.dot_general(wt[r0:r0 + 320, KA:D], x_v[pl.ds(t0, TB), KA:D], NT,
                                           preferred_element_type=F32) + part0[r0:r0 + 320, pl.ds(t0, TB)]
        return memo["wide"][160 * (g % 2):160 * (g % 2 + 1)]

    def kgrp(g, tb, t0):
        rk = proj(1, g, t0)
        for j in range(4):
            p = 4 * g + j
            r = rk[40 * j:40 * (j + 1)]
            ab = jnp.abs(r)
            mida, midb = jnp.where(low4, ab[16:24], 0.0), jnp.where(low4, 0.0, ab[16:24])
            ms = []
            for hh, (u0, u1, u2) in enumerate(((ab[0:8], ab[8:16], mida), (ab[24:32], ab[32:40], midb))):
                l1 = u0 + u1 + u2
                l1m = jnp.sum(jnp.max(lanefold(l1, jnp.maximum), axis=1, keepdims=True), axis=0, keepdims=True)
                l1s = jnp.sum(jnp.sum(lanefold(l1, jnp.add), axis=1, keepdims=True), axis=0, keepdims=True)
                kst[0, tb, 2 * p + hh:2 * p + hh + 1, :] = jnp.broadcast_to(l1m, (1, 128))
                kst[1, tb, 2 * p + hh:2 * p + hh + 1, :] = jnp.broadcast_to(l1s, (1, 128))
                m = lanefold(jnp.maximum(jnp.maximum(u0, u1), u2), jnp.maximum)
                m = jnp.max(jnp.max(m, axis=0, keepdims=True), axis=1, keepdims=True)
                ms.append(jnp.maximum(m, 1e-30))
            ma, mb = ms
            hi, lo, top = _limbs(r, pairscale(_qscale(ma), _qscale(mb)))
            sk[tb, 2 * p:2 * p + 1, :] = jnp.broadcast_to(ma, (1, 128))
            sk[tb, 2 * p + 1:2 * p + 2, :] = jnp.broadcast_to(mb, (1, 128))
            ka, kb = slots(hi, lo, top, False)
            kk = jnp.concatenate(ka + kb, axis=0).astype(I16).T
            kk = jnp.concatenate([kk[kt * 128 + 16 * i:kt * 128 + 16 * (i + 1)]
                                  for kt in range(TB // 128) for i in reversed(range(8))], axis=0)
            k8[p, pl.ds(t0, TB), :] = kk.astype(I8)

    def qgrp(g, tb, t0):
        rq = proj(0, g, t0)
        for j in range(4):
            p = 4 * g + j
            r = rq[40 * j:40 * (j + 1)]
            ma, mb = headred(jnp.abs(r), jnp.maximum, jnp.max)
            ma = jnp.maximum(ma, 1e-30)
            mb = jnp.maximum(mb, 1e-30)
            hi, lo, top = _limbs(r, pairscale(_qscale(ma), _qscale(mb)))
            sq[2 * p:2 * p + 1, pl.ds(t0, TB)] = ma * DEQ
            sq[2 * p + 1:2 * p + 2, pl.ds(t0, TB)] = mb * DEQ
            pa, pb = slots(hi, top, lo, True)
            q8[2 * p, :, pl.ds(t0, TB)] = jnp.concatenate(pa, axis=0).astype(I8)
            q8[2 * p + 1, :, pl.ds(t0, TB)] = jnp.concatenate(pb, axis=0).astype(I8)

    def vgrp(g, tb, t0):
        rv = proj(2, g, t0)
        vmx[8 * g:8 * (g + 1), pl.ds(t0, TB)] = jnp.max(jnp.abs(rv).reshape(20, 8, TB), axis=0)
        for j in range(4):
            p = 4 * g + j
            r = rv[40 * j:40 * (j + 1)]
            mid = r[16:24]
            vt[2 * p, :, pl.ds(t0, TB)] = jnp.concatenate([r[0:16], jnp.where(low4, mid, 1.0)], axis=0)
            vt[2 * p + 1, :, pl.ds(t0, TB)] = jnp.concatenate([jnp.where(low4, 1.0, mid), r[24:40]], axis=0)

    grp = {"K": kgrp, "Q": qgrp, "V": vgrp}

    def wtr(rows, tiles):
        for t in tiles:
            wt[t * 128:(t + 1) * 128, rows] = wqkv_v[rows, t * 128:(t + 1) * 128].T

    def pa(part, tb):
        part0[part * D:(part + 1) * D, tb * TB:(tb + 1) * TB] = lax.dot_general(
            wt[part * D:(part + 1) * D, 0:KA], x_v[tb * TB:(tb + 1) * TB, 0:KA], NT, preferred_element_type=F32)

    for c in cp_a1:
        c.wait()
    wtr(slice(0, KA), range(0, LT))
    pa(0, 0)
    pa(0, 1)
    for c in cp_a2:
        c.wait()
    wtr(slice(0, KA), range(LT, 3 * LT))
    jobs = [(0, 2), (0, 3)] + [(part, tb) for part in (1, 2) for tb in range(NB)]
    for job in jobs[:5]:
        pa(*job)
    cp_b.wait()
    wtr(slice(KA, D), range(3 * LT))
    for job in jobs[5:]:
        pa(*job)

    def p1(tb, carry):
        t0 = pl.multiple_of(tb * TB, TB)
        cp_x(tb).wait()
        for ch in "QKV":
            for g in range(4):
                grp[ch](g, tb, t0)
        return carry

    lax.fori_loop(0, NB, p1, 0)

    for c in late:
        c.wait()

    qinf = jnp.max(sq[...], axis=1, keepdims=True) * (SCALE2 / DEQ)
    bad = jnp.where(jnp.max(vmx[...], axis=1, keepdims=True) <= 2.0 ** 50, 0.0, 1.0)
    for tb in range(NB):
        bad = bad + jnp.where(qinf * kst[0, tb] <= 60.0, 0.0, 1.0)
        bad = bad + jnp.where(qinf + kst[0, tb] <= 1e15, 0.0, 1.0)
        bad = bad + jnp.where(sk[tb] * (DH * TB) <= 10.0 * kst[1, tb] + 1e-25, 0.0, 1.0)
    fast = jnp.sum(bad) == 0.0

    def reim(val):
        n = val.shape[1]
        val = val.reshape(16, 16, n)
        return val[:, 0:8], val[:, 8:16]

    sh = shift_v[...].astype(F32)
    hprev = [None] * LT

    def hdft(c0, lt):
        ls = slice(lt * 128, (lt + 1) * 128)
        hb = jnp.concatenate([ssm_v[ls, (c0 + i) * C:(c0 + i + 1) * C] for i in range(HN)], axis=0)
        hr, hi = reim(lax.dot_general(dft_v[0:256, :], hb, NT, preferred_element_type=F32))
        for i in range(HN):
            cr, ci = hr[:, :, i * 128:(i + 1) * 128], hi[:, :, i * 128:(i + 1) * 128]
            if hprev[lt] is None:
                hs[:, c0 + i, :, ls] = cr
                hs[:, NC + c0 + i, :, ls] = ci
            else:
                pr, pi = hprev[lt]
                hs[:, c0 + i, :, ls] = jnp.concatenate([cr[0:8] - pi[0:8], cr[8:] + pi[8:]], axis=0)
                hs[:, NC + c0 + i, :, ls] = jnp.concatenate([ci[0:8] + pr[0:8], ci[8:] - pr[8:]], axis=0)
            hprev[lt] = (cr, ci)

    def udft(c0, lt):
        ls = slice(lt * 128, (lt + 1) * 128)
        r0, n = c0 * C, HN * C
        win = k_v[r0:r0 + n + 16, ls].astype(F32)
        ks = (win[16:] * sh[0:1, ls] + win[15:n + 15] * sh[1:2, ls]
              + win[14:n + 14] * sh[2:3, ls] + win[13:n + 13] * sh[3:4, ls])
        kv = ks * v_v[r0:r0 + n, ls].astype(F32)
        kvb[r0:r0 + n, ls] = kv.astype(BF16)
        kw = jnp.concatenate([kv[i * C:(i + 1) * C] for i in range(HN)], axis=1).astype(BF16)
        ur, ui = reim(jnp.dot(dft_v[0:256, :], kw, preferred_element_type=F32))
        for i in range(HN):
            us[:, c0 + i, :, ls] = ur[:, :, i * 128:(i + 1) * 128]
            us[:, NC + c0 + i, :, ls] = ui[:, :, i * 128:(i + 1) * 128]

    for lt in range(LT):
        for c0 in range(0, NC, HN):
            hdft(c0, lt)
            udft(c0, lt)

    def mac_tasks(ft, lts):
        tasks = []

        def lanes(lt):
            return slice(lt * 128, (lt + 1) * 128) if isinstance(lt, int) else pl.ds(pl.multiple_of(lt * 128, 128), 128)

        for li, lt in enumerate(lts):
            for ab in range(NC // MB):
                st = {"r": [None] * MB, "i": [None] * MB, "id": (len(tasks), li, ab)}
                for cb in range(ab + 1):
                    for m in range(2):
                        for i in range(MB):
                            js = [j for j in range(MB) if (ab - cb) * MB + i - j >= 0]

                            def task(cache, z, lt=lt, ab=ab, m=m, cb=cb, i=i, js=js, st=st):
                                yr, yi = st["r"], st["i"]

                                def ld(ref, name, slot, pin):
                                    key = (st["id"], name, slot)
                                    if key not in cache:
                                        val = ref[ft, slot, :, lanes(lt)]
                                        cache[key] = val + z if (pin and z is not None) else val
                                    return cache[key]

                                for j in js:
                                    hv = ld(hs, "h", m * NC + (ab - cb) * MB + i - j, True)
                                    ta = ld(us, "u", cb * MB + j, False) * hv
                                    tb_ = ld(us, "u", NC + cb * MB + j, False) * hv
                                    if m == 0:
                                        yr[i] = ta if yr[i] is None else yr[i] + ta
                                        yi[i] = tb_ if yi[i] is None else yi[i] + tb_
                                    else:
                                        yr[i] = yr[i] - tb_
                                        yi[i] = yi[i] + ta
                                if cb == ab and m == 1:
                                    ys[ft, ab * MB + i, :, lanes(lt)] = yr[i]
                                    ys[ft, NC + ab * MB + i, :, lanes(lt)] = yi[i]

                            tasks.append((4 * len(js), task))
        return tasks

    def finish(p, hh, acc, cols):
        if hh == 0:
            ot[p, 0:24, cols] = acc * _recip(acc[20:21])
        else:
            b = acc * _recip(acc[0:1])
            ot[p, 20:24, cols] = b[4:8]
            ot[p, 24:40, cols] = b[8:24]

    def pv_tile(h, t, pt, acc):
        o = lax.dot_general(vt[h, :, t * 128:(t + 1) * 128], pt, NN, preferred_element_type=F32)
        return o if acc is None else o + acc

    def drain(p):
        acc = acar[...]
        for i in range(2):
            acc = pv_tile(2 * p + 1, NKT - 2 + i, pcar[i], acc)
        finish(p, 1, acc, slice(JL * TQ, (JL + 1) * TQ))

    def p2(pb, carry):
        heads = [(pi, j, hh) for pi in range(PU) for j in range(S // TQ) for hh in range(2)]
        hu = S // G
        sizes = [FIRST]
        while len(heads) * hu - sum(sizes) - LAST > STEP:
            sizes.append(STEP)
        sizes += [len(heads) * hu - sum(sizes) - LAST, LAST]
        steps, g0 = [], 0
        for left in sizes:
            segs = []
            while left:
                u, h0 = divmod(g0, hu)
                nh = min(left, hu - h0)
                segs.append(heads[u] + (h0, nh))
                g0 += nh
                left -= nh
            steps.append(segs)
        tasks = [(c, t, pi) for pi in range(PU) for c, t in mac_tasks(pb * PU + pi, range(LT))]
        accs, pend, part, pos = {}, [], [], [0]

        def qk(pi, j, hh, h0, nh):
            p = pb * PU + pi
            h = 2 * p + hh
            wq = sq[pl.ds(h, 1), j * TQ:(j + 1) * TQ]
            qh = [q8[h, :, j * TQ:(j + 1) * TQ], jnp.zeros((64, TQ), I8)]
            s = jnp.dot(k8[p, h0 * G:(h0 + nh) * G, :], jnp.concatenate(qh if hh == 0 else qh[::-1], axis=0),
                        preferred_element_type=I32)
            ws = {}
            for t in range(nh):
                kb = (h0 + t) * G // TB
                if kb not in ws:
                    ws[kb] = wq * jnp.concatenate([sk[kb, pl.ds(h, 1), :]] * (TQ // 128), axis=1)
                e = jnp.exp2(s[t * G:(t + 1) * G].astype(F32) * ws[kb])
                part.extend(e[16 * i:16 * (i + 1)] for i in range(G // 16))
                pos[0] += 1
                if len(part) == 8:
                    pt = jnp.concatenate(part[::-1], axis=0).astype(BF16)
                    pend.append((pos[0], pi, j, hh, (h0 + t) * G // 128, pt))
                    part.clear()

        def pv(_, pi, j, hh, t, pt):
            p = pb * PU + pi
            acc = pv_tile(2 * p + hh, t, pt, accs.get((j, hh)))
            accs[(j, hh)] = acc
            if t == NKT - 1:
                finish(p, hh, accs.pop((j, hh)), slice(j * TQ, (j + 1) * TQ))
            return acc

        n = len(steps)
        wts, issued, tiles = [], 0, -2
        for i in range(n - 1):
            issued += sizes[i]
            nd = (issued - LAG) * G // 128
            wts.append(nd - tiles - (W_FIN if nd // NKT != tiles // NKT else 0.0)
                       - (W_STR if len(steps[i + 1]) > 1 else 0.0))
            tiles = nd
        total = float(sum(t[0] for t in tasks))
        ti, done, cum = 0, 0.0, 0.0
        for i in range(n):
            for seg in steps[i]:
                qk(*seg)
            if i == 0:
                drain(jnp.maximum(pb * PU - 1, 0))
            outs = []
            while pend and (pend[0][0] <= pos[0] - LAG if i < n - 1 else len(pend) > 2):
                outs.append(pv(*pend.pop(0)))
            if i < n - 1:
                for ui in range(2):
                    z = jnp.minimum(jnp.abs(outs[min(ui, len(outs) - 1)][0:8, 0:128]), 0.0)
                    cum += wts[i] / sum(wts) * total / 2
                    caches = {}
                    while ti < len(tasks) and (done + tasks[ti][0] / 2 <= cum or (i == n - 2 and ui == 1)):
                        tasks[ti][1](caches.setdefault(tasks[ti][2], {}), z)
                        done += tasks[ti][0]
                        ti += 1
        for i in range(2):
            pcar[i] = pend[i][5]
        acar[...] = accs.pop((JL, 1))
        return carry

    pcar[...] = jnp.zeros((2, 128, TQ), BF16)
    acar[...] = jnp.ones((24, TQ), F32)

    def attn_fast():
        lax.fori_loop(0, NP // PU, p2, 0)

    def attn_general():
        def fb1(i, carry):
            r0 = pl.multiple_of((i // NKT) * 128, 128)
            t0 = pl.multiple_of((i % NKT) * 128, 128)
            qkt[pl.ds(r0, 128), pl.ds(t0, 128)] = lax.dot_general(
                wt[pl.ds(r0, 128), :], x_v[pl.ds(t0, 128), :], NT, preferred_element_type=F32)
            return carry

        lax.fori_loop(0, 2 * LT * NKT, fb1, 0)

        def fb2(p, carry):
            r0 = pl.multiple_of(40 * p, 8)

            def tr(kt, c2):
                c0 = pl.multiple_of(kt * 128, 128)
                blk = jnp.concatenate([qkt[pl.ds(D + r0, 40), pl.ds(c0, 128)], jnp.zeros((88, 128), F32)], axis=0)
                kn[pl.ds(c0, 128), :] = blk.T.astype(BF16)
                return c2

            lax.fori_loop(0, NKT, tr, 0)
            rows = lax.broadcasted_iota(I32, (40, TQ), 0)

            def qtile(i, c2):
                hh = i // (S // TQ)
                c0 = pl.multiple_of((i % (S // TQ)) * TQ, TQ)
                qm = jnp.where((rows >= DH * hh) & (rows < DH * hh + DH), qkt[pl.ds(r0, 40), pl.ds(c0, TQ)], 0.0)
                qm = jnp.concatenate([qm, jnp.zeros((88, TQ), F32)], axis=0).astype(BF16)

                def kchunk(c, st):
                    m, acc = st
                    k0 = pl.multiple_of(c * 128, 128)
                    s = jnp.dot(kn[pl.ds(k0, 128), :], qm, preferred_element_type=F32) * SCALE2
                    mn = jnp.maximum(m, jnp.max(s, axis=0, keepdims=True))
                    e = jnp.exp2(s - mn).astype(BF16)
                    o = lax.dot_general(vt[2 * p + hh, :, pl.ds(k0, 128)], e, NN, preferred_element_type=F32)
                    return mn, o + acc * jnp.exp2(m - mn)

                m0 = jnp.full((1, TQ), -jnp.inf, F32)
                _, acc = lax.fori_loop(0, NKT, kchunk, (m0, jnp.zeros((24, TQ), F32)))
                lax.cond(hh == 0, lambda: finish(p, 0, acc, pl.ds(c0, TQ)), lambda: finish(p, 1, acc, pl.ds(c0, TQ)))
                acar[...] = acc
                return c2

            lax.fori_loop(0, 2 * S // TQ, qtile, 0)

            def mac(lt, c2):
                cache = {}
                for _, task in mac_tasks(p, [lt]):
                    task(cache, None)
                return c2

            lax.fori_loop(0, LT, mac, 0)
            return carry

        lax.fori_loop(0, NP, fb2, 0)

    lax.cond(fast, attn_fast, attn_general)

    gw = gw_v[...].astype(F32).reshape(1, D)
    dv = dvec_v[...].astype(F32).reshape(1, D)

    drain(NP - 1)
    c0, o2 = 0, None
    for sb, oc in enumerate(OBS):
        ob, t0 = oc * C, c0 * C
        s0 = (sb % 2) * max(OBS) * LT
        yr = jnp.concatenate([ys[:, c0 + i].reshape(128, D) for i in range(oc)], axis=1)
        yi = jnp.concatenate([ys[:, NC + c0 + i].reshape(128, D) for i in range(oc)], axis=1)
        ar, br, ai, bi = yr[0:64], yr[64:128], yi[0:64], yi[64:128]
        ye = jnp.dot(dft_v[256:320, :], jnp.concatenate([ar + br, ai - bi], axis=0).astype(BF16),
                     preferred_element_type=F32)
        yo = jnp.dot(dft_v[320:384, :], jnp.concatenate([ar - br, ai + bi], axis=0).astype(BF16),
                     preferred_element_type=F32)
        for i in range(oc * LT):
            ysc[s0 + i, pl.ds(0, 64, stride=2), :] = ye[:, i * 128:(i + 1) * 128]
            ysc[s0 + i, pl.ds(1, 64, stride=2), :] = yo[:, i * 128:(i + 1) * 128]
        y = jnp.concatenate(
            [jnp.concatenate([ysc[s0 + i * LT + lt] for lt in range(LT)], axis=1) for i in range(oc)], axis=0)
        if oc > 1:
            o = ot[:, :, t0:t0 + ob].reshape(D, ob).astype(BF16).T
        elif o2 is None:
            o2 = ot[:, :, t0:t0 + 2 * C].reshape(D, 2 * C).astype(BF16).T
            o = o2[0:C]
        else:
            o, o2 = o2[C:2 * C], None
        a = jnp.dot(o, wo_v[...], preferred_element_type=F32)
        xf = x_v[t0:t0 + ob, :].astype(F32)
        g = jax.nn.sigmoid(jnp.sum(xf * gw, axis=-1, keepdims=True))
        b = xf * (y + kvb[t0:t0 + ob, :].astype(F32) * dv)
        out_v[t0:t0 + ob, :] = (b + g * (a - b)).astype(BF16)
        cp_out(t0, ob).start()
        c0 += oc
    cp_out(0, S).wait()


@jax.jit
def pallas_gated_mix__mha_block__ssm_conv_h3__prompt_kernel(A_x, A_wqkv, A_wo, B_q, B_k, B_v, B_shift_k, B_ssm_k, B_ssm_D, gate_w):
    del B_q
    hbm = pl.BlockSpec(memory_space=pl.ANY)
    return pl.pallas_call(
        _kernel,
        out_shape=jax.ShapeDtypeStruct((1, S, D), BF16),
        in_specs=[hbm] * 10,
        out_specs=hbm,
        scratch_shapes=[
            pltpu.VMEM((S, D), BF16),
            pltpu.VMEM((D, 3 * D), BF16),
            pltpu.VMEM((D, D), BF16),
            pltpu.VMEM((S + 16, D), BF16),
            pltpu.VMEM((S, D), BF16),
            pltpu.VMEM((D, S), BF16),
            pltpu.VMEM((S, D), BF16),
            pltpu.VMEM((4, D), BF16),
            pltpu.VMEM((D,), BF16),
            pltpu.VMEM((D,), BF16),
            pltpu.VMEM((384, 128), BF16),
            pltpu.VMEM((3 * D, D), BF16),
            pltpu.VMEM((H, 64, S), I8),
            pltpu.VMEM((NP, S, 128), I8),
            pltpu.VMEM((H, 24, S), F32),
            pltpu.VMEM((H, S), F32),
            pltpu.VMEM((NB, H, 128), F32),
            pltpu.VMEM((2, NB, H, 128), F32),
            pltpu.VMEM((32, S), F32),
            pltpu.VMEM((NP, 40, S), F32),
            pltpu.VMEM((S, D), BF16),
            pltpu.VMEM((16, 2 * NC, 8, D), F32),
            pltpu.VMEM((16, 2 * NC, 8, D), F32),
            pltpu.VMEM((16, 2 * NC, 8, D), F32),
            pltpu.VMEM((2 * max(OBS) * LT, 128, 128), F32),
            pltpu.VMEM((S, 128), BF16),
            pltpu.VMEM((2, 128, TQ), BF16),
            pltpu.VMEM((24, TQ), F32),
            pltpu.VMEM((3 * D, S), F32),
            pltpu.SemaphoreType.DMA((9,)),
        ],
        compiler_params=pltpu.CompilerParams(vmem_limit_bytes=120 * 1024 * 1024),
        name="gmix",
    )(A_x, A_wqkv, A_wo, B_k, B_v, B_ssm_k, B_shift_k.T, B_ssm_D, gate_w, jnp.asarray(_dft_tables(), BF16))
```

```python
import numpy as np
import jax
import jax.numpy as jnp
from jax import lax
import jax.experimental.pallas as pl
import jax.experimental.pallas.tpu as pltpu

S, D, H, DH = 2048, 640, 32, 20
NP = H // 2
TB = 512
NB = S // TB
C = 128
NC = S // C
LT = D // 128
NKT = S // 128
TQ = 512
JL = S // TQ - 1
HN = 2
MB = 4
PU = 2
OBS = (2, 2, 2, 2, 2, 2, 2, 1, 1)
G, FIRST, STEP, LAST, LAG = 64, 5, 6, 4, 3
W_FIN, W_STR = 0.4, 0.5
KA = 128

F32, BF16, I32, I16, I8 = jnp.float32, jnp.bfloat16, jnp.int32, jnp.int16, jnp.int8
NT = (((1,), (1,)), ((), ()))
NN = (((1,), (0,)), ((), ()))
QMAX = 2038.0
MAGIC = 12582912.0
MAGIC_BITS = 0x4B400000
SCALE2 = (DH ** -0.5) * 1.4426950408889634
DEQ = 256.0 / (QMAX * QMAX) * SCALE2


def _dft_tables():
    r = np.arange(64, dtype=np.float64)
    f = np.concatenate([2 * r, 127 - 2 * r])
    n = np.arange(128, dtype=np.float64)
    ang = 2.0 * np.pi * (f[:, None] + 0.5) * n[None, :] / 256.0
    fwd = np.concatenate([np.cos(ang), -np.sin(ang)], axis=0)
    inv = np.concatenate([np.cos(ang[:64]).T, -np.sin(ang[:64]).T], axis=1) / 128.0
    inv = np.concatenate([inv[0::2], inv[1::2]], axis=0)
    fwd = fwd.reshape(2, 16, 8, 128).transpose(1, 0, 2, 3).reshape(256, 128)
    return np.concatenate([fwd, inv], axis=0).astype(np.float32)


def _limbs(r, inv):
    t = lax.bitcast_convert_type(r * inv + MAGIC, I32) - (MAGIC_BITS - 8)
    return t >> 4, (t & 15) - 8, (t + 120) >> 8


def _recip(m):
    r = pl.reciprocal(m, approx=True)
    return r * (2.0 - m * r)


def _qscale(m):
    r = pl.reciprocal(m, approx=True)
    return (r * QMAX) * (2.0 - m * r)


def _kernel(x_hbm, wqkv_hbm, wo_hbm, k_hbm, v_hbm, ssm_hbm, shift_hbm, dvec_hbm, gw_hbm, dft_hbm, out_hbm,
            x_v, wqkv_v, wo_v, k_v, v_v, ssm_v, out_v, shift_v, dvec_v, gw_v, dft_v,
            wt, q8, k8, vt, sq, sk, kst, vmx, ot, kvb, us, hs, ys, ysc, kn, pcar, acar, part0, sems):
    qkt = part0
    def cp(src, dst, sem):
        return pltpu.make_async_copy(src, dst, sems.at[sem])

    cp_a1 = [cp(wqkv_hbm.at[0:KA, 0:D], wqkv_v.at[0:KA, 0:D], 0),
             cp(x_hbm.at[0, 0:2 * TB, 0:KA], x_v.at[0:2 * TB, 0:KA], 0)]
    cp_a2 = [cp(wqkv_hbm.at[0:KA, D:3 * D], wqkv_v.at[0:KA, D:3 * D], 1),
             cp(x_hbm.at[0, 2 * TB:S, 0:KA], x_v.at[2 * TB:S, 0:KA], 1)]
    cp_b = cp(wqkv_hbm.at[KA:D, :], wqkv_v.at[KA:D, :], 2)

    def cp_x(i):
        return cp(x_hbm.at[0, pl.ds(i * TB, TB), KA:D], x_v.at[pl.ds(i * TB, TB), KA:D], 3 + i)

    late = [
        cp(ssm_hbm, ssm_v, 7),
        cp(k_hbm.at[0], k_v.at[pl.ds(16, S), :], 7),
        cp(v_hbm.at[0], v_v, 7),
        cp(wo_hbm, wo_v, 7),
        cp(shift_hbm, shift_v, 7),
        cp(dvec_hbm, dvec_v, 7),
        cp(gw_hbm, gw_v, 7),
        cp(dft_hbm, dft_v, 7),
    ]

    def cp_out(r0, n):
        return cp(out_v.at[r0:r0 + n, :], out_hbm.at[0, r0:r0 + n, :], 8)

    for c in cp_a1 + cp_a2 + [cp_b] + [cp_x(i) for i in range(NB)] + late:
        c.start()

    k_v[0:16, :] = jnp.zeros((16, D), BF16)

    low4 = lax.broadcasted_iota(I32, (8, TB), 0) < 4

    def headred(a, op, red):
        mid = a[16:24]
        ma = op(op(a[0:8], a[8:16]), jnp.where(low4, mid, 0.0))
        mb = op(op(a[24:32], a[32:40]), jnp.where(low4, 0.0, mid))
        return red(ma, axis=0, keepdims=True), red(mb, axis=0, keepdims=True)

    def pairscale(ia, ib):
        a8 = jnp.broadcast_to(ia, (8, TB))
        b8 = jnp.broadcast_to(ib, (8, TB))
        return jnp.concatenate([a8, a8, jnp.where(low4, a8, b8), b8, b8], axis=0)

    def slots(l1, l2, l3, mask):
        r2 = pltpu.roll(l2[16:24], 4, 0)
        m3 = l3[16:24]
        a = [l1[0:16], l2[0:16], l3[0:16], jnp.where(low4, l1[16:24], r2), jnp.where(low4, m3, 0) if mask else m3]
        b = [l1[24:40], l2[24:40], l3[24:40], jnp.where(low4, r2, l1[16:24]), jnp.where(low4, 0, m3) if mask else m3]
        return a, b

    def lanefold(a, op):
        return op(op(a[:, 0:128], a[:, 128:256]), op(a[:, 256:384], a[:, 384:512]))

    memo = {}

    def proj(part, g, t0):
        r0 = part * D + 160 * g
        if g % 2 == 0:
            memo["wide"] = lax.dot_general(wt[r0:r0 + 320, KA:D], x_v[pl.ds(t0, TB), KA:D], NT,
                                           preferred_element_type=F32) + part0[r0:r0 + 320, pl.ds(t0, TB)]
        return memo["wide"][160 * (g % 2):160 * (g % 2 + 1)]

    def kgrp(g, tb, t0):
        rk = proj(1, g, t0)
        for j in range(4):
            p = 4 * g + j
            r = rk[40 * j:40 * (j + 1)]
            ab = jnp.abs(r)
            mida, midb = jnp.where(low4, ab[16:24], 0.0), jnp.where(low4, 0.0, ab[16:24])
            ms = []
            for hh, (u0, u1, u2) in enumerate(((ab[0:8], ab[8:16], mida), (ab[24:32], ab[32:40], midb))):
                l1 = u0 + u1 + u2
                l1m = jnp.sum(jnp.max(lanefold(l1, jnp.maximum), axis=1, keepdims=True), axis=0, keepdims=True)
                l1s = jnp.sum(jnp.sum(lanefold(l1, jnp.add), axis=1, keepdims=True), axis=0, keepdims=True)
                kst[0, tb, 2 * p + hh:2 * p + hh + 1, :] = jnp.broadcast_to(l1m, (1, 128))
                kst[1, tb, 2 * p + hh:2 * p + hh + 1, :] = jnp.broadcast_to(l1s, (1, 128))
                m = lanefold(jnp.maximum(jnp.maximum(u0, u1), u2), jnp.maximum)
                m = jnp.max(jnp.max(m, axis=0, keepdims=True), axis=1, keepdims=True)
                ms.append(jnp.maximum(m, 1e-30))
            ma, mb = ms
            hi, lo, top = _limbs(r, pairscale(_qscale(ma), _qscale(mb)))
            sk[tb, 2 * p:2 * p + 1, :] = jnp.broadcast_to(ma, (1, 128))
            sk[tb, 2 * p + 1:2 * p + 2, :] = jnp.broadcast_to(mb, (1, 128))
            ka, kb = slots(hi, lo, top, False)
            kk = jnp.concatenate(ka + kb, axis=0).astype(I16).T
            kk = jnp.concatenate([kk[kt * 128 + 16 * i:kt * 128 + 16 * (i + 1)]
                                  for kt in range(TB // 128) for i in reversed(range(8))], axis=0)
            k8[p, pl.ds(t0, TB), :] = kk.astype(I8)

    def qgrp(g, tb, t0):
        rq = proj(0, g, t0)
        for j in range(4):
            p = 4 * g + j
            r = rq[40 * j:40 * (j + 1)]
            ma, mb = headred(jnp.abs(r), jnp.maximum, jnp.max)
            ma = jnp.maximum(ma, 1e-30)
            mb = jnp.maximum(mb, 1e-30)
            hi, lo, top = _limbs(r, pairscale(_qscale(ma), _qscale(mb)))
            sq[2 * p:2 * p + 1, pl.ds(t0, TB)] = ma * DEQ
            sq[2 * p + 1:2 * p + 2, pl.ds(t0, TB)] = mb * DEQ
            pa, pb = slots(hi, top, lo, True)
            q8[2 * p, :, pl.ds(t0, TB)] = jnp.concatenate(pa, axis=0).astype(I8)
            q8[2 * p + 1, :, pl.ds(t0, TB)] = jnp.concatenate(pb, axis=0).astype(I8)

    def vgrp(g, tb, t0):
        rv = proj(2, g, t0)
        vmx[8 * g:8 * (g + 1), pl.ds(t0, TB)] = jnp.max(jnp.abs(rv).reshape(20, 8, TB), axis=0)
        for j in range(4):
            p = 4 * g + j
            r = rv[40 * j:40 * (j + 1)]
            mid = r[16:24]
            vt[2 * p, :, pl.ds(t0, TB)] = jnp.concatenate([r[0:16], jnp.where(low4, mid, 1.0)], axis=0)
            vt[2 * p + 1, :, pl.ds(t0, TB)] = jnp.concatenate([jnp.where(low4, 1.0, mid), r[24:40]], axis=0)

    grp = {"K": kgrp, "Q": qgrp, "V": vgrp}

    def wtr(rows, tiles):
        for t in tiles:
            wt[t * 128:(t + 1) * 128, rows] = wqkv_v[rows, t * 128:(t + 1) * 128].T

    def pa(part, tb):
        part0[part * D:(part + 1) * D, tb * TB:(tb + 1) * TB] = lax.dot_general(
            wt[part * D:(part + 1) * D, 0:KA], x_v[tb * TB:(tb + 1) * TB, 0:KA], NT, preferred_element_type=F32)

    for c in cp_a1:
        c.wait()
    wtr(slice(0, KA), range(0, LT))
    pa(0, 0)
    pa(0, 1)
    for c in cp_a2:
        c.wait()
    wtr(slice(0, KA), range(LT, 3 * LT))
    jobs = [(0, 2), (0, 3)] + [(part, tb) for part in (1, 2) for tb in range(NB)]
    for job in jobs[:5]:
        pa(*job)
    cp_b.wait()
    wtr(slice(KA, D), range(3 * LT))
    for job in jobs[5:]:
        pa(*job)

    def p1(tb, carry):
        t0 = pl.multiple_of(tb * TB, TB)
        cp_x(tb).wait()
        for ch in "QKV":
            for g in range(4):
                grp[ch](g, tb, t0)
        return carry

    lax.fori_loop(0, NB, p1, 0)

    for c in late:
        c.wait()

    qinf = jnp.max(sq[...], axis=1, keepdims=True) * (SCALE2 / DEQ)
    bad = jnp.where(jnp.max(vmx[...], axis=1, keepdims=True) <= 2.0 ** 50, 0.0, 1.0)
    for tb in range(NB):
        bad = bad + jnp.where(qinf * kst[0, tb] <= 60.0, 0.0, 1.0)
        bad = bad + jnp.where(qinf + kst[0, tb] <= 1e15, 0.0, 1.0)
        bad = bad + jnp.where(sk[tb] * (DH * TB) <= 10.0 * kst[1, tb] + 1e-25, 0.0, 1.0)
    fast = jnp.sum(bad) == 0.0

    def reim(val):
        n = val.shape[1]
        val = val.reshape(16, 16, n)
        return val[:, 0:8], val[:, 8:16]

    sh = shift_v[...].astype(F32)
    hprev = [None] * LT

    def hdft(c0, lt):
        ls = slice(lt * 128, (lt + 1) * 128)
        hb = jnp.concatenate([ssm_v[ls, (c0 + i) * C:(c0 + i + 1) * C] for i in range(HN)], axis=0)
        hr, hi = reim(lax.dot_general(dft_v[0:256, :], hb, NT, preferred_element_type=F32))
        for i in range(HN):
            cr, ci = hr[:, :, i * 128:(i + 1) * 128], hi[:, :, i * 128:(i + 1) * 128]
            if hprev[lt] is None:
                hs[:, c0 + i, :, ls] = cr
                hs[:, NC + c0 + i, :, ls] = ci
            else:
                pr, pi = hprev[lt]
                hs[:, c0 + i, :, ls] = jnp.concatenate([cr[0:8] - pi[0:8], cr[8:] + pi[8:]], axis=0)
                hs[:, NC + c0 + i, :, ls] = jnp.concatenate([ci[0:8] + pr[0:8], ci[8:] - pr[8:]], axis=0)
            hprev[lt] = (cr, ci)

    def udft(c0, lt):
        ls = slice(lt * 128, (lt + 1) * 128)
        r0, n = c0 * C, HN * C
        win = k_v[r0:r0 + n + 16, ls].astype(F32)
        ks = (win[16:] * sh[0:1, ls] + win[15:n + 15] * sh[1:2, ls]
              + win[14:n + 14] * sh[2:3, ls] + win[13:n + 13] * sh[3:4, ls])
        kv = ks * v_v[r0:r0 + n, ls].astype(F32)
        kvb[r0:r0 + n, ls] = kv.astype(BF16)
        kw = jnp.concatenate([kv[i * C:(i + 1) * C] for i in range(HN)], axis=1).astype(BF16)
        ur, ui = reim(jnp.dot(dft_v[0:256, :], kw, preferred_element_type=F32))
        for i in range(HN):
            us[:, c0 + i, :, ls] = ur[:, :, i * 128:(i + 1) * 128]
            us[:, NC + c0 + i, :, ls] = ui[:, :, i * 128:(i + 1) * 128]

    for lt in range(LT):
        for c0 in range(0, NC, HN):
            hdft(c0, lt)
            udft(c0, lt)

    def mac_tasks(ft, lts):
        tasks = []

        def lanes(lt):
            return slice(lt * 128, (lt + 1) * 128) if isinstance(lt, int) else pl.ds(pl.multiple_of(lt * 128, 128), 128)

        for li, lt in enumerate(lts):
            for ab in range(NC // MB):
                st = {"r": [None] * MB, "i": [None] * MB, "id": (len(tasks), li, ab)}
                for cb in range(ab + 1):
                    for m in range(2):
                        for i in range(MB):
                            js = [j for j in range(MB) if (ab - cb) * MB + i - j >= 0]

                            def task(cache, z, lt=lt, ab=ab, m=m, cb=cb, i=i, js=js, st=st):
                                yr, yi = st["r"], st["i"]

                                def ld(ref, name, slot, pin):
                                    key = (st["id"], name, slot)
                                    if key not in cache:
                                        val = ref[ft, slot, :, lanes(lt)]
                                        cache[key] = val + z if (pin and z is not None) else val
                                    return cache[key]

                                for j in js:
                                    hv = ld(hs, "h", m * NC + (ab - cb) * MB + i - j, True)
                                    ta = ld(us, "u", cb * MB + j, False) * hv
                                    tb_ = ld(us, "u", NC + cb * MB + j, False) * hv
                                    if m == 0:
                                        yr[i] = ta if yr[i] is None else yr[i] + ta
                                        yi[i] = tb_ if yi[i] is None else yi[i] + tb_
                                    else:
                                        yr[i] = yr[i] - tb_
                                        yi[i] = yi[i] + ta
                                if cb == ab and m == 1:
                                    ys[ft, ab * MB + i, :, lanes(lt)] = yr[i]
                                    ys[ft, NC + ab * MB + i, :, lanes(lt)] = yi[i]

                            tasks.append((4 * len(js), task))
        return tasks

    def finish(p, hh, acc, cols):
        if hh == 0:
            ot[p, 0:24, cols] = acc * _recip(acc[20:21])
        else:
            b = acc * _recip(acc[0:1])
            ot[p, 20:24, cols] = b[4:8]
            ot[p, 24:40, cols] = b[8:24]

    def pv_tile(h, t, pt, acc):
        o = lax.dot_general(vt[h, :, t * 128:(t + 1) * 128], pt, NN, preferred_element_type=F32)
        return o if acc is None else o + acc

    def drain(p):
        acc = acar[...]
        for i in range(2):
            acc = pv_tile(2 * p + 1, NKT - 2 + i, pcar[i], acc)
        finish(p, 1, acc, slice(JL * TQ, (JL + 1) * TQ))

    def p2(pb, carry):
        heads = [(pi, j, hh) for pi in range(PU) for j in range(S // TQ) for hh in range(2)]
        hu = S // G
        sizes = [FIRST]
        while len(heads) * hu - sum(sizes) - LAST > STEP:
            sizes.append(STEP)
        sizes += [len(heads) * hu - sum(sizes) - LAST, LAST]
        steps, g0 = [], 0
        for left in sizes:
            segs = []
            while left:
                u, h0 = divmod(g0, hu)
                nh = min(left, hu - h0)
                segs.append(heads[u] + (h0, nh))
                g0 += nh
                left -= nh
            steps.append(segs)
        tasks = [(c, t, pi) for pi in range(PU) for c, t in mac_tasks(pb * PU + pi, range(LT))]
        accs, pend, part, pos = {}, [], [], [0]

        def qk(pi, j, hh, h0, nh):
            p = pb * PU + pi
            h = 2 * p + hh
            wq = sq[pl.ds(h, 1), j * TQ:(j + 1) * TQ]
            qh = [q8[h, :, j * TQ:(j + 1) * TQ], jnp.zeros((64, TQ), I8)]
            s = jnp.dot(k8[p, h0 * G:(h0 + nh) * G, :], jnp.concatenate(qh if hh == 0 else qh[::-1], axis=0),
                        preferred_element_type=I32)
            ws = {}
            for t in range(nh):
                kb = (h0 + t) * G // TB
                if kb not in ws:
                    ws[kb] = wq * jnp.concatenate([sk[kb, pl.ds(h, 1), :]] * (TQ // 128), axis=1)
                e = jnp.exp2(s[t * G:(t + 1) * G].astype(F32) * ws[kb])
                part.extend(e[16 * i:16 * (i + 1)] for i in range(G // 16))
                pos[0] += 1
                if len(part) == 8:
                    pt = jnp.concatenate(part[::-1], axis=0).astype(BF16)
                    pend.append((pos[0], pi, j, hh, (h0 + t) * G // 128, pt))
                    part.clear()

        def pv(_, pi, j, hh, t, pt):
            p = pb * PU + pi
            acc = pv_tile(2 * p + hh, t, pt, accs.get((j, hh)))
            accs[(j, hh)] = acc
            if t == NKT - 1:
                finish(p, hh, accs.pop((j, hh)), slice(j * TQ, (j + 1) * TQ))
            return acc

        n = len(steps)
        wts, issued, tiles = [], 0, -2
        for i in range(n - 1):
            issued += sizes[i]
            nd = (issued - LAG) * G // 128
            wts.append(nd - tiles - (W_FIN if nd // NKT != tiles // NKT else 0.0)
                       - (W_STR if len(steps[i + 1]) > 1 else 0.0))
            tiles = nd
        total = float(sum(t[0] for t in tasks))
        ti, done, cum = 0, 0.0, 0.0
        for i in range(n):
            for seg in steps[i]:
                qk(*seg)
            if i == 0:
                drain(jnp.maximum(pb * PU - 1, 0))
            outs = []
            while pend and (pend[0][0] <= pos[0] - LAG if i < n - 1 else len(pend) > 2):
                outs.append(pv(*pend.pop(0)))
            if i < n - 1:
                for ui in range(2):
                    z = jnp.minimum(jnp.abs(outs[min(ui, len(outs) - 1)][0:8, 0:128]), 0.0)
                    cum += wts[i] / sum(wts) * total / 2
                    caches = {}
                    while ti < len(tasks) and (done + tasks[ti][0] / 2 <= cum or (i == n - 2 and ui == 1)):
                        tasks[ti][1](caches.setdefault(tasks[ti][2], {}), z)
                        done += tasks[ti][0]
                        ti += 1
        for i in range(2):
            pcar[i] = pend[i][5]
        acar[...] = accs.pop((JL, 1))
        return carry

    pcar[...] = jnp.zeros((2, 128, TQ), BF16)
    acar[...] = jnp.ones((24, TQ), F32)

    def attn_fast():
        lax.fori_loop(0, NP // PU, p2, 0)

    def attn_general():
        def fb1(i, carry):
            r0 = pl.multiple_of((i // NKT) * 128, 128)
            t0 = pl.multiple_of((i % NKT) * 128, 128)
            qkt[pl.ds(r0, 128), pl.ds(t0, 128)] = lax.dot_general(
                wt[pl.ds(r0, 128), :], x_v[pl.ds(t0, 128), :], NT, preferred_element_type=F32)
            return carry

        lax.fori_loop(0, 2 * LT * NKT, fb1, 0)

        def fb2(p, carry):
            r0 = pl.multiple_of(40 * p, 8)

            def tr(kt, c2):
                c0 = pl.multiple_of(kt * 128, 128)
                blk = jnp.concatenate([qkt[pl.ds(D + r0, 40), pl.ds(c0, 128)], jnp.zeros((88, 128), F32)], axis=0)
                kn[pl.ds(c0, 128), :] = blk.T.astype(BF16)
                return c2

            lax.fori_loop(0, NKT, tr, 0)
            rows = lax.broadcasted_iota(I32, (40, TQ), 0)

            def qtile(i, c2):
                hh = i // (S // TQ)
                c0 = pl.multiple_of((i % (S // TQ)) * TQ, TQ)
                qm = jnp.where((rows >= DH * hh) & (rows < DH * hh + DH), qkt[pl.ds(r0, 40), pl.ds(c0, TQ)], 0.0)
                qm = jnp.concatenate([qm, jnp.zeros((88, TQ), F32)], axis=0).astype(BF16)

                def kchunk(c, st):
                    m, acc = st
                    k0 = pl.multiple_of(c * 128, 128)
                    s = jnp.dot(kn[pl.ds(k0, 128), :], qm, preferred_element_type=F32) * SCALE2
                    mn = jnp.maximum(m, jnp.max(s, axis=0, keepdims=True))
                    e = jnp.exp2(s - mn).astype(BF16)
                    o = lax.dot_general(vt[2 * p + hh, :, pl.ds(k0, 128)], e, NN, preferred_element_type=F32)
                    return mn, o + acc * jnp.exp2(m - mn)

                m0 = jnp.full((1, TQ), -jnp.inf, F32)
                _, acc = lax.fori_loop(0, NKT, kchunk, (m0, jnp.zeros((24, TQ), F32)))
                lax.cond(hh == 0, lambda: finish(p, 0, acc, pl.ds(c0, TQ)), lambda: finish(p, 1, acc, pl.ds(c0, TQ)))
                acar[...] = acc
                return c2

            lax.fori_loop(0, 2 * S // TQ, qtile, 0)

            def mac(lt, c2):
                cache = {}
                for _, task in mac_tasks(p, [lt]):
                    task(cache, None)
                return c2

            lax.fori_loop(0, LT, mac, 0)
            return carry

        lax.fori_loop(0, NP, fb2, 0)

    lax.cond(fast, attn_fast, attn_general)

    gw = gw_v[...].astype(F32).reshape(1, D)
    dv = dvec_v[...].astype(F32).reshape(1, D)

    drain(NP - 1)
    c0, o2, outs = 0, None, []
    for sb, oc in enumerate(OBS):
        ob, t0 = oc * C, c0 * C
        s0 = (sb % 2) * max(OBS) * LT
        yr = jnp.concatenate([ys[:, c0 + i].reshape(128, D) for i in range(oc)], axis=1)
        yi = jnp.concatenate([ys[:, NC + c0 + i].reshape(128, D) for i in range(oc)], axis=1)
        ar, br, ai, bi = yr[0:64], yr[64:128], yi[0:64], yi[64:128]
        ye = jnp.dot(dft_v[256:320, :], jnp.concatenate([ar + br, ai - bi], axis=0).astype(BF16),
                     preferred_element_type=F32)
        yo = jnp.dot(dft_v[320:384, :], jnp.concatenate([ar - br, ai + bi], axis=0).astype(BF16),
                     preferred_element_type=F32)
        for i in range(oc * LT):
            ysc[s0 + i, pl.ds(0, 64, stride=2), :] = ye[:, i * 128:(i + 1) * 128]
            ysc[s0 + i, pl.ds(1, 64, stride=2), :] = yo[:, i * 128:(i + 1) * 128]
        y = jnp.concatenate(
            [jnp.concatenate([ysc[s0 + i * LT + lt] for lt in range(LT)], axis=1) for i in range(oc)], axis=0)
        if oc > 1:
            o = ot[:, :, t0:t0 + ob].reshape(D, ob).astype(BF16).T
        elif o2 is None:
            o2 = ot[:, :, t0:t0 + 2 * C].reshape(D, 2 * C).astype(BF16).T
            o = o2[0:C]
        else:
            o, o2 = o2[C:2 * C], None
        a = jnp.dot(o, wo_v[...], preferred_element_type=F32)
        xf = x_v[t0:t0 + ob, :].astype(F32)
        g = jax.nn.sigmoid(jnp.sum(xf * gw, axis=-1, keepdims=True))
        b = xf * (y + kvb[t0:t0 + ob, :].astype(F32) * dv)
        out_v[t0:t0 + ob, :] = (b + g * (a - b)).astype(BF16)
        outs.append(cp_out(t0, ob))
        outs[-1].start()
        c0 += oc
    for c in outs:
        c.wait()


@jax.jit
def pallas_gated_mix__mha_block__ssm_conv_h3__prompt_kernel(A_x, A_wqkv, A_wo, B_q, B_k, B_v, B_shift_k,
        B_ssm_k, B_ssm_D, gate_w):
    del B_q
    hbm = pl.BlockSpec(memory_space=pl.ANY)
    return pl.pallas_call(
        _kernel,
        out_shape=jax.ShapeDtypeStruct((1, S, D), BF16),
        in_specs=[hbm] * 10,
        out_specs=hbm,
        scratch_shapes=[
            pltpu.VMEM((S, D), BF16),
            pltpu.VMEM((D, 3 * D), BF16),
            pltpu.VMEM((D, D), BF16),
            pltpu.VMEM((S + 16, D), BF16),
            pltpu.VMEM((S, D), BF16),
            pltpu.VMEM((D, S), BF16),
            pltpu.VMEM((S, D), BF16),
            pltpu.VMEM((4, D), BF16),
            pltpu.VMEM((D,), BF16),
            pltpu.VMEM((D,), BF16),
            pltpu.VMEM((384, 128), BF16),
            pltpu.VMEM((3 * D, D), BF16),
            pltpu.VMEM((H, 64, S), I8),
            pltpu.VMEM((NP, S, 128), I8),
            pltpu.VMEM((H, 24, S), F32),
            pltpu.VMEM((H, S), F32),
            pltpu.VMEM((NB, H, 128), F32),
            pltpu.VMEM((2, NB, H, 128), F32),
            pltpu.VMEM((32, S), F32),
            pltpu.VMEM((NP, 40, S), F32),
            pltpu.VMEM((S, D), BF16),
            pltpu.VMEM((16, 2 * NC, 8, D), F32),
            pltpu.VMEM((16, 2 * NC, 8, D), F32),
            pltpu.VMEM((16, 2 * NC, 8, D), F32),
            pltpu.VMEM((2 * max(OBS) * LT, 128, 128), F32),
            pltpu.VMEM((S, 128), BF16),
            pltpu.VMEM((2, 128, TQ), BF16),
            pltpu.VMEM((24, TQ), F32),
            pltpu.VMEM((3 * D, S), F32),
            pltpu.SemaphoreType.DMA((9,)),
        ],
        compiler_params=pltpu.CompilerParams(vmem_limit_bytes=120 * 1024 * 1024),
        name="gmix",
    )(A_x, A_wqkv, A_wo, B_k, B_v, B_ssm_k, B_shift_k.T, B_ssm_D, gate_w, jnp.asarray(_dft_tables(), BF16))
```
